```python
import os as _os
_os.environ.setdefault("JAX_PLATFORMS", "cpu")
import jax
import jax.numpy as jnp

def _softmax(x, axis=-1):
    return jax.nn.softmax(x, axis=axis)
def _gelu(x):
    return jax.nn.gelu(x, approximate=True)
def _silu(x):
    return jax.nn.silu(x)
def _sigmoid(x):
    return jax.nn.sigmoid(x)
def _layernorm(x, axis=-1, eps=1e-5):
    m = jnp.mean(x, axis=axis, keepdims=True)
    v = jnp.var(x, axis=axis, keepdims=True)
    return (x - m) / jnp.sqrt(v + eps)
def _scatter_add(tgt, idx, src, axis=0):
    return tgt.at[idx].add(src)
def _segment_sum(src, seg, n):
    return jax.ops.segment_sum(src, seg, n)
class _Rng:
    def __init__(self, key):
        self._k = key
    def _next(self):
        self._k, sub = jax.random.split(self._k)
        return sub
    def normal(self, shape):
        return jax.random.normal(self._next(), shape, dtype=jnp.bfloat16)
    def randint(self, lo, hi, shape):
        return jax.random.randint(self._next(), shape, lo, hi, dtype=jnp.int32)
    def uniform(self, shape, lo=0.0, hi=1.0):
        return jax.random.uniform(self._next(), shape, jnp.bfloat16, lo, hi)
    def permutation(self, n):
        return jax.random.permutation(self._next(), n)


kernel_name = 'concat_heads__spectral_gfnet__sliding_block__prompt'

def setup_inputs():
    _rng = _Rng(jax.random.key(int.from_bytes(__import__("os").urandom(4), "little")))
    _w = (lambda a: (lambda t: t.astype(jnp.bfloat16) if jnp.issubdtype(t.dtype, jnp.floating) else t)(jnp.asarray(a)))
    def _A_setup():
        B, S, D = 1, 2048, 640
        Df = D // 2 + 1
        return {
            "x": _w((lambda *s: _rng.normal(s) * 0.05)(B, S, D)),
            "w_r": _w((lambda *s: _rng.normal(s) * 0.4)(S, Df) * 0.02),
            "w_i": _w((lambda *s: _rng.normal(s) * 0.4)(S, Df) * 0.02),
        }
    _A_in = _A_setup()

    def _B_setup():
        B, S, D = 1, 2048, 640
        return {
            "x": _w((lambda *s: _rng.normal(s) * 0.2)(B, S, D)),
            "wqkv": _w((lambda *s: _rng.normal(s) * 0.2)(D, 3 * D)),
            "wo": _w((lambda *s: _rng.normal(s) * 0.05)(D, D)),
        }
    _B_in = _B_setup()

    return {
        "A_x": _A_in["x"],
        "A_w_r": _A_in["w_r"],
        "A_w_i": _A_in["w_i"],
        "B_x": _B_in["x"],
        "B_wqkv": _B_in["wqkv"],
        "B_wo": _B_in["wo"],
    }

def reference(A_x, A_w_r, A_w_i, B_x, B_wqkv, B_wo):
    def _A_ref(x, w_r, w_i):
        B, S, D = x.shape
        X = (lambda x, axes=(-2,-1): jnp.fft.rfft2(x.astype(jnp.float32), axes=axes))(x, axes=(-2, -1))
        W = w_r + 1j * w_i
        X = X * W
        y = (lambda x, s, axes=(-2,-1): jnp.fft.irfft2(x, s=s, axes=axes).astype(jnp.bfloat16))(X, (S, D), axes=(-2, -1))
        return y

    def _B_ref(x, wqkv, wo):
        B, S, D = x.shape
        H = 32; Dh = D // H; W = 256
        qkv = (lambda x, *d: x.transpose(*d))((x @ wqkv).reshape(B, S, 3, H, Dh), 2, 0, 3, 1, 4)
        q, k, v = qkv[0], qkv[1], qkv[2]
        scores = jnp.einsum("bhqd,bhkd->bhqk", q, k) * (Dh ** -0.5)
        idx = jnp.arange(S)
        mask = (idx[:, None] - idx[None, :] >= 0) & (idx[:, None] - idx[None, :] < W)
        scores = jnp.where(mask[None, None], scores, -1e9)
        p = _softmax(scores, axis=-1)
        o = jnp.einsum("bhqk,bhkd->bhqd", p, v)
        return (lambda x, *d: x.transpose(*d))(o, 0, 2, 1, 3).reshape(B, S, D) @ wo

    a = _A_ref(A_x, A_w_r, A_w_i)
    b = _B_ref(B_x, B_wqkv, B_wo)
    return jnp.concatenate([a, b], axis=-1)
```

```python
import numpy as np
import ml_dtypes
import jax
import jax.numpy as jnp
from jax import lax
import jax.experimental.pallas as pl
import jax.experimental.pallas.tpu as pltpu

S = 2048
D = 640
DF = 321
H = 32
DH = 20
NB = S // 128
R = 336
NEG = -1e30
f32 = jnp.float32
bf = jnp.bfloat16
i32 = jnp.int32

C1 = float(np.cos(2 * np.pi / 5))
C2 = float(np.cos(4 * np.pi / 5))
S1 = float(np.sin(2 * np.pi / 5))
S2 = float(np.sin(4 * np.pi / 5))


def _pack_rows(a):
    u = np.ascontiguousarray(a.astype(ml_dtypes.bfloat16)).view(np.uint16).astype(np.uint32)
    return (u[..., 0::2, :] | (u[..., 1::2, :] << 16)).astype(np.uint32).view(np.int32)


def _make_consts():
    b5 = np.arange(128)

    def cs(k):
        th = 2 * np.pi * np.outer(k, b5) / D
        return np.cos(th), np.sin(th)

    k0 = 5 * np.arange(65)
    c, s = cs(k0)
    F0 = np.zeros((160, 256))
    F0[0:65, 0:128] = c
    F0[80:145, 0:128] = -s

    def fwd(j):
        ka = j + 5 * np.arange(64)
        kb = (5 - j) + 5 * np.arange(64)
        ca, sa = cs(ka)
        cb, sb = cs(kb)
        F = np.zeros((256, 256))
        F[0:64, 0:128] = ca;      F[0:64, 128:256] = -sa
        F[128:192, 0:128] = -sa;  F[128:192, 128:256] = -ca
        F[64:128, 0:128] = cb;    F[64:128, 128:256] = sb
        F[192:256, 0:128] = -sb;  F[192:256, 128:256] = cb
        return F

    FF = np.concatenate([F0, fwd(1), fwd(2)], 0)

    b = np.arange(128)
    f2 = np.arange(128)
    RR = np.zeros((16, 256, 256))
    for a in range(16):
        th = -2 * np.pi * (np.outer(b, f2) / 128.0 + a * f2[None, :] / float(S))
        Mr, Mi = np.cos(th), np.sin(th)
        RR[a, 0:128, 0:128] = Mr
        RR[a, 0:128, 128:256] = Mi
        RR[a, 128:256, 0:128] = -Mi
        RR[a, 128:256, 128:256] = Mr

    sc = 1.0 / (S * D)
    G0 = np.zeros((128, 256))
    al = np.full(65, 2.0)
    al[0] = 1.0
    al[64] = 1.0
    G0[:, 0:64] = (al[0:64, None] * c[0:64]).T
    G0[:, 64:128] = (-al[0:64, None] * s[0:64]).T
    G0[:, 64] = al[64] * c[64]

    def inv(j):
        ka = j + 5 * np.arange(64)
        kb = (5 - j) + 5 * np.arange(64)
        ca, sa = cs(ka)
        cb, sb = cs(kb)
        G = np.zeros((256, 256))
        G[0:128, 0:64] = 2 * ca.T;     G[0:128, 128:192] = -2 * sa.T
        G[128:256, 0:64] = 2 * sa.T;   G[128:256, 128:192] = 2 * ca.T
        G[0:128, 64:128] = 2 * cb.T;   G[0:128, 192:256] = -2 * sb.T
        G[128:256, 64:128] = -2 * sb.T; G[128:256, 192:256] = -2 * cb.T
        return G

    GG = np.concatenate([G0, inv(1), inv(2)], 0) * sc
    return _pack_rows(FF), _pack_rows(GG), _pack_rows(RR)


_NT = (((1,), (1,)), ((), ()))


def _dot(a, b):
    return jnp.dot(a, b, preferred_element_type=f32)


def _dot_nt(a, b):
    return lax.dot_general(a, b, _NT, preferred_element_type=f32)


def _b16(x):
    return pltpu.bitcast(x, bf)


def _packi(a, b):
    return pltpu.pack_elementwise([a, b], packed_dtype=bf)


def _unpacki(x, idx):
    return pltpu.unpack_elementwise(x, index=idx, packed_dtype=bf, unpacked_dtype=f32)


def _dft4(z, inv):
    (a, b, c, d) = z
    t0 = (a[0] + c[0], a[1] + c[1])
    t1 = (a[0] - c[0], a[1] - c[1])
    t2 = (b[0] + d[0], b[1] + d[1])
    t3 = (b[0] - d[0], b[1] - d[1])
    o0 = (t0[0] + t2[0], t0[1] + t2[1])
    o2 = (t0[0] - t2[0], t0[1] - t2[1])
    p = (t1[0] + t3[1], t1[1] - t3[0])
    q = (t1[0] - t3[1], t1[1] + t3[0])
    return [o0, q, o2, p] if inv else [o0, p, o2, q]


def _tw16(z, e, inv):
    if e == 0:
        return z
    zr, zi = z
    if e == 4:
        return (-zi, zr) if inv else (zi, -zr)
    h = float(np.sqrt(0.5))
    if e == 2:
        return ((zr - zi) * h, (zr + zi) * h) if inv else ((zr + zi) * h, (zi - zr) * h)
    if e == 6:
        return ((-zr - zi) * h, (zr - zi) * h) if inv else ((zi - zr) * h, (-zr - zi) * h)
    sgn = 1.0 if inv else -1.0
    c = float(np.cos(2 * np.pi * e / 16))
    s = float(sgn * np.sin(2 * np.pi * e / 16))
    return (zr * c - zi * s, zr * s + zi * c)


def _fft16(z, inv):
    hh = [_dft4([z[a0 + 4 * a1] for a1 in range(4)], inv) for a0 in range(4)]
    out = [None] * 16
    for fa in range(4):
        o = _dft4([_tw16(hh[a0][fa], a0 * fa, inv) for a0 in range(4)], inv)
        for fb in range(4):
            out[fa + 4 * fb] = o[fb]
    return out


def _gwin(g):
    lo, hi = 80 * g, 80 * g + 79
    if lo // 128 == hi // 128:
        return ("nat", lo // 128, lo - 128 * (lo // 128))
    t = (lo - 64) // 128
    return ("shf", t, lo - 64 - 128 * t)


def _kernel(xa_hbm, wr_hbm, wi_hbm, xb_hbm, wqkv_hbm, wo_hbm, ff_hbm, gg_hbm, rr_hbm, out_hbm,
            xa32, wtr, wti, w32r, w32i, ff32, gg32, rr32, ys_ref, zs_ref, ysc_ref, oa32,
            xb32, wqkv32, wo32, wvt_ref, s_ref, p_ref, ob_ref, ot_ref, qw_ref, xu_ref, obo_ref,
            sem, osem, *groups):
    gs_refs = groups[0:3]
    kw_refs = groups[3:11]
    vt_refs = groups[11:19]

    def copy(src, dst, k):
        return pltpu.make_async_copy(src, dst, sem.at[k])

    xbh = xb_hbm.bitcast(i32)
    wqh = wqkv_hbm.bitcast(i32)
    c_x0 = copy(xbh.at[pl.ds(0, 128)], xb32.at[pl.ds(0, 128)], 0)
    c_wkv = copy(wqh.at[:, pl.ds(640, 1280)], wqkv32.at[:, pl.ds(640, 1280)], 1)
    c_x0.start()
    c_wkv.start()
    c_x0.wait()
    c_wkv.wait()
    c_wq = copy(wqh.at[:, pl.ds(0, 640)], wqkv32.at[:, pl.ds(0, 640)], 2)
    c_x1 = copy(xbh.at[pl.ds(128, 896)], xb32.at[pl.ds(128, 896)], 3)
    xah = xa_hbm.bitcast(i32)
    c_xa = [copy(xah.at[:, pl.ds(128 * t, 128)], xa32.at[t], 4 + t) for t in range(5)]
    c_ff = copy(ff_hbm, ff32, 9)
    c_rr0 = copy(rr_hbm.at[pl.ds(0, 4)], rr32.at[pl.ds(0, 4)], 10)
    c_rr1 = copy(rr_hbm.at[pl.ds(4, 12)], rr32.at[pl.ds(4, 12)], 11)
    for cp in [c_wq, c_x1] + c_xa + [c_ff, c_rr0, c_rr1]:
        cp.start()

    scale = float(DH ** -0.5 * np.log2(np.e))
    rr_ = lax.broadcasted_iota(i32, (32, 128), 0)
    ll_ = lax.broadcasted_iota(i32, (32, 128), 1) & 31
    pos_ = rr_ & 15
    key_ = (rr_ & 16) + jnp.where(pos_ < 8, 2 * pos_, 2 * (pos_ - 8) + 1)
    le32 = key_ <= ll_
    wr_ = lax.broadcasted_iota(i32, (16, 128), 0)
    wq_ = lax.broadcasted_iota(i32, (16, 128), 1) & 31
    le_pk = (jnp.where(2 * wr_ <= wq_, jnp.int32(0xFFFF), jnp.int32(0))
             | jnp.where(2 * wr_ + 1 <= wq_, jnp.int32(-65536), jnp.int32(0)))
    lane8 = lax.broadcasted_iota(i32, (8, 128), 1)
    lane16 = lax.broadcasted_iota(i32, (16, 128), 1)
    bit0 = (lane16 & 32) != 0
    bit1 = (lane16 & 64) != 0
    bit0_8 = (lane8 & 32) != 0
    sub4 = lax.broadcasted_iota(i32, (8, 128), 0) < 4
    sub0 = lax.broadcasted_iota(i32, (8, 128), 0) == 0
    ones8 = jnp.ones((8, 128), f32)
    lo64 = {64: lax.broadcasted_iota(i32, (64, 128), 1) < 64,
            128: lax.broadcasted_iota(i32, (128, 128), 1) < 64}

    def rows_of(i):
        return i * 128 if isinstance(i, int) else pl.multiple_of(i * 128, 128)

    def wrows_of(i):
        return i * 64 if isinstance(i, int) else pl.multiple_of(i * 64, 64)

    def prep_wvt():
        for tr in range(5):
            wvt_ref[tr * 128:(tr + 1) * 128, :] = _b16(wqkv32[:, 1280 + tr * 128:1280 + (tr + 1) * 128]).T

    def prep_x(i):
        w = xb32[pl.ds(wrows_of(i), 64), :]
        parts = []
        for gq in range(8):
            wg = w[8 * gq:8 * gq + 8]
            parts.append(_unpacki(wg, 0))
            parts.append(_unpacki(wg, 1))
        xu_ref[...] = jnp.concatenate(parts, 0).astype(bf)

    def win_ready(tiles, rolled, done, emit):
        for g in range(8):
            if g in done:
                continue
            kind, t, _ = _gwin(g)
            if kind == "nat":
                if t in tiles:
                    emit(g, tiles[t])
                    done.add(g)
            elif t in tiles and (t + 1) in tiles:
                for tt in (t, t + 1):
                    if tt not in rolled:
                        rolled[tt] = pltpu.roll(tiles[tt], 64, 1)
                emit(g, jnp.where(lo64[tiles[t].shape[0]], rolled[t], rolled[t + 1]))
                done.add(g)

    def proj_pieces(i, do_q=True, do_kv=True):
        pieces = {}
        r0 = rows_of(i)
        if do_kv:
            v8 = {}
            vdone = set()

            def vpiece(r):
                def f():
                    xb = _b16(xb32[pl.ds(wrows_of(i), 64), :])
                    vt = _dot_nt(wvt_ref[128 * r:128 * r + 128, :], xb)
                    for j in range(16):
                        v8[16 * r + j] = vt[8 * j:8 * j + 8]
                    for p in range(16):
                        if p in vdone or any((5 * p + j) not in v8 for j in range(5)):
                            continue
                        v = [v8[5 * p + j] for j in range(5)]
                        h0, h1 = 2 * p, 2 * p + 1
                        vt_refs[h0 // 4][h0 % 4, i] = jnp.concatenate([v[0], v[1], v[2], ones8], 0).astype(bf)
                        vt_refs[h1 // 4][h1 % 4, i] = jnp.concatenate([v[2], v[3], v[4], ones8], 0).astype(bf)
                        vdone.add(p)
                return f

            kt, kr, kd = {}, {}, set()

            def kpiece(t):
                def f():
                    kt[t] = _dot(xu_ref[...], _b16(wqkv32[:, 640 + 128 * t:640 + 128 * t + 128]))

                    def emit(g, val):
                        kw_refs[g][pl.ds(r0, 128), :] = val.astype(bf)
                    win_ready(kt, kr, kd, emit)
                return f

            for r in range(5):
                pieces["v%d" % r] = vpiece(r)
                pieces["k%d" % r] = kpiece(r)
        if do_q:
            qt, qr, qd = {}, {}, set()

            def qpiece(t):
                def f():
                    q = _dot(xu_ref[...], _b16(wqkv32[:, 128 * t:128 * t + 128])) * scale
                    qt[t] = jnp.concatenate(
                        [_packi(q[16 * j:16 * j + 8], q[16 * j + 8:16 * j + 16]) for j in range(8)], 0)

                    def emit(g, val):
                        qw_ref[g] = val
                    win_ready(qt, qr, qd, emit)
                return f

            for t in range(5):
                pieces["q%d" % t] = qpiece(t)
        return pieces

    def out_pieces(i):
        def opiece(t):
            def f():
                res = _dot(ob_ref[...], _b16(wo32[:, 128 * t:128 * t + 128]))
                obo_ref[pl.ds(rows_of(i), 128), 128 * t:128 * t + 128] = res.astype(bf)
            return f
        return {"o%d" % t: opiece(t) for t in range(5)}

    def key_tiles(i):
        return list(range(3)) if (not isinstance(i, int) or i >= 2) else list(range(2 - i, 3))

    def pv_group(g, i):
        tiles = key_tiles(i)
        sl = g % 2
        outs = []
        for e in range(4):
            P = _b16(p_ref[sl, e, 64 * tiles[0]:192, :])
            if len(tiles) > 1:
                vw = jnp.concatenate([vt_refs[g][e, i - 2 + j] for j in tiles], 1)
            else:
                vw = vt_refs[g][e, i]
            o = _dot(vw, P)
            rl = pltpu.reciprocal(o[24:32])
            res = [o[0:8] * rl, o[8:16] * rl, o[16:24] * rl]
            if e == 2:
                res = [pltpu.roll(r, 64, 1) for r in res]
            elif e == 1:
                res = [jnp.where(bit0_8, pltpu.roll(r, 32, 1), pltpu.roll(r, 96, 1)) for r in res]
            elif e == 3:
                res = [jnp.where(bit0_8, pltpu.roll(r, 96, 1), pltpu.roll(r, 32, 1)) for r in res]
            outs.append(res)
        ot = []
        for p in range(2):
            a, b = outs[2 * p], outs[2 * p + 1]
            ot += [a[0], a[1], jnp.where(sub4, a[2], b[0]), b[1], b[2]]
        ot_ref[80 * g:80 * g + 80, :] = jnp.concatenate(ot, 0)

    def fin_tile(t):
        ob_ref[:, 128 * t:128 * t + 128] = ot_ref[128 * t:128 * t + 128, :].T.astype(bf)

    def finish(i):
        def f():
            pv_group(7, i)
            fin_tile(4)
        return f

    def attn(i, plan, head=None):
        static = isinstance(i, int)
        lov = (lambda u: max(0, 8 - u - 4 * i)) if static else (lambda u: 0)
        tiles = key_tiles(i)
        ms = {}

        def phase_a(g):
            sl = g % 2
            _, _, off = _gwin(g)
            hm = [jnp.where((lane16 >= off + 20 * e) & (lane16 < off + 20 * e + 20), jnp.int32(-1), jnp.int32(0))
                  for e in range(4)]
            for u in range(4):
                lo = lov(u)
                nrow = 32 * (9 - lo)
                k0 = 128 * i - 256 + 32 * u + 32 * lo
                if not static:
                    k0 = pl.multiple_of(k0, 32)
                kw = kw_refs[g][pl.ds(k0, nrow), :]
                qu = qw_ref[g, 16 * u:16 * u + 16, :]
                qm = _b16(jnp.concatenate([qu & hm[lam ^ u] for lam in range(4)], 0))
                s = _dot_nt(kw, qm)
                sd = s[nrow - 32:nrow]
                if lo == 0:
                    T = jnp.where(le32, sd, s[0:32])
                    F = s[32:256]
                else:
                    T = jnp.where(le32, sd, NEG)
                    F = s[0:nrow - 32]
                m = jnp.max(T, axis=0, keepdims=True)
                s_ref[sl, u, 0:32] = T
                if F.shape[0] > 0:
                    m = jnp.maximum(m, jnp.max(F, axis=0, keepdims=True))
                    s_ref[sl, u, 32:32 + F.shape[0]] = F
                ms[(g, u)] = m

        def sel(m, a, b):
            if a is None and b is None:
                return None
            if a is None:
                a = jnp.zeros((16, 128), i32)
            if b is None:
                b = jnp.zeros((16, 128), i32)
            return jnp.where(m, a, b)

        def phase_b1(g):
            sl = g % 2
            lo_ = [lov(u) for u in range(4)]
            nf = [7 if lo_[u] == 0 else 8 - lo_[u] for u in range(4)]

            def pblock(u, row0):
                p = jnp.exp2(s_ref[sl, u, row0:row0 + 32] - ms[(g, u)])
                return jnp.concatenate([_packi(p[16 * j:16 * j + 8], p[16 * j + 8:16 * j + 16]) for j in range(2)], 0)

            tri = {}

            def block(u, rel):
                if rel < 0 or rel > 8:
                    return None
                if rel == 0 or rel == 8:
                    if u not in tri:
                        pt = pblock(u, 0)
                        if lo_[u] == 0:
                            p8 = pt & le_pk
                            tri[u] = {8: p8, 0: pt ^ p8}
                        else:
                            tri[u] = {8: pt, 0: None}
                    return tri[u][rel]
                first = 8 - nf[u]
                if rel < first:
                    return None
                return pblock(u, 32 + 32 * (rel - first))

            for beta in range(4 * tiles[0], 12):
                src = [block(u, beta - u) for u in range(4)]
                a0 = sel(bit0, src[1], src[0])
                a1 = sel(bit0, src[0], src[1])
                c0 = sel(bit0, src[3], src[2])
                c1 = sel(bit0, src[2], src[3])
                o4 = [sel(bit1, c0, a0), sel(bit1, c1, a1), sel(bit1, a0, c0), sel(bit1, a1, c1)]
                for e in range(4):
                    p_ref[sl, e, 16 * beta:16 * beta + 16, :] = (
                        o4[e] if o4[e] is not None else jnp.zeros((16, 128), i32))

        for s in range(-1, 8):
            if s == -1 and head is not None:
                head()
            if 0 <= s + 1 < 8:
                phase_a(s + 1)
            if 0 <= s < 8:
                phase_b1(s)
            if 0 <= s - 1 < 8:
                pv_group(s - 1, i)
            for f in plan.get(s, []):
                f()
        for t in range(4):
            fin_tile(t)

    def a1_x(a):
        j, par = a // 2, a % 2
        x = [_unpacki(xa32[t, pl.ds(j, 128, stride=8), :], par) for t in range(5)]
        t1 = x[1] + x[4]
        t2 = x[2] + x[3]
        t3 = x[1] - x[4]
        t4 = x[2] - x[3]
        y0 = x[0] + t1 + t2
        y1r = x[0] + C1 * t1 + C2 * t2
        y2r = x[0] + C2 * t1 + C1 * t2
        y1i = S1 * t3 + S2 * t4
        y2i = S2 * t3 - S1 * t4
        o0 = _dot_nt(_b16(ff32[0:80, 0:128]), y0.astype(bf))
        o1 = _dot_nt(_b16(ff32[80:208, :]), jnp.concatenate([y1r, y1i], 1).astype(bf))
        o2 = _dot_nt(_b16(ff32[208:336, :]), jnp.concatenate([y2r, y2i], 1).astype(bf))
        yr = jnp.concatenate([o0[0:80], o1[0:128], o2[0:128]], 0)
        yi = jnp.concatenate([o0[80:160], o1[128:256], o2[128:256]], 0)
        ys_ref[a % 2] = jnp.concatenate([yr, yi], 1).astype(bf)

    def a1_y(a):
        g_ = _dot(ys_ref[a % 2], _b16(rr32[a]))
        for g in range(R // 8):
            gs_refs[g % 3][a, 8 * (g // 3):8 * (g // 3) + 8, :] = g_[8 * g:8 * g + 8]

    def wprep(t):
        for (src, dst) in ((wtr, w32r), (wti, w32i)):
            dst[t, 0:320, :] = src[0:320, 128 * t:128 * t + 128].astype(f32)
            dst[t, 320:328, :] = jnp.concatenate(
                [src[320:321, 128 * t:128 * t + 128].astype(f32), jnp.zeros((7, 128), f32)], 0)
            dst[t, 328:352, :] = jnp.zeros((24, 128), f32)

    def a2_group(n, gq):
        g = 3 * gq + n
        if isinstance(gq, int):
            cls = 0 if g < 10 else (1 if g < 18 else (4 if g < 26 else (2 if g < 34 else 3)))
            m0 = (g if g < 10 else (g - 10) % 8) * 8
            k0 = cls + 5 * m0
            r0 = 8 * gq
        else:
            cls = jnp.where(g < 10, 0, jnp.where(g < 18, 1, jnp.where(g < 26, 4, jnp.where(g < 34, 2, 3))))
            m0 = jnp.where(g < 10, g, (g - 10) & 7) * 8
            k0 = cls + 5 * m0
            r0 = pl.multiple_of(8 * gq, 8)
        gref = gs_refs[n]
        z = [(gref[a, pl.ds(r0, 8), 0:128], gref[a, pl.ds(r0, 8), 128:256]) for a in range(16)]
        X = _fft16(z, False)
        V = []
        for f1 in range(16):
            wr = w32r[f1, pl.ds(k0, 8, stride=5), :]
            wi = w32i[f1, pl.ds(k0, 8, stride=5), :]
            V.append((X[f1][0] * wr - X[f1][1] * wi, X[f1][0] * wi + X[f1][1] * wr))
        U = _fft16(V, True)
        for a in range(16):
            gref[a, pl.ds(r0, 8), 0:128] = U[a][0]
            gref[a, pl.ds(r0, 8), 128:256] = U[a][1]

    def a3_z(a):
        u = jnp.concatenate([gs_refs[g % 3][a, 8 * (g // 3):8 * (g // 3) + 8, :] for g in range(R // 8)], 0)
        zz = _dot_nt(u.astype(bf), _b16(rr32[a]))
        zr = zz[:, 0:128]
        zi = zz[:, 128:256]
        kop = jnp.concatenate([zr[0:64], jnp.where(sub0, zr[64:72], zi[0:8]), zi[8:64],
                               zr[80:208], zi[80:208], zr[208:336], zi[208:336]], 0)
        zs_ref[a % 2] = kop.astype(bf)

    def a3_d(a):
        sl = a % 2
        v0 = _dot(_b16(gg32[0:64, 0:128]), zs_ref[sl, 0:128, :])
        v1 = _dot(_b16(gg32[64:192, :]), zs_ref[sl, 128:384, :])
        v2 = _dot(_b16(gg32[192:320, :]), zs_ref[sl, 384:640, :])
        v1r, v1i, v2r, v2i = v1[0:128], v1[128:256], v2[0:128], v2[128:256]
        A1 = v0 + C1 * v1r + C2 * v2r
        A2 = v0 + C2 * v1r + C1 * v2r
        B1 = S1 * v1i + S2 * v2i
        B2 = S2 * v1i - S1 * v2i
        y = [v0 + v1r + v2r, A1 - B1, A2 - B2, A2 + B2, A1 + B1]
        if a % 2 == 0:
            for t in range(5):
                ysc_ref[t] = y[t]
        else:
            j = a // 2
            for t in range(5):
                pk = _packi(ysc_ref[t], y[t])
                oa32[t, pl.ds(j, 128, stride=8), :] = pk.T

    def run(pieces, order=None):
        for k in (order or list(pieces)):
            if k in pieces:
                pieces[k]()

    PLAN = {-1: ["v0", "v1"], 0: ["k0", "q0"], 1: ["k1", "q1", "a0"], 2: ["k2", "q2"], 3: ["o0", "o1", "a1"],
            4: ["k3", "q3"], 5: ["o2", "o3", "a2"], 6: ["o4", "v2"], 7: ["k4", "q4", "v3", "v4"]}

    def mkplan(pieces):
        return {s_: [pieces[k] for k in ks if k in pieces] for s_, ks in PLAN.items()}

    ORD = ["v0", "v1", "v2", "v3", "v4", "k0", "k1", "k2", "k3", "k4", "q0", "q1", "q2", "q3", "q4"]

    def out_b_copy(i):
        return pltpu.make_async_copy(obo_ref.at[pl.ds(rows_of(i), 128)],
                                     out_hbm.at[pl.ds(rows_of(i), 128), pl.ds(D, D)], osem.at[0])

    prep_wvt()
    prep_x(0)
    run(proj_pieces(0, do_q=False), ORD)
    c_x1.wait()
    prep_x(1)
    run(proj_pieces(1, do_q=False), ORD)
    c_wq.wait()
    prep_x(2)
    run(proj_pieces(2), ORD)
    prep_x(3)
    attn(2, mkplan(proj_pieces(3)))

    for cp in c_xa + [c_ff, c_rr0]:
        cp.wait()
    c_w = [copy(wr_hbm, wtr, 12), copy(wi_hbm, wti, 13)]
    c_wo = copy(wo_hbm.bitcast(i32), wo32, 14)
    c_gg = copy(gg_hbm, gg32, 15)
    for cp in c_w + [c_wo, c_gg]:
        cp.start()
    a1_x(0)
    for a in range(16):
        if a + 1 < 16:
            a1_x(a + 1)
        if a == 2:
            c_rr1.wait()
        a1_y(a)
        if a == 7:
            for cp in c_w:
                cp.wait()
        if a >= 8:
            wprep(2 * (a - 8))
            wprep(2 * (a - 8) + 1)
    c_wo.wait()

    def body(i, carry):
        nxt = jnp.minimum(i + 1, NB - 1)
        prep_x(nxt)
        P = proj_pieces(nxt)
        P.update(out_pieces(i - 1))
        for n in range(3):
            P["a%d" % n] = (lambda n=n: a2_group(n, i - 3))
        attn(i, mkplan(P), head=finish(i - 1))
        out_b_copy(i - 1).start()
        return carry

    lax.fori_loop(3, NB, body, 0)

    prep_x(0)
    P = proj_pieces(0, do_kv=False)
    finish(NB - 1)()
    for n in range(3):
        a2_group(n, 13)
        run(P, ["q%d" % n])
    run(P, ["q3", "q4"])

    c_gg.wait()
    a3_z(0)
    for a in range(16):
        if a + 1 < 16:
            a3_z(a + 1)
        a3_d(a)
    oh32 = out_hbm.bitcast(i32)
    c_oa = [pltpu.make_async_copy(oa32.at[t], oh32.at[:, pl.ds(128 * t, 128)], osem.at[1 + t]) for t in range(5)]
    for cp in c_oa:
        cp.start()

    prep_x(1)
    P = proj_pieces(1, do_kv=False)
    P.update(out_pieces(NB - 1))
    attn(0, mkplan(P))
    out_b_copy(NB - 1).start()
    attn(1, mkplan(out_pieces(0)), head=finish(0))
    out_b_copy(0).start()
    finish(1)()
    run(out_pieces(1))
    out_b_copy(1).start()

    for cp in c_oa:
        cp.wait()
    for i in range(NB):
        out_b_copy(i).wait()


def _build(FF32, GG32, RR32):
    scratch = [
        pltpu.VMEM((5, S // 2, 128), i32),
        pltpu.VMEM((DF, S), bf), pltpu.VMEM((DF, S), bf),
        pltpu.VMEM((16, 352, 128), f32), pltpu.VMEM((16, 352, 128), f32),
        pltpu.VMEM(FF32.shape, i32), pltpu.VMEM(GG32.shape, i32), pltpu.VMEM(RR32.shape, i32),
        pltpu.VMEM((2, R, 256), bf),
        pltpu.VMEM((2, 640, 128), bf),
        pltpu.VMEM((5, 128, 128), f32),
        pltpu.VMEM((5, S // 2, 128), i32),
        pltpu.VMEM((S // 2, D), i32),
        pltpu.VMEM((D // 2, 3 * D), i32),
        pltpu.VMEM((D // 2, D), i32),
        pltpu.VMEM((D, D), bf),
        pltpu.VMEM((2, 4, 256, 128), f32),
        pltpu.VMEM((2, 4, 192, 128), i32),
        pltpu.VMEM((128, D), bf),
        pltpu.VMEM((D, 128), f32),
        pltpu.VMEM((8, 64, 128), i32),
        pltpu.VMEM((128, D), bf),
        pltpu.VMEM((S, D), bf),
        pltpu.SemaphoreType.DMA((16,)),
        pltpu.SemaphoreType.DMA((6,)),
    ]
    scratch += [pltpu.VMEM((16, 112, 256), f32)] * 3
    scratch += [pltpu.VMEM((S, 128), bf)] * 8
    scratch += [pltpu.VMEM((4, NB, 32, 128), bf)] * 8
    return pl.pallas_call(
        _kernel,
        out_shape=jax.ShapeDtypeStruct((S, 2 * D), bf),
        in_specs=[pl.BlockSpec(memory_space=pl.ANY)] * 9,
        out_specs=pl.BlockSpec(memory_space=pl.ANY),
        scratch_shapes=scratch,
        compiler_params=pltpu.CompilerParams(vmem_limit_bytes=110 * 2 ** 20),
    )


@jax.jit
def pallas_concat_heads__spectral_gfnet__sliding_block__prompt_kernel(
    A_x: jax.Array,
    A_w_r: jax.Array,
    A_w_i: jax.Array,
    B_x: jax.Array,
    B_wqkv: jax.Array,
    B_wo: jax.Array,
):
    FF32, GG32, RR32 = _make_consts()
    out = _build(FF32, GG32, RR32)(
        A_x.reshape(S, D), A_w_r.T, A_w_i.T, B_x.reshape(S, D), B_wqkv, B_wo,
        jnp.asarray(FF32), jnp.asarray(GG32), jnp.asarray(RR32))
    return out.reshape(1, S, 2 * D)
```

```python
import numpy as np
import ml_dtypes
import jax
import jax.numpy as jnp
from jax import lax
import jax.experimental.pallas as pl
import jax.experimental.pallas.tpu as pltpu

S = 2048
D = 640
DF = 321
H = 32
DH = 20
NB = S // 128
R = 336
NEG = -1e30
CFG = {}
f32 = jnp.float32
bf = jnp.bfloat16
i32 = jnp.int32

C1 = float(np.cos(2 * np.pi / 5))
C2 = float(np.cos(4 * np.pi / 5))
S1 = float(np.sin(2 * np.pi / 5))
S2 = float(np.sin(4 * np.pi / 5))


def _pack_rows(a):
    u = np.ascontiguousarray(a.astype(ml_dtypes.bfloat16)).view(np.uint16).astype(np.uint32)
    return (u[..., 0::2, :] | (u[..., 1::2, :] << 16)).astype(np.uint32).view(np.int32)


def _make_consts():
    b5 = np.arange(128)

    def cs(k):
        th = 2 * np.pi * np.outer(k, b5) / D
        return np.cos(th), np.sin(th)

    m32 = np.arange(32)
    k0 = np.concatenate([10 * m32, 5 + 10 * m32, [320]])
    c, s = cs(k0)
    F0 = np.zeros((160, 256))
    F0[0:65, 0:128] = c
    F0[80:145, 0:128] = -s

    def fwd(j):
        ka = np.concatenate([j + 10 * m32, j + 5 + 10 * m32])
        kb = np.concatenate([5 - j + 10 * m32, 10 - j + 10 * m32])
        ca, sa = cs(ka)
        cb, sb = cs(kb)
        F = np.zeros((256, 256))
        F[0:64, 0:128] = ca;      F[0:64, 128:256] = -sa
        F[128:192, 0:128] = -sa;  F[128:192, 128:256] = -ca
        F[64:128, 0:128] = cb;    F[64:128, 128:256] = sb
        F[192:256, 0:128] = -sb;  F[192:256, 128:256] = cb
        return F

    FF = np.concatenate([F0, fwd(1), fwd(2)], 0)

    b = np.arange(128)
    f2 = np.arange(128)
    RR = np.zeros((16, 256, 256))
    for a in range(16):
        th = -2 * np.pi * (np.outer(b, f2) / 128.0 + a * f2[None, :] / float(S))
        Mr, Mi = np.cos(th), np.sin(th)
        RR[a, 0:128, 0:128] = Mr
        RR[a, 0:128, 128:256] = Mi
        RR[a, 128:256, 0:128] = -Mi
        RR[a, 128:256, 128:256] = Mr

    sc = 1.0 / (S * D)
    G0 = np.zeros((128, 256))
    al = np.full(65, 2.0)
    al[0] = 1.0
    al[64] = 1.0
    G0[:, 0:64] = (al[0:64, None] * c[0:64]).T
    G0[:, 64:128] = (-al[0:64, None] * s[0:64]).T
    G0[:, 64] = al[64] * c[64]

    def inv(j):
        ka = np.concatenate([j + 10 * m32, j + 5 + 10 * m32])
        kb = np.concatenate([5 - j + 10 * m32, 10 - j + 10 * m32])
        ca, sa = cs(ka)
        cb, sb = cs(kb)
        G = np.zeros((256, 256))
        G[0:128, 0:64] = 2 * ca.T;     G[0:128, 128:192] = -2 * sa.T
        G[128:256, 0:64] = 2 * sa.T;   G[128:256, 128:192] = 2 * ca.T
        G[0:128, 64:128] = 2 * cb.T;   G[0:128, 192:256] = -2 * sb.T
        G[128:256, 64:128] = -2 * sb.T; G[128:256, 192:256] = -2 * cb.T
        return G

    GG = np.concatenate([G0, inv(1), inv(2)], 0) * sc
    return _pack_rows(FF), _pack_rows(GG), _pack_rows(RR)


_NT = (((1,), (1,)), ((), ()))


def _dot(a, b):
    return jnp.dot(a, b, preferred_element_type=f32)


def _dot_nt(a, b):
    return lax.dot_general(a, b, _NT, preferred_element_type=f32)


def _b16(x):
    return pltpu.bitcast(x, bf)


def _packi(a, b):
    return pltpu.pack_elementwise([a, b], packed_dtype=bf)


def _unpacki(x, idx):
    return pltpu.unpack_elementwise(x, index=idx, packed_dtype=bf, unpacked_dtype=f32)


def _zip16(x):
    n = x.shape[0] // 16
    return jnp.concatenate([_packi(x[16 * j:16 * j + 8], x[16 * j + 8:16 * j + 16]) for j in range(n)], 0)


def _dft4(z, inv):
    (a, b, c, d) = z
    t0 = (a[0] + c[0], a[1] + c[1])
    t1 = (a[0] - c[0], a[1] - c[1])
    t2 = (b[0] + d[0], b[1] + d[1])
    t3 = (b[0] - d[0], b[1] - d[1])
    o0 = (t0[0] + t2[0], t0[1] + t2[1])
    o2 = (t0[0] - t2[0], t0[1] - t2[1])
    p = (t1[0] + t3[1], t1[1] - t3[0])
    q = (t1[0] - t3[1], t1[1] + t3[0])
    return [o0, q, o2, p] if inv else [o0, p, o2, q]


def _tw16(z, e, inv):
    if e == 0:
        return z
    zr, zi = z
    if e == 4:
        return (-zi, zr) if inv else (zi, -zr)
    h = float(np.sqrt(0.5))
    if e == 2:
        return ((zr - zi) * h, (zr + zi) * h) if inv else ((zr + zi) * h, (zi - zr) * h)
    if e == 6:
        return ((-zr - zi) * h, (zr - zi) * h) if inv else ((zi - zr) * h, (-zr - zi) * h)
    sgn = 1.0 if inv else -1.0
    c = float(np.cos(2 * np.pi * e / 16))
    s = float(sgn * np.sin(2 * np.pi * e / 16))
    return (zr * c - zi * s, zr * s + zi * c)


def _fft16(z, inv):
    hh = [_dft4([z[a0 + 4 * a1] for a1 in range(4)], inv) for a0 in range(4)]
    out = [None] * 16
    for fa in range(4):
        o = _dft4([_tw16(hh[a0][fa], a0 * fa, inv) for a0 in range(4)], inv)
        for fb in range(4):
            out[fa + 4 * fb] = o[fb]
    return out


def _gwin(g):
    lo, hi = 80 * g, 80 * g + 79
    if lo // 128 == hi // 128:
        return ("nat", lo // 128, lo - 128 * (lo // 128))
    t = (lo - 64) // 128
    return ("shf", t, lo - 64 - 128 * t)


def _kernel(xa_hbm, wr_hbm, wi_hbm, xb_hbm, wqkv_hbm, wo_hbm, ff_hbm, gg_hbm, rr_hbm, out_hbm,
            xa32, wr32, wi32, wr_last, wi_last, ff32, gg32, rr32, ys_ref, zs_ref, ysc_ref, oa32,
            xq32, xb32, wqkv32, wo32, wvt32, s_ref, p_ref, ob32, ot_ref, qw_ref, xz_ref, obo32,
            sem, osem, wsem, *groups):
    gs_refs = groups[0:3]
    kw_refs = groups[3:11]
    vt_refs = groups[11:19]

    def copy(src, dst, k):
        return pltpu.make_async_copy(src, dst, sem.at[k])

    xbh = xb_hbm.bitcast(i32)
    wqh = wqkv_hbm.bitcast(i32)
    xah = xa_hbm.bitcast(i32)
    oh32 = out_hbm.bitcast(i32)
    c_x0 = copy(xbh.at[pl.ds(0, 128)], xb32.at[pl.ds(0, 128)], 0)
    c_wk = copy(wqh.at[:, pl.ds(640, 640)], wqkv32.at[:, pl.ds(640, 640)], 1)
    c_wv = copy(wqh.at[:, pl.ds(1280, 640)], wqkv32.at[:, pl.ds(1280, 640)], 2)
    c_x1 = copy(xbh.at[pl.ds(128, 192)], xb32.at[pl.ds(128, 192)], 3)
    c_wq = copy(wqh.at[:, pl.ds(0, 640)], wqkv32.at[:, pl.ds(0, 640)], 4)
    c_ff = copy(ff_hbm, ff32, 5)
    c_xa = [copy(xah.at[:, pl.ds(128 * t, 128)], xa32.at[t], 6 + t) for t in range(5)]
    c_rr0 = copy(rr_hbm.at[pl.ds(0, 4)], rr32.at[pl.ds(0, 4)], 11)
    c_rr1 = copy(rr_hbm.at[pl.ds(4, 12)], rr32.at[pl.ds(4, 12)], 12)
    c_w = []
    for n, (src, dst, dst1) in enumerate(((wr_hbm, wr32, wr_last), (wi_hbm, wi32, wi_last))):
        w320 = src.at[pl.ds(0, 320)].bitcast(i32)
        for t in range(NB):
            c_w.append(pltpu.make_async_copy(w320.at[:, pl.ds(128 * t, 128)], dst.at[t], wsem.at[0]))
        c_w.append(copy(src.at[pl.ds(320, 1)], dst1, 13 + n))
    c_x2 = copy(xbh.at[pl.ds(320, 704)], xb32.at[pl.ds(320, 704)], 21)
    c_wo = copy(wo_hbm.bitcast(i32), wo32, 22)
    c_gg = copy(gg_hbm, gg32, 23)
    c_xq = copy(xbh.at[pl.ds(0, 128)], xq32, 24)
    for cp in ([c_x0, c_wk, c_wv, c_x1, c_wq, c_wo, c_ff] + c_xa + [c_rr0, c_rr1]
               + c_w + [c_x2, c_gg, c_xq]):
        cp.start()

    scale = float(DH ** -0.5 * np.log2(np.e))
    def _qpos(l):
        return (l & 16) + 4 * (l & 3) + ((l & 15) >> 2)
    rr_ = lax.broadcasted_iota(i32, (32, 128), 0)
    ll_ = _qpos(lax.broadcasted_iota(i32, (32, 128), 1))
    pos_ = rr_ & 15
    key_ = (rr_ & 16) + jnp.where(pos_ < 8, 2 * pos_, 2 * (pos_ - 8) + 1)
    le32 = key_ <= ll_
    wr_ = lax.broadcasted_iota(i32, (16, 128), 0)
    wq_ = _qpos(lax.broadcasted_iota(i32, (16, 128), 1))
    le_pk = (jnp.where(2 * wr_ <= wq_, jnp.int32(0xFFFF), jnp.int32(0))
             | jnp.where(2 * wr_ + 1 <= wq_, jnp.int32(-65536), jnp.int32(0)))
    lane8 = lax.broadcasted_iota(i32, (8, 128), 1)
    lane16 = lax.broadcasted_iota(i32, (16, 128), 1)
    bit0 = (lane16 & 32) != 0
    bit1 = (lane16 & 64) != 0
    bit0_8 = (lane8 & 32) != 0
    sub4 = lax.broadcasted_iota(i32, (8, 128), 0) < 4
    sub0 = lax.broadcasted_iota(i32, (8, 128), 0) == 0
    ones8 = jnp.ones((8, 128), f32)
    lo64 = lax.broadcasted_iota(i32, (64, 128), 1) < 64

    def rows_of(i):
        return i * 128 if isinstance(i, int) else pl.multiple_of(i * 128, 128)

    def wrows_of(i):
        return i * 64 if isinstance(i, int) else pl.multiple_of(i * 64, 64)

    def prep_wvt():
        for tr in range(5):
            wvt32[64 * tr:64 * tr + 64, :] = pltpu.bitcast(
                _b16(wqkv32[:, 1280 + tr * 128:1280 + (tr + 1) * 128]).T, i32)

    def prep_x(i, src=None):
        w = (xb32 if src is None else src)[pl.ds(wrows_of(i), 64), :]
        z1 = _zip16(_b16(w).astype(f32))
        xz_ref[0] = z1
        xz_ref[1] = _zip16(_b16(z1).astype(f32))

    def win_ready(tiles, rolled, done, emit):
        for g in range(8):
            if g in done:
                continue
            kind, t, _ = _gwin(g)
            if kind == "nat":
                if t in tiles:
                    emit(g, tiles[t])
                    done.add(g)
            elif t in tiles and (t + 1) in tiles:
                for tt in (t, t + 1):
                    if tt not in rolled:
                        rolled[tt] = pltpu.roll(tiles[tt], 64, 1)
                emit(g, jnp.where(lo64, rolled[t], rolled[t + 1]))
                done.add(g)

    def proj_pieces(i, do_q=True, do_kv=True):
        pieces = {}
        if do_kv:
            v8 = {}
            vdone = set()

            def vpiece(r):
                def f():
                    xb = _b16(xb32[pl.ds(wrows_of(i), 64), :])
                    vt = _dot_nt(_b16(wvt32[64 * r:64 * r + 64, :]), xb)
                    for j in range(16):
                        v8[16 * r + j] = vt[8 * j:8 * j + 8]
                    for p in range(16):
                        if p in vdone or any((5 * p + j) not in v8 for j in range(5)):
                            continue
                        v = [v8[5 * p + j] for j in range(5)]
                        h0, h1 = 2 * p, 2 * p + 1
                        vt_refs[h0 // 4][h0 % 4, i] = jnp.concatenate([v[0], v[1], v[2], ones8], 0).astype(bf)
                        vt_refs[h1 // 4][h1 % 4, i] = jnp.concatenate([v[2], v[3], v[4], ones8], 0).astype(bf)
                        vdone.add(p)
                return f

            kt, kr, kd = {}, {}, set()

            def kpiece(t):
                def f():
                    kt[t] = _zip16(_dot(_b16(xz_ref[1]), _b16(wqkv32[:, 640 + 128 * t:640 + 128 * t + 128])))

                    def emit(g, val):
                        kw_refs[g][pl.ds(wrows_of(i), 64), :] = val
                    win_ready(kt, kr, kd, emit)
                return f

            for r in range(5):
                pieces["v%d" % r] = vpiece(r)
                pieces["k%d" % r] = kpiece(r)
        if do_q:
            qt, qr, qd = {}, {}, set()

            def qpiece(t):
                def f():
                    qt[t] = _zip16(_dot(_b16(xz_ref[0]), _b16(wqkv32[:, 128 * t:128 * t + 128])) * scale)

                    def emit(g, val):
                        qw_ref[g] = val
                    win_ready(qt, qr, qd, emit)
                return f

            for t in range(5):
                pieces["q%d" % t] = qpiece(t)
        return pieces

    def out_pieces(i):
        def opiece(t):
            def f():
                res = _dot(_b16(ob32[...]), _b16(wo32[:, 128 * t:128 * t + 128]))
                obo32[pl.ds(wrows_of(i), 64), 128 * t:128 * t + 128] = _zip16(res)
            return f
        return {"o%d" % t: opiece(t) for t in range(5)}

    NSL = CFG.get('slots', 2)

    def key_tiles(i):
        return list(range(3)) if (not isinstance(i, int) or i >= 2) else list(range(2 - i, 3))

    pv_outs = {}
    last_pv = [None]

    def pv_group(g, i, es=(0, 1, 2, 3)):
        tiles = key_tiles(i)
        sl = g % NSL
        for e in es:
            P = _b16(p_ref[sl, e, 64 * tiles[0]:192, :])
            if len(tiles) > 1:
                vw = jnp.concatenate([vt_refs[g][e, i - 2 + j] for j in tiles], 1)
            else:
                vw = vt_refs[g][e, i]
            o = _dot(vw, P)
            rl = pltpu.reciprocal(o[24:32])
            res = [o[0:8] * rl, o[8:16] * rl, o[16:24] * rl]
            if e == 2:
                res = [pltpu.roll(r, 64, 1) for r in res]
            elif e == 1:
                res = [jnp.where(bit0_8, pltpu.roll(r, 32, 1), pltpu.roll(r, 96, 1)) for r in res]
            elif e == 3:
                res = [jnp.where(bit0_8, pltpu.roll(r, 96, 1), pltpu.roll(r, 32, 1)) for r in res]
            pv_outs[(g, e)] = res
            last_pv[0] = rl
            if (g, e ^ 1) in pv_outs:
                p = e // 2
                a, b = pv_outs.pop((g, 2 * p)), pv_outs.pop((g, 2 * p + 1))
                ot_ref[80 * g + 40 * p:80 * g + 40 * p + 40, :] = jnp.concatenate(
                    [a[0], a[1], jnp.where(sub4, a[2], b[0]), b[1], b[2]], 0)

    def fin_tile(t):
        ob32[:, 128 * t:128 * t + 128] = _zip16(ot_ref[128 * t:128 * t + 128, :].T)

    def finish(i):
        def f():
            pv_group(7, i)
            fin_tile(4)
        return f

    last_m = {}

    def token(n):
        kind = CFG.get("tok", {"0": "m", "1": "m", "2": "m"}).get(str(n))
        if kind == "m":
            g, u = max(last_m)
            return jnp.broadcast_to(last_m[(g, u)], (8, 128))
        if kind == "p":
            return last_pv[0]
        return None

    def attn(i, plan, head=None):
        static = isinstance(i, int)
        lov = (lambda u: max(0, 8 - u - 4 * i)) if static else (lambda u: 0)
        tiles = key_tiles(i)
        ms = last_m

        def phase_a(g, us):
            sl = g % NSL
            _, _, off = _gwin(g)
            hm = [jnp.where((lane16 >= off + 20 * e) & (lane16 < off + 20 * e + 20), jnp.int32(-1), jnp.int32(0))
                  for e in range(4)]
            for u in us:
                lo = lov(u)
                nrow = 32 * (9 - lo)
                k0 = 64 * i - 128 + 16 * u + 16 * lo
                if not static:
                    k0 = pl.multiple_of(k0, 16)
                kw = _b16(kw_refs[g][pl.ds(k0, nrow // 2), :])
                qu = qw_ref[g, 16 * u:16 * u + 16, :]
                qm = _b16(jnp.concatenate([qu & hm[lam ^ u] for lam in range(4)], 0))
                s = _dot_nt(kw, qm)
                sd = s[nrow - 32:nrow]
                if lo == 0:
                    T = jnp.where(le32, sd, s[0:32])
                    F = s[32:256]
                else:
                    T = jnp.where(le32, sd, NEG)
                    F = s[0:nrow - 32]
                m = jnp.max(T, axis=0, keepdims=True)
                s_ref[sl, u, 0:32] = T
                if F.shape[0] > 0:
                    m = jnp.maximum(m, jnp.max(F, axis=0, keepdims=True))
                    s_ref[sl, u, 32:32 + F.shape[0]] = F
                ms[(g, u)] = m

        def sel(m, a, b):
            if a is None and b is None:
                return None
            if a is None:
                a = jnp.zeros((16, 128), i32)
            if b is None:
                b = jnp.zeros((16, 128), i32)
            return jnp.where(m, a, b)

        def phase_b1(g):
            sl = g % NSL
            lo_ = [lov(u) for u in range(4)]
            nf = [7 if lo_[u] == 0 else 8 - lo_[u] for u in range(4)]

            def pblock(u, row0):
                p = jnp.exp2(s_ref[sl, u, row0:row0 + 32] - ms[(g, u)])
                return jnp.concatenate([_packi(p[16 * j:16 * j + 8], p[16 * j + 8:16 * j + 16]) for j in range(2)], 0)

            tri = {}

            def block(u, rel):
                if rel < 0 or rel > 8:
                    return None
                if rel == 0 or rel == 8:
                    if u not in tri:
                        pt = pblock(u, 0)
                        if lo_[u] == 0:
                            p8 = pt & le_pk
                            tri[u] = {8: p8, 0: pt ^ p8}
                        else:
                            tri[u] = {8: pt, 0: None}
                    return tri[u][rel]
                first = 8 - nf[u]
                if rel < first:
                    return None
                return pblock(u, 32 + 32 * (rel - first))

            for beta in range(4 * tiles[0], 12):
                src = [block(u, beta - u) for u in range(4)]
                a0 = sel(bit0, src[1], src[0])
                a1 = sel(bit0, src[0], src[1])
                c0 = sel(bit0, src[3], src[2])
                c1 = sel(bit0, src[2], src[3])
                o4 = [sel(bit1, c0, a0), sel(bit1, c1, a1), sel(bit1, a0, c0), sel(bit1, a1, c1)]
                for e in range(4):
                    p_ref[sl, e, 16 * beta:16 * beta + 16, :] = (
                        o4[e] if o4[e] is not None else jnp.zeros((16, 128), i32))

        order = CFG.get("order", "A0 P0 A1 A2 P1 A3 P2 X X P3 B Y")
        for s in range(-1, 8):
            if s == -1 and head is not None:
                head()
            px = plan.get(s, [])
            todo = list(range(len(px)))
            for tok in order.split():
                if tok[0] == "A" and 0 <= s + 1 < 8:
                    phase_a(s + 1, [int(c) for c in tok[1:]])
                if tok[0] == "B" and 0 <= s < 8:
                    phase_b1(s)
                if tok[0] == "P" and 0 <= s - 1 < 8:
                    pv_group(s - 1, i, [int(c) for c in tok[1:]])
                if tok[0] == "X" and todo:
                    px[todo.pop(0)]()
                if tok[0] == "Y":
                    while todo:
                        px[todo.pop(0)]()
            while todo:
                px[todo.pop(0)]()
        for t in range(4):
            fin_tile(t)

    def a1_x(a):
        j, par = a // 2, a % 2
        x = [_unpacki(xa32[t, pl.ds(j, 128, stride=8), :], par) for t in range(5)]
        t1 = x[1] + x[4]
        t2 = x[2] + x[3]
        t3 = x[1] - x[4]
        t4 = x[2] - x[3]
        y0 = x[0] + t1 + t2
        y1r = x[0] + C1 * t1 + C2 * t2
        y2r = x[0] + C2 * t1 + C1 * t2
        y1i = S1 * t3 + S2 * t4
        y2i = S2 * t3 - S1 * t4
        o0 = _dot_nt(_b16(ff32[0:80, 0:128]), y0.astype(bf))
        o1 = _dot_nt(_b16(ff32[80:208, :]), jnp.concatenate([y1r, y1i], 1).astype(bf))
        o2 = _dot_nt(_b16(ff32[208:336, :]), jnp.concatenate([y2r, y2i], 1).astype(bf))
        yr = jnp.concatenate([o0[0:80], o1[0:128], o2[0:128]], 0)
        yi = jnp.concatenate([o0[80:160], o1[128:256], o2[128:256]], 0)
        ys_ref[a % 2] = jnp.concatenate([yr, yi], 1).astype(bf)

    def a1_y(a):
        g_ = _dot(ys_ref[a % 2], _b16(rr32[a]))
        for g in range(R // 8):
            gs_refs[g % 3][a, 8 * (g // 3):8 * (g // 3) + 8, :] = g_[8 * g:8 * g + 8]

    def a2_group(n, gq, token=None):
        g = 3 * gq + n
        special = isinstance(gq, int) and g == 8
        if isinstance(gq, int):
            w8 = g if g < 8 else (g - 10) % 8
            c10 = [0, 1, 4, 2, 3][0 if g < 8 else (g - 10) // 8 + 1] + 5 * (w8 // 4)
            r0 = 8 * gq
        else:
            w8 = jnp.where(g < 8, g, (g - 10) & 7)
            blk = jnp.where(g < 8, 0, ((g - 10) >> 3) + 1)
            c10 = jnp.where(blk == 2, 4, jnp.where(blk > 2, blk - 1, blk)) + 5 * (w8 >> 2)
            r0 = pl.multiple_of(8 * gq, 8)
        w0 = (c10 >> 1) + 40 * (w8 & 3)
        sh = 16 * (1 - (c10 & 1))

        def wload(ref, last, f1):
            if special:
                return jnp.broadcast_to(last[0:1, 128 * f1:128 * f1 + 128].astype(f32), (8, 128))
            return pltpu.bitcast((ref[f1, pl.ds(w0, 8, stride=5), :] << sh) & jnp.int32(-65536), f32)

        gref = gs_refs[n]
        if token is not None:
            gref[16, pl.ds(pl.multiple_of(8 * (gq & 15), 8), 8), 0:128] = token
        z = [(gref[a, pl.ds(r0, 8), 0:128], gref[a, pl.ds(r0, 8), 128:256]) for a in range(16)]
        X = _fft16(z, False)
        V = []
        for f1 in range(16):
            wr = wload(wr32, wr_last, f1)
            wi = wload(wi32, wi_last, f1)
            V.append((X[f1][0] * wr - X[f1][1] * wi, X[f1][0] * wi + X[f1][1] * wr))
        U = _fft16(V, True)
        for a in range(16):
            gref[a, pl.ds(r0, 8), 0:128] = U[a][0]
            gref[a, pl.ds(r0, 8), 128:256] = U[a][1]

    def a3_z(a):
        u = jnp.concatenate([gs_refs[g % 3][a, 8 * (g // 3):8 * (g // 3) + 8, :] for g in range(R // 8)], 0)
        zz = _dot_nt(u.astype(bf), _b16(rr32[a]))
        zr = zz[:, 0:128]
        zi = zz[:, 128:256]
        kop = jnp.concatenate([zr[0:64], jnp.where(sub0, zr[64:72], zi[0:8]), zi[8:64],
                               zr[80:208], zi[80:208], zr[208:336], zi[208:336]], 0)
        zs_ref[a % 2] = kop.astype(bf)

    def a3_d(a):
        sl = a % 2
        v0 = _dot(_b16(gg32[0:64, 0:128]), zs_ref[sl, 0:128, :])
        v1 = _dot(_b16(gg32[64:192, :]), zs_ref[sl, 128:384, :])
        v2 = _dot(_b16(gg32[192:320, :]), zs_ref[sl, 384:640, :])
        v1r, v1i, v2r, v2i = v1[0:128], v1[128:256], v2[0:128], v2[128:256]
        A1 = v0 + C1 * v1r + C2 * v2r
        A2 = v0 + C2 * v1r + C1 * v2r
        B1 = S1 * v1i + S2 * v2i
        B2 = S2 * v1i - S1 * v2i
        y = [v0 + v1r + v2r, A1 - B1, A2 - B2, A2 + B2, A1 + B1]
        if a % 2 == 0:
            for t in range(5):
                ysc_ref[t] = y[t]
        else:
            j = a // 2
            for t in range(5):
                pk = _packi(ysc_ref[t], y[t])
                oa32[t, pl.ds(j, 128, stride=8), :] = pk.T

    def run(pieces, order=None):
        for k in (order or list(pieces)):
            if k in pieces:
                pieces[k]()

    PLAN = {-1: ["v0", "v1"], 0: ["k0", "q0"], 1: ["k1", "q1"], 2: ["k2", "q2", "a0"], 3: ["o0", "o1"],
            4: ["k3", "q3", "a1"], 5: ["o2", "o3"], 6: ["o4", "v2", "a2"], 7: ["k4", "q4", "v3", "v4"]}

    if 'plan' in CFG:
        PLAN = {int(k): v for k, v in CFG['plan'].items()}

    def mkplan(pieces):
        return {s_: [pieces[k] for k in ks if k in pieces] for s_, ks in PLAN.items()}

    ORD = ["v0", "v1", "v2", "v3", "v4", "k0", "k1", "k2", "k3", "k4", "q0", "q1", "q2", "q3", "q4"]

    def out_b_copy(i):
        return pltpu.make_async_copy(obo32.at[pl.ds(wrows_of(i), 64)],
                                     oh32.at[pl.ds(wrows_of(i), 64), pl.ds(D, D)], osem.at[0])

    c_x0.wait()
    c_wk.wait()
    prep_x(0)
    P0 = proj_pieces(0, do_q=False)
    run(P0, ["k0", "k1", "k2", "k3", "k4"])
    prep_x(1)
    P1 = proj_pieces(1, do_q=False)
    run(P1, ["k0", "k1", "k2", "k3", "k4"])
    c_wv.wait()
    prep_wvt()
    run(P0, ["v0", "v1", "v2", "v3", "v4"])
    run(P1, ["v0", "v1", "v2", "v3", "v4"])
    c_x1.wait()
    c_wq.wait()
    prep_x(2)
    run(proj_pieces(2), ORD)
    c_wo.wait()
    prep_x(3)
    attn(2, mkplan(proj_pieces(3)))
    prep_x(4)
    P = proj_pieces(4)
    P.update(out_pieces(2))
    attn(3, mkplan(P), head=finish(2))

    for cp in [c_ff] + c_xa + [c_rr0]:
        cp.wait()
    a1_x(0)
    for a in range(16):
        if a + 1 < 16:
            a1_x(a + 1)
        if a == 3:
            c_rr1.wait()
        a1_y(a)
    for cp in c_w:
        cp.wait()
    c_x2.wait()

    def body(i, carry):
        nxt = jnp.minimum(i + 1, NB - 1)
        prep_x(nxt)
        P = proj_pieces(nxt)
        P.update(out_pieces(i - 1))
        for n in range(3):
            P["a%d" % n] = (lambda n=n: a2_group(n, (i - 4) + ((i - 4 >= [3, 99, 2][n]).astype(i32)), token(n)))
        last_m.clear()
        attn(i, mkplan(P), head=finish(i - 1))
        out_b_copy(i - 1).start()
        return carry

    out_b_copy(2).start()
    lax.fori_loop(4, NB, body, 0)

    finish(NB - 1)()
    P = out_pieces(NB - 1)
    for (n, gq), k in zip(((0, 13), (1, 12), (2, 13), (1, 13), (2, 2)), ("o0", "o1", "o2", "o3", "o4")):
        a2_group(n, gq)
        run(P, [k])
    out_b_copy(NB - 1).start()

    c_gg.wait()
    a3_z(0)
    for a in range(16):
        if a + 1 < 16:
            a3_z(a + 1)
        a3_d(a)
    c_oa = [pltpu.make_async_copy(oa32.at[t], oh32.at[:, pl.ds(128 * t, 128)], osem.at[1 + t]) for t in range(5)]
    for cp in c_oa:
        cp.start()

    c_xq.wait()
    prep_x(0, xq32)
    run(proj_pieces(0, do_kv=False), ORD)
    prep_x(1, xq32)
    attn(0, mkplan(proj_pieces(1, do_kv=False)))
    attn(1, mkplan(out_pieces(0)), head=finish(0))
    out_b_copy(0).start()
    finish(1)()
    run(out_pieces(1))
    out_b_copy(1).start()

    for cp in c_oa:
        cp.wait()
    for i in range(NB):
        out_b_copy(i).wait()


def _build(FF32, GG32, RR32):
    scratch = [
        pltpu.VMEM((5, S // 2, 128), i32),
        pltpu.VMEM((NB, 160, 128), i32), pltpu.VMEM((NB, 160, 128), i32),
        pltpu.VMEM((1, S), bf), pltpu.VMEM((1, S), bf),
        pltpu.VMEM(FF32.shape, i32), pltpu.VMEM(GG32.shape, i32), pltpu.VMEM(RR32.shape, i32),
        pltpu.VMEM((2, R, 256), bf),
        pltpu.VMEM((2, 640, 128), bf),
        pltpu.VMEM((5, 128, 128), f32),
        pltpu.VMEM((5, S // 2, 128), i32),
        pltpu.VMEM((128, D), i32),
        pltpu.VMEM((S // 2, D), i32),
        pltpu.VMEM((D // 2, 3 * D), i32),
        pltpu.VMEM((D // 2, D), i32),
        pltpu.VMEM((D // 2, D), i32),
        pltpu.VMEM((CFG.get('slots', 2), 4, 256, 128), f32),
        pltpu.VMEM((CFG.get('slots', 2), 4, 192, 128), i32),
        pltpu.VMEM((64, D), i32),
        pltpu.VMEM((D, 128), f32),
        pltpu.VMEM((8, 64, 128), i32),
        pltpu.VMEM((2, 64, D), i32),
        pltpu.VMEM((S // 2, D), i32),
        pltpu.SemaphoreType.DMA((25,)),
        pltpu.SemaphoreType.DMA((6,)),
        pltpu.SemaphoreType.DMA((1,)),
    ]
    scratch += [pltpu.VMEM((17, 112, 256), f32)] * 3
    scratch += [pltpu.VMEM((S // 2, 128), i32)] * 8
    scratch += [pltpu.VMEM((4, NB, 32, 128), bf)] * 8
    return pl.pallas_call(
        _kernel,
        out_shape=jax.ShapeDtypeStruct((S, 2 * D), bf),
        in_specs=[pl.BlockSpec(memory_space=pl.ANY)] * 9,
        out_specs=pl.BlockSpec(memory_space=pl.ANY),
        scratch_shapes=scratch,
        compiler_params=pltpu.CompilerParams(vmem_limit_bytes=110 * 2 ** 20),
    )


@jax.jit
def pallas_concat_heads__spectral_gfnet__sliding_block__prompt_kernel(
    A_x: jax.Array,
    A_w_r: jax.Array,
    A_w_i: jax.Array,
    B_x: jax.Array,
    B_wqkv: jax.Array,
    B_wo: jax.Array,
):
    FF32, GG32, RR32 = _make_consts()
    out = _build(FF32, GG32, RR32)(
        A_x.reshape(S, D), A_w_r.T, A_w_i.T, B_x.reshape(S, D), B_wqkv, B_wo,
        jnp.asarray(FF32), jnp.asarray(GG32), jnp.asarray(RR32))
    return out.reshape(1, S, 2 * D)
```

```python
import numpy as np
import ml_dtypes
import jax
import jax.numpy as jnp
from jax import lax
import jax.experimental.pallas as pl
import jax.experimental.pallas.tpu as pltpu

S = 2048
D = 640
DF = 321
H = 32
DH = 20
NB = S // 128
R = 336
NEG = -1e30
CFG = {}
f32 = jnp.float32
bf = jnp.bfloat16
i32 = jnp.int32

C1 = float(np.cos(2 * np.pi / 5))
C2 = float(np.cos(4 * np.pi / 5))
S1 = float(np.sin(2 * np.pi / 5))
S2 = float(np.sin(4 * np.pi / 5))


def _pack_rows(a):
    u = np.ascontiguousarray(a.astype(ml_dtypes.bfloat16)).view(np.uint16).astype(np.uint32)
    return (u[..., 0::2, :] | (u[..., 1::2, :] << 16)).astype(np.uint32).view(np.int32)


def _make_consts():
    b5 = np.arange(128)

    def cs(k):
        th = 2 * np.pi * np.outer(k, b5) / D
        return np.cos(th), np.sin(th)

    m32 = np.arange(32)
    k0 = np.concatenate([10 * m32, 5 + 10 * m32, [320]])
    c, s = cs(k0)
    F0 = np.zeros((160, 128))
    F0[0:65] = c
    F0[80:145] = -s

    def kpair(j):
        return (np.concatenate([j + 10 * m32, j + 5 + 10 * m32]),
                np.concatenate([5 - j + 10 * m32, 10 - j + 10 * m32]))

    def fwd(j):
        ka, kb = kpair(j)
        (ca, sa), (cb, sb) = cs(ka), cs(kb)
        return np.concatenate([ca, cb, ca + sa, cb - sb, ca - sa, cb + sb], 0)

    FF = np.concatenate([F0, fwd(1), fwd(2)], 0)

    b = np.arange(128)
    f2 = np.arange(128)
    RR = np.zeros((16, 3, 128, 128))
    for a in range(16):
        th = -2 * np.pi * (np.outer(b, f2) / 128.0 + a * f2[None, :] / float(S))
        Mr, Mi = np.cos(th), np.sin(th)
        RR[a, 0] = Mr
        RR[a, 1] = Mr + Mi
        RR[a, 2] = Mr - Mi

    sc = 1.0 / (S * D)
    G0 = np.zeros((128, 128))
    al = np.full(65, 2.0)
    al[0] = 1.0
    al[64] = 1.0
    G0[:, 0:64] = (al[0:64, None] * c[0:64]).T
    G0[:, 64:128] = (-al[0:64, None] * s[0:64]).T
    G0[:, 64] = al[64] * c[64]

    def inv(j):
        ka, kb = kpair(j)
        (ca, sa), (cb, sb) = cs(ka), cs(kb)
        return 2 * np.concatenate([np.concatenate([ca, cb], 0).T,
                                   np.concatenate([ca + sa, sb - cb], 0).T,
                                   np.concatenate([sa - ca, -sb - cb], 0).T], 0)

    GG = np.concatenate([G0, inv(1), inv(2)], 0) * sc
    return _pack_rows(FF), _pack_rows(GG), _pack_rows(RR)


_NT = (((1,), (1,)), ((), ()))


def _dot(a, b):
    return jnp.dot(a, b, preferred_element_type=f32)


def _dot_nt(a, b):
    return lax.dot_general(a, b, _NT, preferred_element_type=f32)


def _b16(x):
    return pltpu.bitcast(x, bf)


def _packi(a, b):
    return pltpu.pack_elementwise([a, b], packed_dtype=bf)


def _unpacki(x, idx):
    return pltpu.unpack_elementwise(x, index=idx, packed_dtype=bf, unpacked_dtype=f32)


def _zip16(x):
    n = x.shape[0] // 16
    return jnp.concatenate([_packi(x[16 * j:16 * j + 8], x[16 * j + 8:16 * j + 16]) for j in range(n)], 0)


def _dft4(z, inv):
    (a, b, c, d) = z
    t0 = (a[0] + c[0], a[1] + c[1])
    t1 = (a[0] - c[0], a[1] - c[1])
    t2 = (b[0] + d[0], b[1] + d[1])
    t3 = (b[0] - d[0], b[1] - d[1])
    o0 = (t0[0] + t2[0], t0[1] + t2[1])
    o2 = (t0[0] - t2[0], t0[1] - t2[1])
    p = (t1[0] + t3[1], t1[1] - t3[0])
    q = (t1[0] - t3[1], t1[1] + t3[0])
    return [o0, q, o2, p] if inv else [o0, p, o2, q]


def _tw16(z, e, inv):
    if e == 0:
        return z
    zr, zi = z
    if e == 4:
        return (-zi, zr) if inv else (zi, -zr)
    h = float(np.sqrt(0.5))
    if e == 2:
        return ((zr - zi) * h, (zr + zi) * h) if inv else ((zr + zi) * h, (zi - zr) * h)
    if e == 6:
        return ((-zr - zi) * h, (zr - zi) * h) if inv else ((zi - zr) * h, (-zr - zi) * h)
    sgn = 1.0 if inv else -1.0
    c = float(np.cos(2 * np.pi * e / 16))
    s = float(sgn * np.sin(2 * np.pi * e / 16))
    return (zr * c - zi * s, zr * s + zi * c)


def _fft16(z, inv):
    hh = [_dft4([z[a0 + 4 * a1] for a1 in range(4)], inv) for a0 in range(4)]
    out = [None] * 16
    for fa in range(4):
        o = _dft4([_tw16(hh[a0][fa], a0 * fa, inv) for a0 in range(4)], inv)
        for fb in range(4):
            out[fa + 4 * fb] = o[fb]
    return out


def _gwin(g):
    lo, hi = 80 * g, 80 * g + 79
    if lo // 128 == hi // 128:
        return ("nat", lo // 128, lo - 128 * (lo // 128))
    t = (lo - 64) // 128
    return ("shf", t, lo - 64 - 128 * t)


def _kernel(xa_hbm, wr_hbm, wi_hbm, xb_hbm, wqkv_hbm, wo_hbm, ff_hbm, gg_hbm, rr_hbm, out_hbm,
            xa32, wr32, wi32, wr_last, wi_last, ff32, gg32, rr32, ys_ref, zs_ref, ysc_ref, oa32,
            pin_ref, qw01_ref, xb32, wqkv32, wo32, wvt32, s_ref, p_ref, ob32, ot_ref, qw_ref, xz_ref, obo32,
            sem, osem, wsem, *groups):
    gs_refs = groups[0:4]
    kw_refs = groups[4:12]
    vt_refs = groups[12:20]

    def copy(src, dst, k):
        return pltpu.make_async_copy(src, dst, sem.at[k])

    xbh = xb_hbm.bitcast(i32)
    wqh = wqkv_hbm.bitcast(i32)
    xah = xa_hbm.bitcast(i32)
    oh32 = out_hbm.bitcast(i32)
    c_x0 = copy(xbh.at[pl.ds(0, 128)], xb32.at[pl.ds(0, 128)], 0)
    c_wk = copy(wqh.at[:, pl.ds(640, 640)], wqkv32.at[:, pl.ds(640, 640)], 1)
    c_wv = copy(wqh.at[:, pl.ds(1280, 640)], wqkv32.at[:, pl.ds(1280, 640)], 2)
    c_x1 = copy(xbh.at[pl.ds(128, 192)], xb32.at[pl.ds(128, 192)], 3)
    c_wq = copy(wqh.at[:, pl.ds(0, 640)], wqkv32.at[:, pl.ds(0, 640)], 4)
    c_ff = copy(ff_hbm, ff32, 5)
    c_xa = [copy(xah.at[:, pl.ds(128 * t, 128)], xa32.at[t], 6 + t) for t in range(5)]
    c_rr = copy(rr_hbm, rr32, 11)
    c_w = []
    for n, (src, dst, dst1) in enumerate(((wr_hbm, wr32, wr_last), (wi_hbm, wi32, wi_last))):
        w320 = src.at[pl.ds(0, 320)].bitcast(i32)
        for t in range(NB):
            c_w.append(pltpu.make_async_copy(w320.at[:, pl.ds(128 * t, 128)], dst.at[t], wsem.at[0]))
        c_w.append(copy(src.at[pl.ds(320, 1)], dst1, 13 + n))
    c_x2 = copy(xbh.at[pl.ds(320, 704)], xb32.at[pl.ds(320, 704)], 21)
    c_wo = copy(wo_hbm.bitcast(i32), wo32, 22)
    c_gg = copy(gg_hbm, gg32, 23)
    c_pin = copy(xbh.at[pl.ds(0, 8), pl.ds(0, 128)], pin_ref, 24)
    for cp in ([c_x0, c_wk, c_wv, c_x1, c_wq, c_wo, c_ff] + c_xa + [c_rr]
               + c_w + [c_x2, c_gg, c_pin]):
        cp.start()

    scale = float(DH ** -0.5 * np.log2(np.e))
    def _qpos(l):
        return (l & 16) + 4 * (l & 3) + ((l & 15) >> 2)
    rr_ = lax.broadcasted_iota(i32, (32, 128), 0)
    ll_ = _qpos(lax.broadcasted_iota(i32, (32, 128), 1))
    pos_ = rr_ & 15
    key_ = (rr_ & 16) + jnp.where(pos_ < 8, 2 * pos_, 2 * (pos_ - 8) + 1)
    le32 = key_ <= ll_
    wr_ = lax.broadcasted_iota(i32, (16, 128), 0)
    wq_ = _qpos(lax.broadcasted_iota(i32, (16, 128), 1))
    le_pk = (jnp.where(2 * wr_ <= wq_, jnp.int32(0xFFFF), jnp.int32(0))
             | jnp.where(2 * wr_ + 1 <= wq_, jnp.int32(-65536), jnp.int32(0)))
    lane8 = lax.broadcasted_iota(i32, (8, 128), 1)
    lane16 = lax.broadcasted_iota(i32, (16, 128), 1)
    bit0 = (lane16 & 32) != 0
    bit1 = (lane16 & 64) != 0
    bit0_8 = (lane8 & 32) != 0
    sub4 = lax.broadcasted_iota(i32, (8, 128), 0) < 4
    sub0 = lax.broadcasted_iota(i32, (8, 128), 0) == 0
    ones8 = jnp.ones((8, 128), f32)
    lo64 = lax.broadcasted_iota(i32, (64, 128), 1) < 64

    def rows_of(i):
        return i * 128 if isinstance(i, int) else pl.multiple_of(i * 128, 128)

    def wrows_of(i):
        return i * 64 if isinstance(i, int) else pl.multiple_of(i * 64, 64)

    def prep_wvt():
        for tr in range(5):
            wvt32[64 * tr:64 * tr + 64, :] = pltpu.bitcast(
                _b16(wqkv32[:, 1280 + tr * 128:1280 + (tr + 1) * 128]).T, i32)

    def prep_x(i):
        w = xb32[pl.ds(wrows_of(i), 64), :]
        z1 = _zip16(_b16(w).astype(f32))
        xz_ref[0] = z1
        xz_ref[1] = _zip16(_b16(z1).astype(f32))

    def win_ready(tiles, rolled, done, emit):
        for g in range(8):
            if g in done:
                continue
            kind, t, _ = _gwin(g)
            if kind == "nat":
                if t in tiles:
                    emit(g, tiles[t])
                    done.add(g)
            elif t in tiles and (t + 1) in tiles:
                for tt in (t, t + 1):
                    if tt not in rolled:
                        rolled[tt] = pltpu.roll(tiles[tt], 64, 1)
                emit(g, jnp.where(lo64, rolled[t], rolled[t + 1]))
                done.add(g)

    def proj_pieces(i, do_q=True, do_kv=True, qdst=None):
        qdst = qw_ref if qdst is None else qdst
        pieces = {}
        if do_kv:
            v8 = {}
            vdone = set()

            def vpiece(r):
                def f():
                    xb = _b16(xb32[pl.ds(wrows_of(i), 64), :])
                    vt = _dot_nt(_b16(wvt32[64 * r:64 * r + 64, :]), xb)
                    for j in range(16):
                        v8[16 * r + j] = vt[8 * j:8 * j + 8]
                    for p in range(16):
                        if p in vdone or any((5 * p + j) not in v8 for j in range(5)):
                            continue
                        v = [v8[5 * p + j] for j in range(5)]
                        h0, h1 = 2 * p, 2 * p + 1
                        vt_refs[h0 // 4][h0 % 4, i] = jnp.concatenate([v[0], v[1], v[2], ones8], 0).astype(bf)
                        vt_refs[h1 // 4][h1 % 4, i] = jnp.concatenate([v[2], v[3], v[4], ones8], 0).astype(bf)
                        vdone.add(p)
                return f

            kt, kr, kd = {}, {}, set()

            def kpiece(t):
                def f():
                    kt[t] = _zip16(_dot(_b16(xz_ref[1]), _b16(wqkv32[:, 640 + 128 * t:640 + 128 * t + 128])))

                    def emit(g, val):
                        kw_refs[g][pl.ds(wrows_of(i), 64), :] = val
                    win_ready(kt, kr, kd, emit)
                return f

            for r in range(5):
                pieces["v%d" % r] = vpiece(r)
                pieces["k%d" % r] = kpiece(r)
        if do_q:
            qt, qr, qd = {}, {}, set()

            def qpiece(t):
                def f():
                    qt[t] = _zip16(_dot(_b16(xz_ref[0]), _b16(wqkv32[:, 128 * t:128 * t + 128])) * scale)

                    def emit(g, val):
                        qdst[g] = val
                    win_ready(qt, qr, qd, emit)
                return f

            for t in range(5):
                pieces["q%d" % t] = qpiece(t)
        return pieces

    def out_pieces(i, slot=1):
        def opiece(t):
            def f():
                res = _dot(_b16(ob32[slot]), _b16(wo32[:, 128 * t:128 * t + 128]))
                obo32[pl.ds(wrows_of(i), 64), 128 * t:128 * t + 128] = _zip16(res)
            return f
        return {"o%d" % t: opiece(t) for t in range(5)}

    NSL = CFG.get('slots', 2)

    def key_tiles(i):
        return list(range(3)) if (not isinstance(i, int) or i >= 2) else list(range(2 - i, 3))

    pv_outs = {}
    last_pv = [None]

    def pv_group(g, i, es=(0, 1, 2, 3)):
        tiles = key_tiles(i)
        sl = g % NSL
        for e in es:
            P = _b16(p_ref[sl, e, 64 * tiles[0]:192, :])
            if len(tiles) > 1:
                vw = jnp.concatenate([vt_refs[g][e, i - 2 + j] for j in tiles], 1)
            else:
                vw = vt_refs[g][e, i]
            o = _dot(vw, P)
            rl = pltpu.reciprocal(o[24:32])
            res = [o[0:8] * rl, o[8:16] * rl, o[16:24] * rl]
            if e == 2:
                res = [pltpu.roll(r, 64, 1) for r in res]
            elif e == 1:
                res = [jnp.where(bit0_8, pltpu.roll(r, 32, 1), pltpu.roll(r, 96, 1)) for r in res]
            elif e == 3:
                res = [jnp.where(bit0_8, pltpu.roll(r, 96, 1), pltpu.roll(r, 32, 1)) for r in res]
            pv_outs[(g, e)] = res
            last_pv[0] = rl
            if (g, e ^ 1) in pv_outs:
                p = e // 2
                a, b = pv_outs.pop((g, 2 * p)), pv_outs.pop((g, 2 * p + 1))
                ot_ref[80 * g + 40 * p:80 * g + 40 * p + 40, :] = jnp.concatenate(
                    [a[0], a[1], jnp.where(sub4, a[2], b[0]), b[1], b[2]], 0)

    def fin_tile(t, slot):
        ob32[slot, :, 128 * t:128 * t + 128] = _zip16(ot_ref[128 * t:128 * t + 128, :].T)

    def ob_slot(i):
        return (0 if i in (0, 2) else (2 if i == 1 else 1)) if isinstance(i, int) else 1

    def finish(i):
        def f():
            pv_group(7, i)
            fin_tile(4, ob_slot(i))
        return f

    last_m = {}

    def token(n):
        kind = CFG.get("tok", {"0": "m", "1": "m", "2": "m", "3": "m"}).get(str(n))
        if kind == "m":
            g, u = max(last_m)
            return jnp.broadcast_to(last_m[(g, u)], (8, 128))
        if kind == "p":
            return last_pv[0]
        return None

    def attn(i, plan, head=None, qsrc=None, lazy=False):
        qsrc = qw_ref if qsrc is None else qsrc
        static = isinstance(i, int)
        lov = (lambda u: max(0, 8 - u - 4 * i)) if static else (lambda u: 0)
        tiles = key_tiles(i)
        ms = last_m

        def phase_a(g, us):
            sl = g % NSL
            _, _, off = _gwin(g)
            hm = [jnp.where((lane16 >= off + 20 * e) & (lane16 < off + 20 * e + 20), jnp.int32(-1), jnp.int32(0))
                  for e in range(4)]
            for u in us:
                lo = lov(u)
                nrow = 32 * (9 - lo)
                k0 = 64 * i - 128 + 16 * u + 16 * lo
                if not static:
                    k0 = pl.multiple_of(k0, 16)
                kw = _b16(kw_refs[g][pl.ds(k0, nrow // 2), :])
                qu = qsrc[g, 16 * u:16 * u + 16, :]
                qm = _b16(jnp.concatenate([qu & hm[lam ^ u] for lam in range(4)], 0))
                s = _dot_nt(kw, qm)
                sd = s[nrow - 32:nrow]
                if lo == 0:
                    T = jnp.where(le32, sd, s[0:32])
                    F = s[32:256]
                else:
                    T = jnp.where(le32, sd, NEG)
                    F = s[0:nrow - 32]
                m = jnp.max(T, axis=0, keepdims=True)
                s_ref[sl, u, 0:32] = T
                if F.shape[0] > 0:
                    m = jnp.maximum(m, jnp.max(F, axis=0, keepdims=True))
                    s_ref[sl, u, 32:32 + F.shape[0]] = F
                ms[(g, u)] = m

        def sel(m, a, b):
            if a is None and b is None:
                return None
            if a is None:
                a = jnp.zeros((16, 128), i32)
            if b is None:
                b = jnp.zeros((16, 128), i32)
            return jnp.where(m, a, b)

        def phase_b1(g):
            sl = g % NSL
            lo_ = [lov(u) for u in range(4)]
            nf = [7 if lo_[u] == 0 else 8 - lo_[u] for u in range(4)]

            def pblock(u, row0):
                p = jnp.exp2(s_ref[sl, u, row0:row0 + 32] - ms[(g, u)])
                return jnp.concatenate([_packi(p[16 * j:16 * j + 8], p[16 * j + 8:16 * j + 16]) for j in range(2)], 0)

            tri = {}

            def block(u, rel):
                if rel < 0 or rel > 8:
                    return None
                if rel == 0 or rel == 8:
                    if u not in tri:
                        pt = pblock(u, 0)
                        if lo_[u] == 0:
                            p8 = pt & le_pk
                            tri[u] = {8: p8, 0: pt ^ p8}
                        else:
                            tri[u] = {8: pt, 0: None}
                    return tri[u][rel]
                first = 8 - nf[u]
                if rel < first:
                    return None
                return pblock(u, 32 + 32 * (rel - first))

            for beta in range(4 * tiles[0], 12):
                src = [block(u, beta - u) for u in range(4)]
                a0 = sel(bit0, src[1], src[0])
                a1 = sel(bit0, src[0], src[1])
                c0 = sel(bit0, src[3], src[2])
                c1 = sel(bit0, src[2], src[3])
                o4 = [sel(bit1, c0, a0), sel(bit1, c1, a1), sel(bit1, a0, c0), sel(bit1, a1, c1)]
                for e in range(4):
                    p_ref[sl, e, 16 * beta:16 * beta + 16, :] = (
                        o4[e] if o4[e] is not None else jnp.zeros((16, 128), i32))

        order = CFG.get("order", "A0 P0 A1 A2 P1 A3 P2 X X P3 B Y")

        def step(s):
            if s == -1 and head is not None:
                head()
            px = plan.get(s, [])
            todo = list(range(len(px)))
            for tok in order.split():
                if tok[0] == "A" and 0 <= s + 1 < 8:
                    phase_a(s + 1, [int(c) for c in tok[1:]])
                if tok[0] == "B" and 0 <= s < 8:
                    phase_b1(s)
                if tok[0] == "P" and 0 <= s - 1 < 8:
                    pv_group(s - 1, i, [int(c) for c in tok[1:]])
                if tok[0] == "X" and todo:
                    px[todo.pop(0)]()
                if tok[0] == "Y":
                    while todo:
                        px[todo.pop(0)]()
            while todo:
                px[todo.pop(0)]()
            if s == 7:
                for t in range(4):
                    fin_tile(t, ob_slot(i))

        steps = [(lambda s=s: step(s)) for s in range(-1, 8)]
        if lazy:
            return steps
        for f in steps:
            f()

    def a1_x(a):
        j, par = a // 2, a % 2
        x = [_unpacki(xa32[t, pl.ds(j, 128, stride=8), :], par) for t in range(5)]
        t1 = x[1] + x[4]
        t2 = x[2] + x[3]
        t3 = x[1] - x[4]
        t4 = x[2] - x[3]
        y0 = x[0] + t1 + t2
        y1r = x[0] + C1 * t1 + C2 * t2
        y2r = x[0] + C2 * t1 + C1 * t2
        y1i = S1 * t3 + S2 * t4
        y2i = S2 * t3 - S1 * t4
        o0 = _dot_nt(_b16(ff32[0:80]), y0.astype(bf))
        re, im = [o0[0:80]], [o0[80:160]]
        for jj, (p, q) in enumerate(((y1r, y1i), (y2r, y2i))):
            w0 = 80 + 192 * jj
            t1 = _dot_nt(_b16(ff32[w0:w0 + 64]), (p + q).astype(bf))
            t2 = _dot_nt(_b16(ff32[w0 + 64:w0 + 128]), q.astype(bf))
            t3 = _dot_nt(_b16(ff32[w0 + 128:w0 + 192]), p.astype(bf))
            re.append(t1 - t2)
            im += [t3[0:64] - t1[0:64], t1[64:128] - t3[64:128]]
        yr = jnp.concatenate(re, 0)
        yi = jnp.concatenate(im, 0)
        ys_ref[a % 2, 0] = (yr + yi).astype(bf)
        ys_ref[a % 2, 1] = yi.astype(bf)
        ys_ref[a % 2, 2] = yr.astype(bf)

    def a1_y(a):
        t1 = _dot(ys_ref[a % 2, 0], _b16(rr32[a, 0]))
        t2 = _dot(ys_ref[a % 2, 1], _b16(rr32[a, 1]))
        t3 = _dot(ys_ref[a % 2, 2], _b16(rr32[a, 2]))
        g_ = jnp.concatenate([t1 - t2, t1 - t3], 1)
        for g in range(R // 8):
            gs_refs[g % 4][a, 8 * (g // 4):8 * (g // 4) + 8, :] = g_[8 * g:8 * g + 8]

    def a2_group(n, gq, token=None):
        g = 4 * gq + n
        special = isinstance(gq, int) and g == 8
        if isinstance(gq, int):
            w8 = g if g < 8 else (g - 10) % 8
            c10 = [0, 1, 4, 2, 3][0 if g < 8 else (g - 10) // 8 + 1] + 5 * (w8 // 4)
            r0 = 8 * gq
        else:
            w8 = jnp.where(g < 8, g, (g - 10) & 7)
            blk = jnp.minimum(jnp.where(g < 10, 0, ((g - 10) >> 3) + 1), 4)
            c10 = jnp.where(blk == 2, 4, jnp.where(blk > 2, blk - 1, blk)) + 5 * (w8 >> 2)
            r0 = 8 * gq
            if n == 0:
                r0 = jnp.where(g == 8, 96, r0)
            r0 = pl.multiple_of(r0, 8)
        w0 = (c10 >> 1) + 40 * (w8 & 3)
        sh = 16 * (1 - (c10 & 1))

        def wload(ref, last, f1):
            if special:
                return jnp.broadcast_to(last[0:1, 128 * f1:128 * f1 + 128].astype(f32), (8, 128))
            return pltpu.bitcast((ref[f1, pl.ds(w0, 8, stride=5), :] << sh) & jnp.int32(-65536), f32)

        gref = gs_refs[n]
        if token is not None:
            gref[16, pl.ds(pl.multiple_of(8 * (gq & 15), 8), 8), 0:128] = token
        z = [(gref[a, pl.ds(r0, 8), 0:128], gref[a, pl.ds(r0, 8), 128:256]) for a in range(16)]
        X = _fft16(z, False)
        V = []
        for f1 in range(16):
            wr = wload(wr32, wr_last, f1)
            wi = wload(wi32, wi_last, f1)
            V.append((X[f1][0] * wr - X[f1][1] * wi, X[f1][0] * wi + X[f1][1] * wr))
        U = _fft16(V, True)
        for a in range(16):
            gref[a, pl.ds(r0, 8), 0:128] = U[a][0]
            gref[a, pl.ds(r0, 8), 128:256] = U[a][1]

    def a3_z(a):
        u = jnp.concatenate([gs_refs[g % 4][a, 8 * (g // 4):8 * (g // 4) + 8, :] for g in range(R // 8)], 0)
        ur = u[:, 0:128]
        ui = u[:, 128:256]
        t1 = _dot_nt((ur + ui).astype(bf), _b16(rr32[a, 0]))
        t2 = _dot_nt(ui.astype(bf), _b16(rr32[a, 2]))
        t3 = _dot_nt(ur.astype(bf), _b16(rr32[a, 1]))
        zr = t1 - t2
        zi = t1 - t3
        kop = [zr[0:64], jnp.where(sub0, zr[64:72], zi[0:8]), zi[8:64]]
        for r0 in (80, 208):
            kop += [zr[r0:r0 + 64] + zi[r0:r0 + 64], zr[r0 + 64:r0 + 128] - zi[r0 + 64:r0 + 128],
                    zi[r0:r0 + 128], zr[r0:r0 + 128]]
        zs_ref[a % 2] = jnp.concatenate(kop, 0).astype(bf)

    def a3_d(a):
        sl = a % 2
        v0 = _dot(_b16(gg32[0:64]), zs_ref[sl, 0:128, :])
        vv = []
        for jj in range(2):
            w0, z0 = 64 + 192 * jj, 128 + 384 * jj
            t1 = _dot(_b16(gg32[w0:w0 + 64]), zs_ref[sl, z0:z0 + 128, :])
            t2 = _dot(_b16(gg32[w0 + 64:w0 + 128]), zs_ref[sl, z0 + 128:z0 + 256, :])
            t3 = _dot(_b16(gg32[w0 + 128:w0 + 192]), zs_ref[sl, z0 + 256:z0 + 384, :])
            vv += [t1 - t2, t1 + t3]
        v1r, v1i, v2r, v2i = vv
        A1 = v0 + C1 * v1r + C2 * v2r
        A2 = v0 + C2 * v1r + C1 * v2r
        B1 = S1 * v1i + S2 * v2i
        B2 = S2 * v1i - S1 * v2i
        y = [v0 + v1r + v2r, A1 - B1, A2 - B2, A2 + B2, A1 + B1]
        if a % 2 == 0:
            for t in range(5):
                ysc_ref[t] = y[t]
        else:
            j = a // 2
            for t in range(5):
                pk = _packi(ysc_ref[t], y[t])
                oa32[t, pl.ds(j, 128, stride=8), :] = pk.T

    def run(pieces, order=None):
        for k in (order or list(pieces)):
            if k in pieces:
                pieces[k]()

    PLAN = {-1: ["v0", "v1"], 0: ["k0", "q0"], 1: ["k1", "q1", "a0"], 2: ["k2", "q2"], 3: ["o0", "o1", "a1"],
            4: ["k3", "q3"], 5: ["o2", "o3", "a2"], 6: ["o4", "v2", "a3"], 7: ["k4", "q4", "v3", "v4"]}

    if 'plan' in CFG:
        PLAN = {int(k): v for k, v in CFG['plan'].items()}

    def mkplan(pieces):
        return {s_: [pieces[k] for k in ks if k in pieces] for s_, ks in PLAN.items()}

    ORD = ["v0", "v1", "v2", "v3", "v4", "k0", "k1", "k2", "k3", "k4", "q0", "q1", "q2", "q3", "q4"]

    def out_b_copy(i):
        return pltpu.make_async_copy(obo32.at[pl.ds(wrows_of(i), 64)],
                                     oh32.at[pl.ds(wrows_of(i), 64), pl.ds(D, D)], osem.at[0])

    for g in range(R // 8, 44):
        gs_refs[g % 4][0:16, 8 * (g // 4):8 * (g // 4) + 8, :] = jnp.zeros((16, 8, 256), f32)
    gs_refs[0][0:16, 96:104, :] = jnp.zeros((16, 8, 256), f32)
    c_x0.wait()
    c_wk.wait()
    prep_x(0)
    P0 = proj_pieces(0, do_q=False)
    run(P0, ["k0", "k1", "k2", "k3", "k4"])
    prep_x(1)
    P1 = proj_pieces(1, do_q=False)
    run(P1, ["k0", "k1", "k2", "k3", "k4"])
    c_wv.wait()
    prep_wvt()
    run(P0, ["v0", "v1", "v2", "v3", "v4"])
    run(P1, ["v0", "v1", "v2", "v3", "v4"])
    c_x1.wait()
    c_wq.wait()
    prep_x(2)
    run(proj_pieces(2), ORD)
    prep_x(3)
    attn(2, mkplan(proj_pieces(3)))
    prep_x(4)
    attn(3, mkplan(proj_pieces(4)), head=finish(2))
    for i_ in range(2):
        prep_x(i_)
        run(proj_pieces(i_, do_kv=False, qdst=qw01_ref.at[i_]), ORD)

    for cp in [c_wo, c_ff] + c_xa + [c_rr]:
        cp.wait()
    P2 = out_pieces(2, slot=0)
    run(P2, ["o0", "o1", "o2"])
    a1_x(0)
    run(P2, ["o3", "o4"])
    for a in range(16):
        if a + 1 < 16:
            a1_x(a + 1)
        a1_y(a)
    for cp in c_w:
        cp.wait()
    c_x2.wait()
    c_gg.wait()

    def one_block(i):
        nxt = jnp.minimum(i + 1, NB - 1)
        prep_x(nxt)
        P = proj_pieces(nxt)
        P.update(out_pieces(i - 1))
        for n in range(4):
            P["a%d" % n] = (lambda n=n: a2_group(n, i - 4, token(n)))
        last_m.clear()
        attn(i, mkplan(P), head=finish(i - 1))

    UNR = CFG.get("unroll", 1)

    def body(it, carry):
        for u_ in range(UNR):
            i = 4 + UNR * it + u_
            one_block(i)
            out_b_copy(i - 1).start()
        return carry

    out_b_copy(2).start()
    lax.fori_loop(0, NB - 5, body, 0)

    finish(NB - 2)()
    a2_group(0, 2)

    extra = attn(0, {}, qsrc=qw01_ref.at[0], lazy=True) + attn(1, {}, head=finish(0), qsrc=qw01_ref.at[1], lazy=True)
    extra += [lambda: pv_group(7, 1)] + list(out_pieces(0, slot=0).values())
    extra += [lambda: fin_tile(4, 2)] + list(out_pieces(1, slot=2).values())
    a3_z(0)
    done = 0
    for a in range(16):
        if a + 1 < 16:
            a3_z(a + 1)
        a3_d(a)
        upto = (len(extra) * (a + 1)) // 16
        for f in extra[done:upto]:
            f()
        done = upto
    out_b_copy(0).start()
    out_b_copy(1).start()
    c_oa = [pltpu.make_async_copy(oa32.at[t], oh32.at[:, pl.ds(128 * t, 128)], osem.at[1 + t]) for t in range(5)]
    for cp in c_oa:
        cp.start()
    c_pin.wait()

    P = out_pieces(NB - 2)
    last_m.clear()
    attn(NB - 1, {s_: [P[k] for k in ks] for s_, ks in
                  {-1: ["o0"], 0: ["o1"], 2: ["o2"], 4: ["o3"], 7: ["o4"]}.items()})
    out_b_copy(NB - 2).start()
    finish(NB - 1)()
    run(out_pieces(NB - 1))
    out_b_copy(NB - 1).start()

    for cp in c_oa:
        cp.wait()
    for i in range(NB):
        out_b_copy(i).wait()


def _build(FF32, GG32, RR32):
    scratch = [
        pltpu.VMEM((5, S // 2, 128), i32),
        pltpu.VMEM((NB, 160, 128), i32), pltpu.VMEM((NB, 160, 128), i32),
        pltpu.VMEM((1, S), bf), pltpu.VMEM((1, S), bf),
        pltpu.VMEM(FF32.shape, i32), pltpu.VMEM(GG32.shape, i32), pltpu.VMEM(RR32.shape, i32),
        pltpu.VMEM((2, 3, R, 128), bf),
        pltpu.VMEM((2, 896, 128), bf),
        pltpu.VMEM((5, 128, 128), f32),
        pltpu.VMEM((5, S // 2, 128), i32),
        pltpu.VMEM((8, 128), i32),
        pltpu.VMEM((2, 8, 64, 128), i32),
        pltpu.VMEM((S // 2, D), i32),
        pltpu.VMEM((D // 2, 3 * D), i32),
        pltpu.VMEM((D // 2, D), i32),
        pltpu.VMEM((D // 2, D), i32),
        pltpu.VMEM((CFG.get('slots', 2), 4, 256, 128), f32),
        pltpu.VMEM((CFG.get('slots', 2), 4, 192, 128), i32),
        pltpu.VMEM((3, 64, D), i32),
        pltpu.VMEM((D, 128), f32),
        pltpu.VMEM((8, 64, 128), i32),
        pltpu.VMEM((2, 64, D), i32),
        pltpu.VMEM((S // 2, D), i32),
        pltpu.SemaphoreType.DMA((25,)),
        pltpu.SemaphoreType.DMA((6,)),
        pltpu.SemaphoreType.DMA((1,)),
    ]
    scratch += [pltpu.VMEM((17, 104, 256), f32)] * 4
    scratch += [pltpu.VMEM((S // 2, 128), i32)] * 8
    scratch += [pltpu.VMEM((4, NB, 32, 128), bf)] * 8
    return pl.pallas_call(
        _kernel,
        out_shape=jax.ShapeDtypeStruct((S, 2 * D), bf),
        in_specs=[pl.BlockSpec(memory_space=pl.ANY)] * 9,
        out_specs=pl.BlockSpec(memory_space=pl.ANY),
        scratch_shapes=scratch,
        compiler_params=pltpu.CompilerParams(vmem_limit_bytes=110 * 2 ** 20),
    )


@jax.jit
def pallas_concat_heads__spectral_gfnet__sliding_block__prompt_kernel(
    A_x: jax.Array,
    A_w_r: jax.Array,
    A_w_i: jax.Array,
    B_x: jax.Array,
    B_wqkv: jax.Array,
    B_wo: jax.Array,
):
    FF32, GG32, RR32 = _make_consts()
    out = _build(FF32, GG32, RR32)(
        A_x.reshape(S, D), A_w_r.T, A_w_i.T, B_x.reshape(S, D), B_wqkv, B_wo,
        jnp.asarray(FF32), jnp.asarray(GG32), jnp.asarray(RR32))
    return out.reshape(1, S, 2 * D)
```

```python
import numpy as np
import ml_dtypes
import jax
import jax.numpy as jnp
from jax import lax
import jax.experimental.pallas as pl
import jax.experimental.pallas.tpu as pltpu

S = 2048
D = 640
DF = 321
H = 32
DH = 20
NB = S // 128
R = 336
NEG = -1e30
CFG = {}
f32 = jnp.float32
bf = jnp.bfloat16
i32 = jnp.int32

C1 = float(np.cos(2 * np.pi / 5))
C2 = float(np.cos(4 * np.pi / 5))
S1 = float(np.sin(2 * np.pi / 5))
S2 = float(np.sin(4 * np.pi / 5))


def _pack_rows(a):
    u = np.ascontiguousarray(a.astype(ml_dtypes.bfloat16)).view(np.uint16).astype(np.uint32)
    return (u[..., 0::2, :] | (u[..., 1::2, :] << 16)).astype(np.uint32).view(np.int32)


def _make_consts():
    b5 = np.arange(128)

    def cs(k):
        th = 2 * np.pi * np.outer(k, b5) / D
        return np.cos(th), np.sin(th)

    m32 = np.arange(32)
    k0 = np.concatenate([10 * m32, 5 + 10 * m32, [320]])
    c, s = cs(k0)
    F0 = np.zeros((160, 128))
    F0[0:65] = c
    F0[80:145] = -s

    def kpair(j):
        return (np.concatenate([j + 10 * m32, j + 5 + 10 * m32]),
                np.concatenate([5 - j + 10 * m32, 10 - j + 10 * m32]))

    def fwd(j):
        ka, kb = kpair(j)
        (ca, sa), (cb, sb) = cs(ka), cs(kb)
        return np.concatenate([ca, cb, ca + sa, cb - sb, ca - sa, cb + sb], 0)

    FF = np.concatenate([F0, fwd(1), fwd(2)], 0)

    b = np.arange(128)
    f2 = np.arange(128)
    RR = np.zeros((16, 3, 128, 128))
    for a in range(16):
        th = -2 * np.pi * (np.outer(b, f2) / 128.0 + a * f2[None, :] / float(S))
        Mr, Mi = np.cos(th), np.sin(th)
        RR[a, 0] = Mr
        RR[a, 1] = Mr + Mi
        RR[a, 2] = Mr - Mi

    sc = 1.0 / (S * D)
    G0 = np.zeros((128, 128))
    al = np.full(65, 2.0)
    al[0] = 1.0
    al[64] = 1.0
    G0[:, 0:64] = (al[0:64, None] * c[0:64]).T
    G0[:, 64:128] = (-al[0:64, None] * s[0:64]).T
    G0[:, 64] = al[64] * c[64]

    def inv(j):
        ka, kb = kpair(j)
        (ca, sa), (cb, sb) = cs(ka), cs(kb)
        return 2 * np.concatenate([np.concatenate([ca, cb], 0).T,
                                   np.concatenate([ca + sa, sb - cb], 0).T,
                                   np.concatenate([sa - ca, -sb - cb], 0).T], 0)

    GG = np.concatenate([G0, inv(1), inv(2)], 0) * sc
    GG = GG.reshape(7, 128, 128).transpose(0, 2, 1).reshape(896, 128)
    return _pack_rows(FF), _pack_rows(GG), _pack_rows(RR)


_NT = (((1,), (1,)), ((), ()))


def _dot(a, b):
    return jnp.dot(a, b, preferred_element_type=f32)


def _dot_nt(a, b):
    return lax.dot_general(a, b, _NT, preferred_element_type=f32)


def _b16(x):
    return pltpu.bitcast(x, bf)


def _packi(a, b):
    return pltpu.pack_elementwise([a, b], packed_dtype=bf)


def _unpacki(x, idx):
    return pltpu.unpack_elementwise(x, index=idx, packed_dtype=bf, unpacked_dtype=f32)


def _zip16(x):
    n = x.shape[0] // 16
    return jnp.concatenate([_packi(x[16 * j:16 * j + 8], x[16 * j + 8:16 * j + 16]) for j in range(n)], 0)


def _dft4(z, inv):
    (a, b, c, d) = z
    t0 = (a[0] + c[0], a[1] + c[1])
    t1 = (a[0] - c[0], a[1] - c[1])
    t2 = (b[0] + d[0], b[1] + d[1])
    t3 = (b[0] - d[0], b[1] - d[1])
    o0 = (t0[0] + t2[0], t0[1] + t2[1])
    o2 = (t0[0] - t2[0], t0[1] - t2[1])
    p = (t1[0] + t3[1], t1[1] - t3[0])
    q = (t1[0] - t3[1], t1[1] + t3[0])
    return [o0, q, o2, p] if inv else [o0, p, o2, q]


def _tw16(z, e, inv):
    if e == 0:
        return z
    zr, zi = z
    if e == 4:
        return (-zi, zr) if inv else (zi, -zr)
    h = float(np.sqrt(0.5))
    if e == 2:
        return ((zr - zi) * h, (zr + zi) * h) if inv else ((zr + zi) * h, (zi - zr) * h)
    if e == 6:
        return ((-zr - zi) * h, (zr - zi) * h) if inv else ((zi - zr) * h, (-zr - zi) * h)
    sgn = 1.0 if inv else -1.0
    c = float(np.cos(2 * np.pi * e / 16))
    s = float(sgn * np.sin(2 * np.pi * e / 16))
    return (zr * c - zi * s, zr * s + zi * c)


def _fft16(z, inv):
    hh = [_dft4([z[a0 + 4 * a1] for a1 in range(4)], inv) for a0 in range(4)]
    out = [None] * 16
    for fa in range(4):
        o = _dft4([_tw16(hh[a0][fa], a0 * fa, inv) for a0 in range(4)], inv)
        for fb in range(4):
            out[fa + 4 * fb] = o[fb]
    return out


def _gwin(g):
    lo, hi = 80 * g, 80 * g + 79
    if lo // 128 == hi // 128:
        return ("nat", lo // 128, lo - 128 * (lo // 128))
    t = (lo - 64) // 128
    return ("shf", t, lo - 64 - 128 * t)


def _kernel(xa_hbm, wr_hbm, wi_hbm, xb_hbm, wqkv_hbm, wo_hbm, ff_hbm, gg_hbm, rr_hbm, out_hbm,
            xa32, wr32, wi32, wr_last, wi_last, ff32, gg32, rr32, ys_ref, zs_ref, ysc_ref, oa32,
            pin_ref, qw01_ref, xb32, wqkv32, wo32, wvt32, s_ref, p_ref, ob32, ot_ref, qw_ref, xz_ref, obo32,
            sem, osem, wsem, *groups):
    gs_refs = groups[0:4]
    kw_refs = groups[4:12]
    vt_refs = groups[12:20]

    def copy(src, dst, k):
        return pltpu.make_async_copy(src, dst, sem.at[k])

    xbh = xb_hbm.bitcast(i32)
    wqh = wqkv_hbm.bitcast(i32)
    xah = xa_hbm.bitcast(i32)
    oh32 = out_hbm.bitcast(i32)
    c_x0 = copy(xbh.at[pl.ds(0, 128)], xb32.at[pl.ds(0, 128)], 0)
    c_wk = copy(wqh.at[:, pl.ds(640, 640)], wqkv32.at[:, pl.ds(640, 640)], 1)
    c_wv = copy(wqh.at[:, pl.ds(1280, 640)], wqkv32.at[:, pl.ds(1280, 640)], 2)
    c_x1 = copy(xbh.at[pl.ds(128, 192)], xb32.at[pl.ds(128, 192)], 3)
    c_wq = copy(wqh.at[:, pl.ds(0, 640)], wqkv32.at[:, pl.ds(0, 640)], 4)
    c_ff = copy(ff_hbm, ff32, 5)
    c_xa = [copy(xah.at[:, pl.ds(128 * t, 128)], xa32.at[t], 6 + t) for t in range(5)]
    c_rr = copy(rr_hbm, rr32, 11)
    c_w = []
    for n, (src, dst, dst1) in enumerate(((wr_hbm, wr32, wr_last), (wi_hbm, wi32, wi_last))):
        w320 = src.at[pl.ds(0, 320)].bitcast(i32)
        for t in range(NB):
            c_w.append(pltpu.make_async_copy(w320.at[:, pl.ds(128 * t, 128)], dst.at[t], wsem.at[0]))
        c_w.append(copy(src.at[pl.ds(320, 1)], dst1, 13 + n))
    c_x2 = copy(xbh.at[pl.ds(320, 704)], xb32.at[pl.ds(320, 704)], 21)
    c_wo = copy(wo_hbm.bitcast(i32), wo32, 22)
    c_gg = copy(gg_hbm, gg32, 23)
    c_pin = copy(xbh.at[pl.ds(0, 8), pl.ds(0, 128)], pin_ref.at[0], 24)
    c_pin2 = copy(xbh.at[pl.ds(0, 8), pl.ds(0, 128)], pin_ref.at[1], 12)
    for cp in ([c_x0, c_wk, c_wv, c_x1, c_wq, c_wo, c_ff] + c_xa + [c_rr]
               + c_w + [c_x2, c_gg, c_pin, c_pin2]):
        cp.start()

    scale = float(DH ** -0.5 * np.log2(np.e))
    def _qpos(l):
        return (l & 16) + 4 * (l & 3) + ((l & 15) >> 2)
    rr_ = lax.broadcasted_iota(i32, (32, 128), 0)
    ll_ = _qpos(lax.broadcasted_iota(i32, (32, 128), 1))
    pos_ = rr_ & 15
    key_ = (rr_ & 16) + jnp.where(pos_ < 8, 2 * pos_, 2 * (pos_ - 8) + 1)
    le32 = key_ <= ll_
    wr_ = lax.broadcasted_iota(i32, (16, 128), 0)
    wq_ = _qpos(lax.broadcasted_iota(i32, (16, 128), 1))
    le_pk = (jnp.where(2 * wr_ <= wq_, jnp.int32(0xFFFF), jnp.int32(0))
             | jnp.where(2 * wr_ + 1 <= wq_, jnp.int32(-65536), jnp.int32(0)))
    lane8 = lax.broadcasted_iota(i32, (8, 128), 1)
    lane16 = lax.broadcasted_iota(i32, (16, 128), 1)
    bit0 = (lane16 & 32) != 0
    bit1 = (lane16 & 64) != 0
    bit0_8 = (lane8 & 32) != 0
    sub4 = lax.broadcasted_iota(i32, (8, 128), 0) < 4
    sub0 = lax.broadcasted_iota(i32, (8, 128), 0) == 0
    ones8 = jnp.ones((8, 128), f32)
    lo64 = lax.broadcasted_iota(i32, (64, 128), 1) < 64

    def rows_of(i):
        return i * 128 if isinstance(i, int) else pl.multiple_of(i * 128, 128)

    def wrows_of(i):
        return i * 64 if isinstance(i, int) else pl.multiple_of(i * 64, 64)

    def prep_wvt():
        for tr in range(5):
            wvt32[64 * tr:64 * tr + 64, :] = pltpu.bitcast(
                _b16(wqkv32[:, 1280 + tr * 128:1280 + (tr + 1) * 128]).T, i32)

    def prep_x(i):
        w = xb32[pl.ds(wrows_of(i), 64), :]
        z1 = _zip16(_b16(w).astype(f32))
        xz_ref[0] = z1
        xz_ref[1] = _zip16(_b16(z1).astype(f32))

    def win_ready(tiles, rolled, done, emit):
        for g in range(8):
            if g in done:
                continue
            kind, t, _ = _gwin(g)
            if kind == "nat":
                if t in tiles:
                    emit(g, tiles[t])
                    done.add(g)
            elif t in tiles and (t + 1) in tiles:
                for tt in (t, t + 1):
                    if tt not in rolled:
                        rolled[tt] = pltpu.roll(tiles[tt], 64, 1)
                emit(g, jnp.where(lo64, rolled[t], rolled[t + 1]))
                done.add(g)

    def proj_pieces(i, do_q=True, do_kv=True, qdst=None):
        qdst = qw_ref if qdst is None else qdst
        pieces = {}
        if do_kv:
            v8 = {}
            vdone = set()

            def vpiece(r):
                def f():
                    xb = _b16(xb32[pl.ds(wrows_of(i), 64), :])
                    vt = _dot_nt(_b16(wvt32[64 * r:64 * r + 64, :]), xb)
                    for j in range(16):
                        v8[16 * r + j] = vt[8 * j:8 * j + 8]
                    for p in range(16):
                        if p in vdone or any((5 * p + j) not in v8 for j in range(5)):
                            continue
                        v = [v8[5 * p + j] for j in range(5)]
                        h0, h1 = 2 * p, 2 * p + 1
                        vt_refs[h0 // 4][h0 % 4, i] = jnp.concatenate([v[0], v[1], v[2], ones8], 0).astype(bf)
                        vt_refs[h1 // 4][h1 % 4, i] = jnp.concatenate([v[2], v[3], v[4], ones8], 0).astype(bf)
                        vdone.add(p)
                return f

            kt, kr, kd = {}, {}, set()

            def kpiece(t):
                def f():
                    kt[t] = _zip16(_dot(_b16(xz_ref[1]), _b16(wqkv32[:, 640 + 128 * t:640 + 128 * t + 128])))

                    def emit(g, val):
                        kw_refs[g][pl.ds(wrows_of(i), 64), :] = val
                    win_ready(kt, kr, kd, emit)
                return f

            for r in range(5):
                pieces["v%d" % r] = vpiece(r)
                pieces["k%d" % r] = kpiece(r)
        if do_q:
            qt, qr, qd = {}, {}, set()

            def qpiece(t):
                def f():
                    qt[t] = _zip16(_dot(_b16(xz_ref[0]), _b16(wqkv32[:, 128 * t:128 * t + 128])) * scale)

                    def emit(g, val):
                        qdst[g] = val
                    win_ready(qt, qr, qd, emit)
                return f

            for t in range(5):
                pieces["q%d" % t] = qpiece(t)
        return pieces

    def out_pieces(i, slot=1):
        def opiece(t):
            def f():
                res = _dot(_b16(ob32[slot]), _b16(wo32[:, 128 * t:128 * t + 128]))
                obo32[pl.ds(wrows_of(i), 64), 128 * t:128 * t + 128] = _zip16(res)
            return f
        return {"o%d" % t: opiece(t) for t in range(5)}

    NSL = CFG.get('slots', 2)

    def key_tiles(i):
        return list(range(3)) if (not isinstance(i, int) or i >= 2) else list(range(2 - i, 3))

    pv_outs = {}
    last_pv = [None]

    def pv_group(g, i, es=(0, 1, 2, 3)):
        tiles = key_tiles(i)
        sl = g % NSL
        for e in es:
            P = _b16(p_ref[sl, e, 64 * tiles[0]:192, :])
            if len(tiles) > 1:
                vw = jnp.concatenate([vt_refs[g][e, i - 2 + j] for j in tiles], 1)
            else:
                vw = vt_refs[g][e, i]
            o = _dot(vw, P)
            rl = pltpu.reciprocal(o[24:32])
            res = [o[0:8] * rl, o[8:16] * rl, o[16:24] * rl]
            if e == 2:
                res = [pltpu.roll(r, 64, 1) for r in res]
            elif e == 1:
                res = [jnp.where(bit0_8, pltpu.roll(r, 32, 1), pltpu.roll(r, 96, 1)) for r in res]
            elif e == 3:
                res = [jnp.where(bit0_8, pltpu.roll(r, 96, 1), pltpu.roll(r, 32, 1)) for r in res]
            pv_outs[(g, e)] = res
            last_pv[0] = rl
            if (g, e ^ 1) in pv_outs:
                p = e // 2
                a, b = pv_outs.pop((g, 2 * p)), pv_outs.pop((g, 2 * p + 1))
                ot_ref[80 * g + 40 * p:80 * g + 40 * p + 40, :] = jnp.concatenate(
                    [a[0], a[1], jnp.where(sub4, a[2], b[0]), b[1], b[2]], 0)

    def fin_tile(t, slot):
        ob32[slot, :, 128 * t:128 * t + 128] = _zip16(ot_ref[128 * t:128 * t + 128, :].T)

    def ob_slot(i):
        return (0 if i in (0, 2) else (2 if i == 1 else 1)) if isinstance(i, int) else 1

    def finish(i):
        def f():
            pv_group(7, i)
            fin_tile(4, ob_slot(i))
        return f

    last_m = {}

    def token(n):
        kind = CFG.get("tok", {"0": "m", "1": "m", "2": "m", "3": "m"}).get(str(n))
        if kind == "m":
            g, u = max(last_m)
            return jnp.broadcast_to(last_m[(g, u)], (8, 128))
        if kind == "p":
            return last_pv[0]
        return None

    def attn(i, plan, head=None, qsrc=None, lazy=False):
        qsrc = qw_ref if qsrc is None else qsrc
        static = isinstance(i, int)
        lov = (lambda u: max(0, 8 - u - 4 * i)) if static else (lambda u: 0)
        tiles = key_tiles(i)
        ms = last_m

        def phase_a(g, us):
            sl = g % NSL
            _, _, off = _gwin(g)
            hm = [jnp.where((lane16 >= off + 20 * e) & (lane16 < off + 20 * e + 20), jnp.int32(-1), jnp.int32(0))
                  for e in range(4)]
            for u in us:
                lo = lov(u)
                nrow = 32 * (9 - lo)
                k0 = 64 * i - 128 + 16 * u + 16 * lo
                if not static:
                    k0 = pl.multiple_of(k0, 16)
                kw = _b16(kw_refs[g][pl.ds(k0, nrow // 2), :])
                qu = qsrc[g, 16 * u:16 * u + 16, :]
                qm = _b16(jnp.concatenate([qu & hm[lam ^ u] for lam in range(4)], 0))
                s = _dot_nt(kw, qm)
                sd = s[nrow - 32:nrow]
                if lo == 0:
                    T = jnp.where(le32, sd, s[0:32])
                    F = s[32:256]
                else:
                    T = jnp.where(le32, sd, NEG)
                    F = s[0:nrow - 32]
                m = jnp.max(T, axis=0, keepdims=True)
                s_ref[sl, u, 0:32] = T
                if F.shape[0] > 0:
                    m = jnp.maximum(m, jnp.max(F, axis=0, keepdims=True))
                    s_ref[sl, u, 32:32 + F.shape[0]] = F
                ms[(g, u)] = m

        def sel(m, a, b):
            if a is None and b is None:
                return None
            if a is None:
                a = jnp.zeros((16, 128), i32)
            if b is None:
                b = jnp.zeros((16, 128), i32)
            return jnp.where(m, a, b)

        def phase_b1(g):
            sl = g % NSL
            lo_ = [lov(u) for u in range(4)]
            nf = [7 if lo_[u] == 0 else 8 - lo_[u] for u in range(4)]

            def pblock(u, row0):
                p = jnp.exp2(s_ref[sl, u, row0:row0 + 32] - ms[(g, u)])
                return jnp.concatenate([_packi(p[16 * j:16 * j + 8], p[16 * j + 8:16 * j + 16]) for j in range(2)], 0)

            tri = {}

            def block(u, rel):
                if rel < 0 or rel > 8:
                    return None
                if rel == 0 or rel == 8:
                    if u not in tri:
                        pt = pblock(u, 0)
                        if lo_[u] == 0:
                            p8 = pt & le_pk
                            tri[u] = {8: p8, 0: pt ^ p8}
                        else:
                            tri[u] = {8: pt, 0: None}
                    return tri[u][rel]
                first = 8 - nf[u]
                if rel < first:
                    return None
                return pblock(u, 32 + 32 * (rel - first))

            for beta in range(4 * tiles[0], 12):
                src = [block(u, beta - u) for u in range(4)]
                a0 = sel(bit0, src[1], src[0])
                a1 = sel(bit0, src[0], src[1])
                c0 = sel(bit0, src[3], src[2])
                c1 = sel(bit0, src[2], src[3])
                o4 = [sel(bit1, c0, a0), sel(bit1, c1, a1), sel(bit1, a0, c0), sel(bit1, a1, c1)]
                for e in range(4):
                    p_ref[sl, e, 16 * beta:16 * beta + 16, :] = (
                        o4[e] if o4[e] is not None else jnp.zeros((16, 128), i32))

        order = CFG.get("order", "A0 P0 A1 A2 P1 A3 P2 X X P3 B Y")

        def step(s):
            if s == -1 and head is not None:
                head()
            px = plan.get(s, [])
            todo = list(range(len(px)))
            for tok in order.split():
                if tok[0] == "A" and 0 <= s + 1 < 8:
                    phase_a(s + 1, [int(c) for c in tok[1:]])
                if tok[0] == "B" and 0 <= s < 8:
                    phase_b1(s)
                if tok[0] == "P" and 0 <= s - 1 < 8:
                    pv_group(s - 1, i, [int(c) for c in tok[1:]])
                if tok[0] == "X" and todo:
                    px[todo.pop(0)]()
                if tok[0] == "Y":
                    while todo:
                        px[todo.pop(0)]()
            while todo:
                px[todo.pop(0)]()
            if s == 7:
                for t in range(4):
                    fin_tile(t, ob_slot(i))

        steps = [(lambda s=s: step(s)) for s in range(-1, 8)]
        if lazy:
            return steps
        for f in steps:
            f()

    def a1_step(ax, ay, order):
        w = {}
        if ax is not None:
            j, par = ax // 2, ax % 2
            x = [_unpacki(xa32[t, pl.ds(j, 128, stride=8), :], par) for t in range(5)]
            t1 = x[1] + x[4]
            t2 = x[2] + x[3]
            t3 = x[1] - x[4]
            t4 = x[2] - x[3]
            p1 = x[0] + C1 * t1 + C2 * t2
            p2 = x[0] + C2 * t1 + C1 * t2
            q1 = S1 * t3 + S2 * t4
            q2 = S2 * t3 - S1 * t4
            ops = [x[0] + t1 + t2, p1 + q1, q1, p1, p2 + q2, q2, p2]
            w0s = [0, 80, 144, 208, 272, 336, 400, 464]
        for tok in order:
            if tok[0] == "x" and ax is not None:
                n = int(tok[1])
                w[tok] = _dot_nt(_b16(ff32[w0s[n]:w0s[n + 1]]), ops[n].astype(bf))
            if tok[0] == "y" and ay is not None:
                n = int(tok[1])
                w[tok] = _dot(ys_ref[ay % 2, n], _b16(rr32[ay, n]))
        if ay is not None:
            g_ = jnp.concatenate([w["y0"] - w["y1"], w["y0"] - w["y2"]], 1)
            for g in range(R // 8):
                gs_refs[g % 4][ay, 8 * (g // 4):8 * (g // 4) + 8, :] = g_[8 * g:8 * g + 8]
        if ax is not None:
            re, im = [w["x0"][0:80]], [w["x0"][80:160]]
            for n in (1, 4):
                t1, t2, t3 = w["x%d" % n], w["x%d" % (n + 1)], w["x%d" % (n + 2)]
                re.append(t1 - t2)
                im += [t3[0:64] - t1[0:64], t1[64:128] - t3[64:128]]
            yr = jnp.concatenate(re, 0)
            yi = jnp.concatenate(im, 0)
            ys_ref[ax % 2, 0] = (yr + yi).astype(bf)
            ys_ref[ax % 2, 1] = yi.astype(bf)
            ys_ref[ax % 2, 2] = yr.astype(bf)

    def a2_group(n, gq, token=None):
        g = 4 * gq + n
        special = isinstance(gq, int) and g == 8
        if isinstance(gq, int):
            w8 = g if g < 8 else (g - 10) % 8
            c10 = [0, 1, 4, 2, 3][0 if g < 8 else (g - 10) // 8 + 1] + 5 * (w8 // 4)
            r0 = 8 * gq
        else:
            w8 = jnp.where(g < 8, g, (g - 10) & 7)
            blk = jnp.minimum(jnp.where(g < 10, 0, ((g - 10) >> 3) + 1), 4)
            c10 = jnp.where(blk == 2, 4, jnp.where(blk > 2, blk - 1, blk)) + 5 * (w8 >> 2)
            r0 = 8 * gq
            if n == 0:
                r0 = jnp.where(g == 8, 96, r0)
            r0 = pl.multiple_of(r0, 8)
        w0 = (c10 >> 1) + 40 * (w8 & 3)
        sh = 16 * (1 - (c10 & 1))

        def wload(ref, last, f1):
            if special:
                return jnp.broadcast_to(last[0:1, 128 * f1:128 * f1 + 128].astype(f32), (8, 128))
            return pltpu.bitcast((ref[f1, pl.ds(w0, 8, stride=5), :] << sh) & jnp.int32(-65536), f32)

        gref = gs_refs[n]
        if token is not None:
            gref[16, pl.ds(pl.multiple_of(8 * (gq & 15), 8), 8), 0:128] = token
        z = [(gref[a, pl.ds(r0, 8), 0:128], gref[a, pl.ds(r0, 8), 128:256]) for a in range(16)]
        X = _fft16(z, False)
        V = []
        for f1 in range(16):
            wr = wload(wr32, wr_last, f1)
            wi = wload(wi32, wi_last, f1)
            V.append((X[f1][0] * wr - X[f1][1] * wi, X[f1][0] * wi + X[f1][1] * wr))
        U = _fft16(V, True)
        for a in range(16):
            gref[a, pl.ds(r0, 8), 0:128] = U[a][0]
            gref[a, pl.ds(r0, 8), 128:256] = U[a][1]

    def a3_step(az, ad, order, extra=()):
        w = {}
        if az is not None:
            u = jnp.concatenate([gs_refs[g % 4][az, 8 * (g // 4):8 * (g // 4) + 8, :] for g in range(R // 8)], 0)
            ur = u[:, 0:128]
            ui = u[:, 128:256]
            zops = [(ur + ui, 0), (ui, 2), (ur, 1)]
        for tok in order:
            if tok[0] == "z" and az is not None:
                v, n = zops[int(tok[1])]
                w[tok] = _dot_nt(v.astype(bf), _b16(rr32[az, n]))
            if tok[0] == "d" and ad is not None:
                n = int(tok[1])
                w[tok] = _dot(zs_ref[ad % 2, n], _b16(gg32[64 * n:64 * n + 64]))
            if tok == "E":
                for f in extra:
                    f()
        if ad is not None:
            v0 = w["d0"]
            v1r, v1i = w["d1"] - w["d2"], w["d1"] + w["d3"]
            v2r, v2i = w["d4"] - w["d5"], w["d4"] + w["d6"]
            A1 = v0 + C1 * v1r + C2 * v2r
            A2 = v0 + C2 * v1r + C1 * v2r
            B1 = S1 * v1i + S2 * v2i
            B2 = S2 * v1i - S1 * v2i
            y = [v0 + v1r + v2r, A1 - B1, A2 - B2, A2 + B2, A1 + B1]
            for t in range(5):
                if ad % 2 == 0:
                    ysc_ref[t] = y[t]
                else:
                    oa32[t, pl.ds(ad // 2, 128, stride=8), :] = _packi(ysc_ref[t], y[t])
        if az is not None:
            zr = w["z0"] - w["z1"]
            zi = w["z0"] - w["z2"]
            kop = [jnp.concatenate([zr[0:64], jnp.where(sub0, zr[64:72], zi[0:8]), zi[8:64]], 0)]
            for r0 in (80, 208):
                kop += [jnp.concatenate([zr[r0:r0 + 64] + zi[r0:r0 + 64], zr[r0 + 64:r0 + 128] - zi[r0 + 64:r0 + 128]], 0),
                        zi[r0:r0 + 128], zr[r0:r0 + 128]]
            for n in range(7):
                zs_ref[az % 2, n] = kop[n].T.astype(bf)

    def run(pieces, order=None):
        for k in (order or list(pieces)):
            if k in pieces:
                pieces[k]()

    PLAN = {-1: ["v0", "v1"], 0: ["k0", "q0"], 1: ["k1", "q1", "a0"], 2: ["k2", "q2"], 3: ["o0", "o1", "a1"],
            4: ["k3", "q3"], 5: ["o2", "o3", "a2"], 6: ["o4", "v2", "a3"], 7: ["k4", "q4", "v3", "v4"]}

    if 'plan' in CFG:
        PLAN = {int(k): v for k, v in CFG['plan'].items()}

    def mkplan(pieces):
        return {s_: [pieces[k] for k in ks if k in pieces] for s_, ks in PLAN.items()}

    ORD = ["v0", "v1", "v2", "v3", "v4", "k0", "k1", "k2", "k3", "k4", "q0", "q1", "q2", "q3", "q4"]

    def out_b_copy(i):
        return pltpu.make_async_copy(obo32.at[pl.ds(wrows_of(i), 64)],
                                     oh32.at[pl.ds(wrows_of(i), 64), pl.ds(D, D)], osem.at[0])

    for g in range(R // 8, 44):
        gs_refs[g % 4][0:16, 8 * (g // 4):8 * (g // 4) + 8, :] = jnp.zeros((16, 8, 256), f32)
    gs_refs[0][0:16, 96:104, :] = jnp.zeros((16, 8, 256), f32)
    c_x0.wait()
    c_wk.wait()
    prep_x(0)
    P0 = proj_pieces(0, do_q=False)
    run(P0, ["k0", "k1", "k2", "k3", "k4"])
    prep_x(1)
    P1 = proj_pieces(1, do_q=False)
    run(P1, ["k0", "k1", "k2", "k3", "k4"])
    c_wv.wait()
    prep_wvt()
    run(P0, ["v0", "v1", "v2", "v3", "v4"])
    run(P1, ["v0", "v1", "v2", "v3", "v4"])
    c_x1.wait()
    c_wq.wait()
    prep_x(2)
    run(proj_pieces(2), ORD)
    prep_x(3)
    attn(2, mkplan(proj_pieces(3)))
    prep_x(4)
    attn(3, mkplan(proj_pieces(4)), head=finish(2))
    for i_ in range(2):
        prep_x(i_)
        run(proj_pieces(i_, do_kv=False, qdst=qw01_ref.at[i_]), ORD)

    for cp in [c_wo, c_ff] + c_xa + [c_rr]:
        cp.wait()
    P2 = out_pieces(2, slot=0)
    run(P2, ["o0", "o1", "o2"])
    a1o = CFG.get("a1", "x0 x1 x2 x3 y0 x4 y1 x5 y2 x6").split()
    a1_step(0, None, a1o)
    run(P2, ["o3", "o4"])
    for a in range(16):
        a1_step(a + 1 if a < 15 else None, a, a1o)
    for cp in c_w:
        cp.wait()
    c_x2.wait()
    c_gg.wait()

    def one_block(i):
        nxt = jnp.minimum(i + 1, NB - 1)
        prep_x(nxt)
        P = proj_pieces(nxt)
        P.update(out_pieces(i - 1))
        for n in range(4):
            P["a%d" % n] = (lambda n=n: a2_group(n, i - 4, token(n)))
        last_m.clear()
        attn(i, mkplan(P), head=finish(i - 1))

    UNR = CFG.get("unroll", 1)

    def body(it, carry):
        for u_ in range(UNR):
            i = 4 + UNR * it + u_
            one_block(i)
            out_b_copy(i - 1).start()
        return carry

    out_b_copy(2).start()
    lax.fori_loop(0, NB - 5, body, 0)

    finish(NB - 2)()
    a2_group(0, 2)

    extra = attn(0, {}, qsrc=qw01_ref.at[0], lazy=True) + attn(1, {}, head=finish(0), qsrc=qw01_ref.at[1], lazy=True)
    extra += [lambda: pv_group(7, 1), lambda: fin_tile(4, 2)]
    a3o = CFG.get("a3", "z0 z1 z2 d0 d1 d2 d3 d4 d5 d6 E").split()
    a3_step(0, None, a3o)
    for a in range(16):
        a3_step(a + 1 if a < 15 else None, a, a3o, extra[(len(extra) * a) // 16:(len(extra) * (a + 1)) // 16])
    c_oa = [pltpu.make_async_copy(oa32.at[t], oh32.at[:, pl.ds(128 * t, 128)], osem.at[1 + t]) for t in range(5)]
    for cp in c_oa:
        cp.start()
    c_pin.wait()

    fill = []
    for t in range(5):
        fill += [out_pieces(0, slot=0)["o%d" % t], out_pieces(1, slot=2)["o%d" % t], out_pieces(NB - 2)["o%d" % t]]
    last_m.clear()
    attn(NB - 1, {s_: fill[(15 * (s_ + 1)) // 9:(15 * (s_ + 2)) // 9] for s_ in range(-1, 8)})
    for i_ in (0, 1, NB - 2):
        out_b_copy(i_).start()
    c_pin2.wait()
    finish(NB - 1)()
    run(out_pieces(NB - 1))
    out_b_copy(NB - 1).start()

    for cp in c_oa:
        cp.wait()
    for i in range(NB):
        out_b_copy(i).wait()


def _build(FF32, GG32, RR32):
    scratch = [
        pltpu.VMEM((5, S // 2, 128), i32),
        pltpu.VMEM((NB, 160, 128), i32), pltpu.VMEM((NB, 160, 128), i32),
        pltpu.VMEM((1, S), bf), pltpu.VMEM((1, S), bf),
        pltpu.VMEM(FF32.shape, i32), pltpu.VMEM(GG32.shape, i32), pltpu.VMEM(RR32.shape, i32),
        pltpu.VMEM((2, 3, R, 128), bf),
        pltpu.VMEM((2, 7, 128, 128), bf),
        pltpu.VMEM((5, 128, 128), f32),
        pltpu.VMEM((5, S // 2, 128), i32),
        pltpu.VMEM((2, 8, 128), i32),
        pltpu.VMEM((2, 8, 64, 128), i32),
        pltpu.VMEM((S // 2, D), i32),
        pltpu.VMEM((D // 2, 3 * D), i32),
        pltpu.VMEM((D // 2, D), i32),
        pltpu.VMEM((D // 2, D), i32),
        pltpu.VMEM((CFG.get('slots', 2), 4, 256, 128), f32),
        pltpu.VMEM((CFG.get('slots', 2), 4, 192, 128), i32),
        pltpu.VMEM((3, 64, D), i32),
        pltpu.VMEM((D, 128), f32),
        pltpu.VMEM((8, 64, 128), i32),
        pltpu.VMEM((2, 64, D), i32),
        pltpu.VMEM((S // 2, D), i32),
        pltpu.SemaphoreType.DMA((25,)),
        pltpu.SemaphoreType.DMA((6,)),
        pltpu.SemaphoreType.DMA((1,)),
    ]
    scratch += [pltpu.VMEM((17, 104, 256), f32)] * 4
    scratch += [pltpu.VMEM((S // 2, 128), i32)] * 8
    scratch += [pltpu.VMEM((4, NB, 32, 128), bf)] * 8
    return pl.pallas_call(
        _kernel,
        out_shape=jax.ShapeDtypeStruct((S, 2 * D), bf),
        in_specs=[pl.BlockSpec(memory_space=pl.ANY)] * 9,
        out_specs=pl.BlockSpec(memory_space=pl.ANY),
        scratch_shapes=scratch,
        compiler_params=pltpu.CompilerParams(vmem_limit_bytes=110 * 2 ** 20),
    )


@jax.jit
def pallas_concat_heads__spectral_gfnet__sliding_block__prompt_kernel(
    A_x: jax.Array,
    A_w_r: jax.Array,
    A_w_i: jax.Array,
    B_x: jax.Array,
    B_wqkv: jax.Array,
    B_wo: jax.Array,
):
    FF32, GG32, RR32 = _make_consts()
    out = _build(FF32, GG32, RR32)(
        A_x.reshape(S, D), A_w_r.T, A_w_i.T, B_x.reshape(S, D), B_wqkv, B_wo,
        jnp.asarray(FF32), jnp.asarray(GG32), jnp.asarray(RR32))
    return out.reshape(1, S, 2 * D)
```

```python
import numpy as np
import ml_dtypes
import jax
import jax.numpy as jnp
from jax import lax
import jax.experimental.pallas as pl
import jax.experimental.pallas.tpu as pltpu

S = 2048
D = 640
DF = 321
H = 32
DH = 20
NB = S // 128
R = 336
NEG = -1e30
CFG = {}
f32 = jnp.float32
bf = jnp.bfloat16
i32 = jnp.int32

C1 = float(np.cos(2 * np.pi / 5))
C2 = float(np.cos(4 * np.pi / 5))
S1 = float(np.sin(2 * np.pi / 5))
S2 = float(np.sin(4 * np.pi / 5))


def _pack_rows(a):
    u = np.ascontiguousarray(a.astype(ml_dtypes.bfloat16)).view(np.uint16).astype(np.uint32)
    return (u[..., 0::2, :] | (u[..., 1::2, :] << 16)).astype(np.uint32).view(np.int32)


def _make_consts():
    b5 = np.arange(128)

    def cs(k):
        th = 2 * np.pi * np.outer(k, b5) / D
        return np.cos(th), np.sin(th)

    m32 = np.arange(32)
    k0 = np.concatenate([10 * m32, 5 + 10 * m32, [320]])
    c, s = cs(k0)
    F0 = np.zeros((160, 128))
    F0[0:65] = c
    F0[80:145] = -s

    def kpair(j):
        return (np.concatenate([j + 10 * m32, j + 5 + 10 * m32]),
                np.concatenate([5 - j + 10 * m32, 10 - j + 10 * m32]))

    def fwd(j):
        ka, kb = kpair(j)
        (ca, sa), (cb, sb) = cs(ka), cs(kb)
        return np.concatenate([ca, cb, ca + sa, cb - sb, ca - sa, cb + sb], 0)

    FF = np.concatenate([F0, fwd(1), fwd(2)], 0)

    b = np.arange(128)
    f2 = np.arange(128)
    RR = np.zeros((16, 3, 128, 128))
    for a in range(16):
        th = -2 * np.pi * (np.outer(b, f2) / 128.0 + a * f2[None, :] / float(S))
        Mr, Mi = np.cos(th), np.sin(th)
        RR[a, 0] = Mr
        RR[a, 1] = Mr + Mi
        RR[a, 2] = Mr - Mi

    sc = 1.0 / (S * D)
    G0 = np.zeros((128, 128))
    al = np.full(65, 2.0)
    al[0] = 1.0
    al[64] = 1.0
    G0[:, 0:64] = (al[0:64, None] * c[0:64]).T
    G0[:, 64:128] = (-al[0:64, None] * s[0:64]).T
    G0[:, 64] = al[64] * c[64]

    def inv(j):
        ka, kb = kpair(j)
        (ca, sa), (cb, sb) = cs(ka), cs(kb)
        return 2 * np.concatenate([np.concatenate([ca, cb], 0).T,
                                   np.concatenate([ca + sa, sb - cb], 0).T,
                                   np.concatenate([sa - ca, -sb - cb], 0).T], 0)

    GG = np.concatenate([G0, inv(1), inv(2)], 0) * sc
    GG = GG.reshape(7, 128, 128).transpose(0, 2, 1).reshape(896, 128)
    return _pack_rows(FF), _pack_rows(GG), _pack_rows(RR)


_NT = (((1,), (1,)), ((), ()))


def _dot(a, b):
    return jnp.dot(a, b, preferred_element_type=f32)


def _dot_nt(a, b):
    return lax.dot_general(a, b, _NT, preferred_element_type=f32)


def _b16(x):
    return pltpu.bitcast(x, bf)


def _packi(a, b):
    return pltpu.pack_elementwise([a, b], packed_dtype=bf)


def _unpacki(x, idx):
    return pltpu.unpack_elementwise(x, index=idx, packed_dtype=bf, unpacked_dtype=f32)


def _zip16(x):
    n = x.shape[0] // 16
    return jnp.concatenate([_packi(x[16 * j:16 * j + 8], x[16 * j + 8:16 * j + 16]) for j in range(n)], 0)


def _dft4(z, inv):
    (a, b, c, d) = z
    t0 = (a[0] + c[0], a[1] + c[1])
    t1 = (a[0] - c[0], a[1] - c[1])
    t2 = (b[0] + d[0], b[1] + d[1])
    t3 = (b[0] - d[0], b[1] - d[1])
    o0 = (t0[0] + t2[0], t0[1] + t2[1])
    o2 = (t0[0] - t2[0], t0[1] - t2[1])
    p = (t1[0] + t3[1], t1[1] - t3[0])
    q = (t1[0] - t3[1], t1[1] + t3[0])
    return [o0, q, o2, p] if inv else [o0, p, o2, q]


def _tw16(z, e, inv):
    if e == 0:
        return z
    zr, zi = z
    if e == 4:
        return (-zi, zr) if inv else (zi, -zr)
    h = float(np.sqrt(0.5))
    if e == 2:
        return ((zr - zi) * h, (zr + zi) * h) if inv else ((zr + zi) * h, (zi - zr) * h)
    if e == 6:
        return ((-zr - zi) * h, (zr - zi) * h) if inv else ((zi - zr) * h, (-zr - zi) * h)
    sgn = 1.0 if inv else -1.0
    c = float(np.cos(2 * np.pi * e / 16))
    s = float(sgn * np.sin(2 * np.pi * e / 16))
    return (zr * c - zi * s, zr * s + zi * c)


def _fft16(z, inv):
    hh = [_dft4([z[a0 + 4 * a1] for a1 in range(4)], inv) for a0 in range(4)]
    out = [None] * 16
    for fa in range(4):
        o = _dft4([_tw16(hh[a0][fa], a0 * fa, inv) for a0 in range(4)], inv)
        for fb in range(4):
            out[fa + 4 * fb] = o[fb]
    return out


def _gwin(g):
    lo, hi = 80 * g, 80 * g + 79
    if lo // 128 == hi // 128:
        return ("nat", lo // 128, lo - 128 * (lo // 128))
    t = (lo - 64) // 128
    return ("shf", t, lo - 64 - 128 * t)


def _kernel(xa_hbm, wr_hbm, wi_hbm, xb_hbm, wqkv_hbm, wo_hbm, ff_hbm, gg_hbm, rr_hbm, out_hbm,
            xa32, wr32, wi32, wr_last, wi_last, ff32, gg32, rr32, ys_ref, zs_ref, ysc_ref, oa32,
            pin_ref, qw01_ref, xb32, wqkv32, wo32, wvt32, s_ref, p_ref, ob32, ot_ref, qw_ref, xz_ref, obo32,
            sem, osem, wsem, *groups):
    gs_refs = groups[0:4]
    kw_refs = groups[4:12]
    vt_refs = groups[12:20]

    def copy(src, dst, k):
        return pltpu.make_async_copy(src, dst, sem.at[k])

    xbh = xb_hbm.bitcast(i32)
    wqh = wqkv_hbm.bitcast(i32)
    xah = xa_hbm.bitcast(i32)
    oh32 = out_hbm.bitcast(i32)
    c_x0 = copy(xbh.at[pl.ds(0, 128)], xb32.at[pl.ds(0, 128)], 0)
    c_wk = copy(wqh.at[:, pl.ds(640, 640)], wqkv32.at[:, pl.ds(640, 640)], 1)
    c_wv = copy(wqh.at[:, pl.ds(1280, 640)], wqkv32.at[:, pl.ds(1280, 640)], 2)
    c_x1 = copy(xbh.at[pl.ds(128, 192)], xb32.at[pl.ds(128, 192)], 3)
    c_wq = copy(wqh.at[:, pl.ds(0, 640)], wqkv32.at[:, pl.ds(0, 640)], 4)
    c_ff = copy(ff_hbm, ff32, 5)
    c_xa = [copy(xah.at[:, pl.ds(128 * t, 128)], xa32.at[t], 6 + t) for t in range(5)]
    c_rr = copy(rr_hbm, rr32, 11)
    c_w = []
    for n, (src, dst, dst1) in enumerate(((wr_hbm, wr32, wr_last), (wi_hbm, wi32, wi_last))):
        w320 = src.at[pl.ds(0, 320)].bitcast(i32)
        for t in range(NB):
            c_w.append(pltpu.make_async_copy(w320.at[:, pl.ds(128 * t, 128)], dst.at[t], wsem.at[0]))
        c_w.append(copy(src.at[pl.ds(320, 1)], dst1, 13 + n))
    c_x2 = copy(xbh.at[pl.ds(320, 704)], xb32.at[pl.ds(320, 704)], 21)
    c_wo = copy(wo_hbm.bitcast(i32), wo32, 22)
    c_gg = copy(gg_hbm, gg32, 23)
    c_pin = copy(xbh.at[pl.ds(0, 8), pl.ds(0, 128)], pin_ref.at[0], 24)
    c_pin2 = copy(xbh.at[pl.ds(0, 8), pl.ds(0, 128)], pin_ref.at[1], 12)
    for cp in ([c_x0, c_wk, c_wv, c_x1, c_wq, c_wo, c_ff] + c_xa + [c_rr]
               + c_w + [c_x2, c_gg, c_pin, c_pin2]):
        cp.start()

    scale = float(DH ** -0.5 * np.log2(np.e))
    def _qpos(l):
        return (l & 16) + 4 * (l & 3) + ((l & 15) >> 2)
    rr_ = lax.broadcasted_iota(i32, (32, 128), 0)
    ll_ = _qpos(lax.broadcasted_iota(i32, (32, 128), 1))
    pos_ = rr_ & 15
    key_ = (rr_ & 16) + jnp.where(pos_ < 8, 2 * pos_, 2 * (pos_ - 8) + 1)
    le32 = key_ <= ll_
    wr_ = lax.broadcasted_iota(i32, (16, 128), 0)
    wq_ = _qpos(lax.broadcasted_iota(i32, (16, 128), 1))
    le_pk = (jnp.where(2 * wr_ <= wq_, jnp.int32(0xFFFF), jnp.int32(0))
             | jnp.where(2 * wr_ + 1 <= wq_, jnp.int32(-65536), jnp.int32(0)))
    lane8 = lax.broadcasted_iota(i32, (8, 128), 1)
    lane16 = lax.broadcasted_iota(i32, (16, 128), 1)
    bit0 = (lane16 & 32) != 0
    bit1 = (lane16 & 64) != 0
    bit0_8 = (lane8 & 32) != 0
    sub4 = lax.broadcasted_iota(i32, (8, 128), 0) < 4
    sub0 = lax.broadcasted_iota(i32, (8, 128), 0) == 0
    ones8 = jnp.ones((8, 128), f32)
    lo64 = lax.broadcasted_iota(i32, (64, 128), 1) < 64

    def rows_of(i):
        return i * 128 if isinstance(i, int) else pl.multiple_of(i * 128, 128)

    def wrows_of(i):
        return i * 64 if isinstance(i, int) else pl.multiple_of(i * 64, 64)

    def prep_wvt():
        for tr in range(5):
            wvt32[64 * tr:64 * tr + 64, :] = pltpu.bitcast(
                _b16(wqkv32[:, 1280 + tr * 128:1280 + (tr + 1) * 128]).T, i32)

    def prep_x(i):
        w = xb32[pl.ds(wrows_of(i), 64), :]
        z1 = _zip16(_b16(w).astype(f32))
        xz_ref[0] = z1
        xz_ref[1] = _zip16(_b16(z1).astype(f32))

    def win_ready(tiles, rolled, done, emit):
        for g in range(8):
            if g in done:
                continue
            kind, t, _ = _gwin(g)
            if kind == "nat":
                if t in tiles:
                    emit(g, tiles[t])
                    done.add(g)
            elif t in tiles and (t + 1) in tiles:
                for tt in (t, t + 1):
                    if tt not in rolled:
                        rolled[tt] = pltpu.roll(tiles[tt], 64, 1)
                emit(g, jnp.where(lo64, rolled[t], rolled[t + 1]))
                done.add(g)

    def proj_pieces(i, do_q=True, do_kv=True, qdst=None):
        qdst = qw_ref if qdst is None else qdst
        pieces = {}
        if do_kv:
            v8 = {}
            vdone = set()

            def vpiece(r):
                def f():
                    xb = _b16(xb32[pl.ds(wrows_of(i), 64), :])
                    vt = _dot_nt(_b16(wvt32[64 * r:64 * r + 64, :]), xb)
                    for j in range(16):
                        v8[16 * r + j] = vt[8 * j:8 * j + 8]
                    for p in range(16):
                        if p in vdone or any((5 * p + j) not in v8 for j in range(5)):
                            continue
                        v = [v8[5 * p + j] for j in range(5)]
                        h0, h1 = 2 * p, 2 * p + 1
                        vt_refs[h0 // 4][h0 % 4, i] = jnp.concatenate([v[0], v[1], v[2], ones8], 0).astype(bf)
                        vt_refs[h1 // 4][h1 % 4, i] = jnp.concatenate([v[2], v[3], v[4], ones8], 0).astype(bf)
                        vdone.add(p)
                return f

            kt, kr, kd = {}, {}, set()

            def kpiece(t):
                def f():
                    kt[t] = _zip16(_dot(_b16(xz_ref[1]), _b16(wqkv32[:, 640 + 128 * t:640 + 128 * t + 128])))

                    def emit(g, val):
                        kw_refs[g][pl.ds(wrows_of(i), 64), :] = val
                    win_ready(kt, kr, kd, emit)
                return f

            for r in range(5):
                pieces["v%d" % r] = vpiece(r)
                pieces["k%d" % r] = kpiece(r)
        if do_q:
            qt, qr, qd = {}, {}, set()

            def qpiece(t):
                def f():
                    qt[t] = _zip16(_dot(_b16(xz_ref[0]), _b16(wqkv32[:, 128 * t:128 * t + 128])) * scale)

                    def emit(g, val):
                        qdst[g] = val
                    win_ready(qt, qr, qd, emit)
                return f

            for t in range(5):
                pieces["q%d" % t] = qpiece(t)
        return pieces

    def out_pieces(i, slot=1):
        def opiece(t):
            def f():
                res = _dot(_b16(ob32[slot]), _b16(wo32[:, 128 * t:128 * t + 128]))
                obo32[pl.ds(wrows_of(i), 64), 128 * t:128 * t + 128] = _zip16(res)
            return f
        return {"o%d" % t: opiece(t) for t in range(5)}

    NSS = CFG.get('ss', 1)
    NSP = CFG.get('sp', 2)

    def key_tiles(i):
        return list(range(3)) if (not isinstance(i, int) or i >= 2) else list(range(2 - i, 3))

    pv_outs = {}
    last_pv = [None]

    def pv_group(g, i, es=(0, 1, 2, 3)):
        tiles = key_tiles(i)
        sl = g % NSP
        for e in es:
            P = _b16(p_ref[sl, e, 64 * tiles[0]:192, :])
            if len(tiles) > 1:
                vw = jnp.concatenate([vt_refs[g][e, i - 2 + j] for j in tiles], 1)
            else:
                vw = vt_refs[g][e, i]
            o = _dot(vw, P)
            rl = pltpu.reciprocal(o[24:32])
            res = [o[0:8] * rl, o[8:16] * rl, o[16:24] * rl]
            if e == 2:
                res = [pltpu.roll(r, 64, 1) for r in res]
            elif e == 1:
                res = [jnp.where(bit0_8, pltpu.roll(r, 32, 1), pltpu.roll(r, 96, 1)) for r in res]
            elif e == 3:
                res = [jnp.where(bit0_8, pltpu.roll(r, 96, 1), pltpu.roll(r, 32, 1)) for r in res]
            pv_outs[(g, e)] = res
            last_pv[0] = rl
            if (g, e ^ 1) in pv_outs:
                p = e // 2
                a, b = pv_outs.pop((g, 2 * p)), pv_outs.pop((g, 2 * p + 1))
                ot_ref[80 * g + 40 * p:80 * g + 40 * p + 40, :] = jnp.concatenate(
                    [a[0], a[1], jnp.where(sub4, a[2], b[0]), b[1], b[2]], 0)

    def fin_tile(t, slot):
        ob32[slot, :, 128 * t:128 * t + 128] = _zip16(ot_ref[128 * t:128 * t + 128, :].T)

    def ob_slot(i):
        return (0 if i in (0, 2) else (2 if i == 1 else 1)) if isinstance(i, int) else 1

    def finish(i):
        def f():
            pv_group(7, i)
            fin_tile(4, ob_slot(i))
        return f

    last_m = {}

    def token(n):
        kind = CFG.get("tok", {"0": "m", "1": "m", "2": "m", "3": "m"}).get(str(n))
        if kind == "m":
            g, u = max(last_m)
            return jnp.broadcast_to(last_m[(g, u)], (8, 128))
        if kind == "p":
            return last_pv[0]
        return None

    def attn(i, plan, head=None, qsrc=None, lazy=False):
        qsrc = qw_ref if qsrc is None else qsrc
        static = isinstance(i, int)
        lov = (lambda u: max(0, 8 - u - 4 * i)) if static else (lambda u: 0)
        tiles = key_tiles(i)
        ms = last_m

        def phase_a(g, us):
            sl = g % NSS
            _, _, off = _gwin(g)
            hm = [jnp.where((lane16 >= off + 20 * e) & (lane16 < off + 20 * e + 20), jnp.int32(-1), jnp.int32(0))
                  for e in range(4)]
            for u in us:
                lo = lov(u)
                nrow = 32 * (9 - lo)
                k0 = 64 * i - 128 + 16 * u + 16 * lo
                if not static:
                    k0 = pl.multiple_of(k0, 16)
                kw = _b16(kw_refs[g][pl.ds(k0, nrow // 2), :])
                qu = qsrc[g, 16 * u:16 * u + 16, :]
                qm = _b16(jnp.concatenate([qu & hm[lam ^ u] for lam in range(4)], 0))
                s = _dot_nt(kw, qm)
                sd = s[nrow - 32:nrow]
                if lo == 0:
                    T = jnp.where(le32, sd, s[0:32])
                    F = s[32:256]
                else:
                    T = jnp.where(le32, sd, NEG)
                    F = s[0:nrow - 32]
                m = jnp.max(T, axis=0, keepdims=True)
                s_ref[sl, u, 0:32] = T
                if F.shape[0] > 0:
                    m = jnp.maximum(m, jnp.max(F, axis=0, keepdims=True))
                    s_ref[sl, u, 32:32 + F.shape[0]] = F
                ms[(g, u)] = m

        def sel(m, a, b):
            if a is None and b is None:
                return None
            if a is None:
                a = jnp.zeros((16, 128), i32)
            if b is None:
                b = jnp.zeros((16, 128), i32)
            return jnp.where(m, a, b)

        def phase_b1(g):
            sl = g % NSS
            slp = g % NSP
            lo_ = [lov(u) for u in range(4)]
            nf = [7 if lo_[u] == 0 else 8 - lo_[u] for u in range(4)]

            def pblock(u, row0):
                p = jnp.exp2(s_ref[sl, u, row0:row0 + 32] - ms[(g, u)])
                return jnp.concatenate([_packi(p[16 * j:16 * j + 8], p[16 * j + 8:16 * j + 16]) for j in range(2)], 0)

            tri = {}

            def block(u, rel):
                if rel < 0 or rel > 8:
                    return None
                if rel == 0 or rel == 8:
                    if u not in tri:
                        pt = pblock(u, 0)
                        if lo_[u] == 0:
                            p8 = pt & le_pk
                            tri[u] = {8: p8, 0: pt ^ p8}
                        else:
                            tri[u] = {8: pt, 0: None}
                    return tri[u][rel]
                first = 8 - nf[u]
                if rel < first:
                    return None
                return pblock(u, 32 + 32 * (rel - first))

            for beta in range(4 * tiles[0], 12):
                src = [block(u, beta - u) for u in range(4)]
                a0 = sel(bit0, src[1], src[0])
                a1 = sel(bit0, src[0], src[1])
                c0 = sel(bit0, src[3], src[2])
                c1 = sel(bit0, src[2], src[3])
                o4 = [sel(bit1, c0, a0), sel(bit1, c1, a1), sel(bit1, a0, c0), sel(bit1, a1, c1)]
                for e in range(4):
                    p_ref[slp, e, 16 * beta:16 * beta + 16, :] = (
                        o4[e] if o4[e] is not None else jnp.zeros((16, 128), i32))

        okey = "order" if not static else ("order_pre" if i in (2, 3) else ("order_post" if i == NB - 1 else "order_01"))
        order = CFG.get(okey, {"order": "B P0 A0 A1 A2 A3 P1 P2 P3 X X Y",
                               "order_pre": "B A0 A1 P0 A2 P1 A3 X P2 X P3 Y",
                               "order_post": "B A0 A1 A2 P0 P1 P2 A3 P3 X X Y",
                               "order_01": "B P0 P1 A0 A1 A2 A3 P2 P3 X X Y"}[okey])

        def step(s):
            if s == -1 and head is not None:
                head()
            px = plan.get(s, [])
            todo = list(range(len(px)))
            for tok in order.split():
                if tok[0] == "A" and 0 <= s + 1 < 8:
                    phase_a(s + 1, [int(c) for c in tok[1:]])
                if tok[0] == "B" and 0 <= s < 8:
                    phase_b1(s)
                if tok[0] == "P" and 0 <= s - 1 < 8:
                    pv_group(s - 1, i, [int(c) for c in tok[1:]])
                if tok[0] == "X" and todo:
                    px[todo.pop(0)]()
                if tok[0] == "Y":
                    while todo:
                        px[todo.pop(0)]()
            while todo:
                px[todo.pop(0)]()
            if s == 7:
                for t in range(4):
                    fin_tile(t, ob_slot(i))

        steps = [(lambda s=s: step(s)) for s in range(-1, 8)]
        if lazy:
            return steps
        for f in steps:
            f()

    def a1_step(ax, ay, order):
        w = {}
        if ax is not None:
            j, par = ax // 2, ax % 2
            x = [_unpacki(xa32[t, pl.ds(j, 128, stride=8), :], par) for t in range(5)]
            t1 = x[1] + x[4]
            t2 = x[2] + x[3]
            t3 = x[1] - x[4]
            t4 = x[2] - x[3]
            p1 = x[0] + C1 * t1 + C2 * t2
            p2 = x[0] + C2 * t1 + C1 * t2
            q1 = S1 * t3 + S2 * t4
            q2 = S2 * t3 - S1 * t4
            ops = [x[0] + t1 + t2, p1 + q1, q1, p1, p2 + q2, q2, p2]
            w0s = [0, 80, 144, 208, 272, 336, 400, 464]
        for tok in order:
            if tok[0] == "x" and ax is not None:
                n = int(tok[1])
                w[tok] = _dot_nt(_b16(ff32[w0s[n]:w0s[n + 1]]), ops[n].astype(bf))
            if tok[0] == "y" and ay is not None:
                n = int(tok[1])
                w[tok] = _dot(ys_ref[ay % 2, n], _b16(rr32[ay, n]))
        if ay is not None:
            g_ = jnp.concatenate([w["y0"] - w["y1"], w["y0"] - w["y2"]], 1)
            for g in range(R // 8):
                gs_refs[g % 4][ay, 8 * (g // 4):8 * (g // 4) + 8, :] = g_[8 * g:8 * g + 8]
        if ax is not None:
            re, im = [w["x0"][0:80]], [w["x0"][80:160]]
            for n in (1, 4):
                t1, t2, t3 = w["x%d" % n], w["x%d" % (n + 1)], w["x%d" % (n + 2)]
                re.append(t1 - t2)
                im += [t3[0:64] - t1[0:64], t1[64:128] - t3[64:128]]
            yr = jnp.concatenate(re, 0)
            yi = jnp.concatenate(im, 0)
            ys_ref[ax % 2, 0] = (yr + yi).astype(bf)
            ys_ref[ax % 2, 1] = yi.astype(bf)
            ys_ref[ax % 2, 2] = yr.astype(bf)

    def a2_group(n, gq, token=None):
        g = 4 * gq + n
        special = isinstance(gq, int) and g == 8
        if isinstance(gq, int):
            w8 = g if g < 8 else (g - 10) % 8
            c10 = [0, 1, 4, 2, 3][0 if g < 8 else (g - 10) // 8 + 1] + 5 * (w8 // 4)
            r0 = 8 * gq
        else:
            w8 = jnp.where(g < 8, g, (g - 10) & 7)
            blk = jnp.minimum(jnp.where(g < 10, 0, ((g - 10) >> 3) + 1), 4)
            c10 = jnp.where(blk == 2, 4, jnp.where(blk > 2, blk - 1, blk)) + 5 * (w8 >> 2)
            r0 = 8 * gq
            if n == 0:
                r0 = jnp.where(g == 8, 96, r0)
            r0 = pl.multiple_of(r0, 8)
        w0 = (c10 >> 1) + 40 * (w8 & 3)
        sh = 16 * (1 - (c10 & 1))

        def wload(ref, last, f1):
            if special:
                return jnp.broadcast_to(last[0:1, 128 * f1:128 * f1 + 128].astype(f32), (8, 128))
            return pltpu.bitcast((ref[f1, pl.ds(w0, 8, stride=5), :] << sh) & jnp.int32(-65536), f32)

        gref = gs_refs[n]
        if token is not None:
            gref[16, pl.ds(pl.multiple_of(8 * (gq & 15), 8), 8), 0:128] = token
        z = [(gref[a, pl.ds(r0, 8), 0:128], gref[a, pl.ds(r0, 8), 128:256]) for a in range(16)]
        X = _fft16(z, False)
        V = []
        for f1 in range(16):
            wr = wload(wr32, wr_last, f1)
            wi = wload(wi32, wi_last, f1)
            V.append((X[f1][0] * wr - X[f1][1] * wi, X[f1][0] * wi + X[f1][1] * wr))
        U = _fft16(V, True)
        for a in range(16):
            gref[a, pl.ds(r0, 8), 0:128] = U[a][0]
            gref[a, pl.ds(r0, 8), 128:256] = U[a][1]

    def a3_step(az, ad, order, extra=()):
        w = {}
        if az is not None:
            u = jnp.concatenate([gs_refs[g % 4][az, 8 * (g // 4):8 * (g // 4) + 8, :] for g in range(R // 8)], 0)
            ur = u[:, 0:128]
            ui = u[:, 128:256]
            zops = [(ur + ui, 0), (ui, 2), (ur, 1)]
        for tok in order:
            if tok[0] == "z" and az is not None:
                v, n = zops[int(tok[1])]
                w[tok] = _dot_nt(v.astype(bf), _b16(rr32[az, n]))
            if tok[0] == "d" and ad is not None:
                n = int(tok[1])
                w[tok] = _dot(zs_ref[ad % 2, n], _b16(gg32[64 * n:64 * n + 64]))
            if tok == "E":
                for f in extra:
                    f()
        if ad is not None:
            v0 = w["d0"]
            v1r, v1i = w["d1"] - w["d2"], w["d1"] + w["d3"]
            v2r, v2i = w["d4"] - w["d5"], w["d4"] + w["d6"]
            A1 = v0 + C1 * v1r + C2 * v2r
            A2 = v0 + C2 * v1r + C1 * v2r
            B1 = S1 * v1i + S2 * v2i
            B2 = S2 * v1i - S1 * v2i
            y = [v0 + v1r + v2r, A1 - B1, A2 - B2, A2 + B2, A1 + B1]
            for t in range(5):
                if ad % 2 == 0:
                    ysc_ref[t] = y[t]
                else:
                    oa32[t, pl.ds(ad // 2, 128, stride=8), :] = _packi(ysc_ref[t], y[t])
        if az is not None:
            zr = w["z0"] - w["z1"]
            zi = w["z0"] - w["z2"]
            kop = [jnp.concatenate([zr[0:64], jnp.where(sub0, zr[64:72], zi[0:8]), zi[8:64]], 0)]
            for r0 in (80, 208):
                kop += [jnp.concatenate([zr[r0:r0 + 64] + zi[r0:r0 + 64], zr[r0 + 64:r0 + 128] - zi[r0 + 64:r0 + 128]], 0),
                        zi[r0:r0 + 128], zr[r0:r0 + 128]]
            for n in range(7):
                zs_ref[az % 2, n] = kop[n].T.astype(bf)

    def run(pieces, order=None):
        for k in (order or list(pieces)):
            if k in pieces:
                pieces[k]()

    PLAN = {-1: ["v0", "v1"], 0: ["k0", "q0"], 1: ["k1", "q1", "a0"], 2: ["k2", "q2"], 3: ["o0", "o1", "a1"],
            4: ["k3", "q3"], 5: ["o2", "o3", "a2"], 6: ["o4", "v2", "a3"], 7: ["k4", "q4", "v3", "v4"]}

    if 'plan' in CFG:
        PLAN = {int(k): v for k, v in CFG['plan'].items()}

    def mkplan(pieces):
        return {s_: [pieces[k] for k in ks if k in pieces] for s_, ks in PLAN.items()}

    ORD = ["v0", "v1", "v2", "v3", "v4", "k0", "k1", "k2", "k3", "k4", "q0", "q1", "q2", "q3", "q4"]

    def out_b_copy(i):
        return pltpu.make_async_copy(obo32.at[pl.ds(wrows_of(i), 64)],
                                     oh32.at[pl.ds(wrows_of(i), 64), pl.ds(D, D)], osem.at[0])

    for g in range(R // 8, 44):
        gs_refs[g % 4][0:16, 8 * (g // 4):8 * (g // 4) + 8, :] = jnp.zeros((16, 8, 256), f32)
    gs_refs[0][0:16, 96:104, :] = jnp.zeros((16, 8, 256), f32)
    c_x0.wait()
    c_wk.wait()
    prep_x(0)
    P0 = proj_pieces(0, do_q=False)
    run(P0, ["k0", "k1", "k2", "k3", "k4"])
    prep_x(1)
    P1 = proj_pieces(1, do_q=False)
    run(P1, ["k0", "k1", "k2", "k3", "k4"])
    c_wv.wait()
    prep_wvt()
    run(P0, ["v0", "v1", "v2", "v3", "v4"])
    run(P1, ["v0", "v1", "v2", "v3", "v4"])
    c_x1.wait()
    c_wq.wait()
    prep_x(2)
    run(proj_pieces(2), ORD)
    prep_x(3)
    attn(2, mkplan(proj_pieces(3)))
    prep_x(4)
    attn(3, mkplan(proj_pieces(4)), head=finish(2))
    for i_ in range(2):
        prep_x(i_)
        run(proj_pieces(i_, do_kv=False, qdst=qw01_ref.at[i_]), ORD)

    for cp in [c_wo, c_ff] + c_xa + [c_rr]:
        cp.wait()
    P2 = out_pieces(2, slot=0)
    run(P2, ["o0", "o1", "o2"])
    a1o = CFG.get("a1", "x0 x1 x2 x3 y0 x4 y1 x5 y2 x6").split()
    a1_step(0, None, a1o)
    run(P2, ["o3", "o4"])
    for a in range(16):
        a1_step(a + 1 if a < 15 else None, a, a1o)
    for cp in c_w:
        cp.wait()
    c_x2.wait()
    c_gg.wait()

    def one_block(i):
        nxt = jnp.minimum(i + 1, NB - 1)
        prep_x(nxt)
        P = proj_pieces(nxt)
        P.update(out_pieces(i - 1))
        for n in range(4):
            P["a%d" % n] = (lambda n=n: a2_group(n, i - 4, token(n)))
        last_m.clear()
        attn(i, mkplan(P), head=finish(i - 1))

    UNR = CFG.get("unroll", 1)

    def body(it, carry):
        for u_ in range(UNR):
            i = 4 + UNR * it + u_
            one_block(i)
            out_b_copy(i - 1).start()
        return carry

    out_b_copy(2).start()
    lax.fori_loop(0, NB - 5, body, 0)

    finish(NB - 2)()
    a2_group(0, 2)

    extra = attn(0, {}, qsrc=qw01_ref.at[0], lazy=True) + attn(1, {}, head=finish(0), qsrc=qw01_ref.at[1], lazy=True)
    extra += [lambda: pv_group(7, 1), lambda: fin_tile(4, 2)]
    a3o = CFG.get("a3", "z0 z1 z2 d0 d1 d2 d3 d4 d5 d6 E").split()
    a3_step(0, None, a3o)
    for a in range(16):
        a3_step(a + 1 if a < 15 else None, a, a3o, extra[(len(extra) * a) // 16:(len(extra) * (a + 1)) // 16])
    c_oa = [pltpu.make_async_copy(oa32.at[t], oh32.at[:, pl.ds(128 * t, 128)], osem.at[1 + t]) for t in range(5)]
    for cp in c_oa:
        cp.start()
    c_pin.wait()

    fill = []
    for t in range(5):
        fill += [out_pieces(0, slot=0)["o%d" % t], out_pieces(1, slot=2)["o%d" % t], out_pieces(NB - 2)["o%d" % t]]
    last_m.clear()
    attn(NB - 1, {s_: fill[(15 * (s_ + 1)) // 9:(15 * (s_ + 2)) // 9] for s_ in range(-1, 8)})
    for i_ in (0, 1, NB - 2):
        out_b_copy(i_).start()
    c_pin2.wait()
    finish(NB - 1)()
    run(out_pieces(NB - 1))
    out_b_copy(NB - 1).start()

    for cp in c_oa:
        cp.wait()
    for i in range(NB):
        out_b_copy(i).wait()


def _build(FF32, GG32, RR32):
    scratch = [
        pltpu.VMEM((5, S // 2, 128), i32),
        pltpu.VMEM((NB, 160, 128), i32), pltpu.VMEM((NB, 160, 128), i32),
        pltpu.VMEM((1, S), bf), pltpu.VMEM((1, S), bf),
        pltpu.VMEM(FF32.shape, i32), pltpu.VMEM(GG32.shape, i32), pltpu.VMEM(RR32.shape, i32),
        pltpu.VMEM((2, 3, R, 128), bf),
        pltpu.VMEM((2, 7, 128, 128), bf),
        pltpu.VMEM((5, 128, 128), f32),
        pltpu.VMEM((5, S // 2, 128), i32),
        pltpu.VMEM((2, 8, 128), i32),
        pltpu.VMEM((2, 8, 64, 128), i32),
        pltpu.VMEM((S // 2, D), i32),
        pltpu.VMEM((D // 2, 3 * D), i32),
        pltpu.VMEM((D // 2, D), i32),
        pltpu.VMEM((D // 2, D), i32),
        pltpu.VMEM((CFG.get('ss', 1), 4, 256, 128), f32),
        pltpu.VMEM((CFG.get('sp', 2), 4, 192, 128), i32),
        pltpu.VMEM((3, 64, D), i32),
        pltpu.VMEM((D, 128), f32),
        pltpu.VMEM((8, 64, 128), i32),
        pltpu.VMEM((2, 64, D), i32),
        pltpu.VMEM((S // 2, D), i32),
        pltpu.SemaphoreType.DMA((25,)),
        pltpu.SemaphoreType.DMA((6,)),
        pltpu.SemaphoreType.DMA((1,)),
    ]
    scratch += [pltpu.VMEM((17, 104, 256), f32)] * 4
    scratch += [pltpu.VMEM((S // 2, 128), i32)] * 8
    scratch += [pltpu.VMEM((4, NB, 32, 128), bf)] * 8
    return pl.pallas_call(
        _kernel,
        out_shape=jax.ShapeDtypeStruct((S, 2 * D), bf),
        in_specs=[pl.BlockSpec(memory_space=pl.ANY)] * 9,
        out_specs=pl.BlockSpec(memory_space=pl.ANY),
        scratch_shapes=scratch,
        compiler_params=pltpu.CompilerParams(vmem_limit_bytes=110 * 2 ** 20),
    )


@jax.jit
def pallas_concat_heads__spectral_gfnet__sliding_block__prompt_kernel(
    A_x: jax.Array,
    A_w_r: jax.Array,
    A_w_i: jax.Array,
    B_x: jax.Array,
    B_wqkv: jax.Array,
    B_wo: jax.Array,
):
    FF32, GG32, RR32 = _make_consts()
    out = _build(FF32, GG32, RR32)(
        A_x.reshape(S, D), A_w_r.T, A_w_i.T, B_x.reshape(S, D), B_wqkv, B_wo,
        jnp.asarray(FF32), jnp.asarray(GG32), jnp.asarray(RR32))
    return out.reshape(1, S, 2 * D)
```

```python
import numpy as np
import ml_dtypes
import jax
import jax.numpy as jnp
from jax import lax
import jax.experimental.pallas as pl
import jax.experimental.pallas.tpu as pltpu

S = 2048
D = 640
DF = 321
H = 32
DH = 20
NB = S // 128
R = 336
NEG = -1e30
CFG = {}
f32 = jnp.float32
bf = jnp.bfloat16
i32 = jnp.int32

C1 = float(np.cos(2 * np.pi / 5))
C2 = float(np.cos(4 * np.pi / 5))
S1 = float(np.sin(2 * np.pi / 5))
S2 = float(np.sin(4 * np.pi / 5))


def _pack_rows(a):
    u = np.ascontiguousarray(a.astype(ml_dtypes.bfloat16)).view(np.uint16).astype(np.uint32)
    return (u[..., 0::2, :] | (u[..., 1::2, :] << 16)).astype(np.uint32).view(np.int32)


def _make_consts():
    b5 = np.arange(128)

    def cs(k):
        th = 2 * np.pi * np.outer(k, b5) / D
        return np.cos(th), np.sin(th)

    m32 = np.arange(32)
    k0 = np.concatenate([10 * m32, 5 + 10 * m32, [320]])
    c, s = cs(k0)
    F0 = np.zeros((160, 128))
    F0[0:65] = c
    F0[80:145] = -s

    def kpair(j):
        return (np.concatenate([j + 10 * m32, j + 5 + 10 * m32]),
                np.concatenate([5 - j + 10 * m32, 10 - j + 10 * m32]))

    def fwd(j):
        ka, kb = kpair(j)
        (ca, sa), (cb, sb) = cs(ka), cs(kb)
        return np.concatenate([ca, cb, ca + sa, cb - sb, ca - sa, cb + sb], 0)

    FF = np.concatenate([F0, fwd(1), fwd(2)], 0)

    b = np.arange(128)
    f2 = np.arange(128)
    RR = np.zeros((16, 3, 128, 128))
    for a in range(16):
        th = -2 * np.pi * (np.outer(b, f2) / 128.0 + a * f2[None, :] / float(S))
        Mr, Mi = np.cos(th), np.sin(th)
        RR[a, 0] = Mr
        RR[a, 1] = Mr + Mi
        RR[a, 2] = Mr - Mi

    sc = 1.0 / (S * D)
    G0 = np.zeros((128, 128))
    al = np.full(65, 2.0)
    al[0] = 1.0
    al[64] = 1.0
    G0[:, 0:64] = (al[0:64, None] * c[0:64]).T
    G0[:, 64:128] = (-al[0:64, None] * s[0:64]).T
    G0[:, 64] = al[64] * c[64]

    def inv(j):
        ka, kb = kpair(j)
        (ca, sa), (cb, sb) = cs(ka), cs(kb)
        return 2 * np.concatenate([np.concatenate([ca, cb], 0).T,
                                   np.concatenate([ca + sa, sb - cb], 0).T,
                                   np.concatenate([sa - ca, -sb - cb], 0).T], 0)

    GG = np.concatenate([G0, inv(1), inv(2)], 0) * sc
    GG = GG.reshape(7, 128, 128).transpose(0, 2, 1).reshape(896, 128)
    return _pack_rows(FF), _pack_rows(GG), _pack_rows(RR)


_NT = (((1,), (1,)), ((), ()))


def _dot(a, b):
    return jnp.dot(a, b, preferred_element_type=f32)


def _dot_nt(a, b):
    return lax.dot_general(a, b, _NT, preferred_element_type=f32)


def _b16(x):
    return pltpu.bitcast(x, bf)


def _packi(a, b):
    return pltpu.pack_elementwise([a, b], packed_dtype=bf)


def _unpacki(x, idx):
    return pltpu.unpack_elementwise(x, index=idx, packed_dtype=bf, unpacked_dtype=f32)


def _zip16(x):
    n = x.shape[0] // 16
    return jnp.concatenate([_packi(x[16 * j:16 * j + 8], x[16 * j + 8:16 * j + 16]) for j in range(n)], 0)


def _dft4(z, inv):
    (a, b, c, d) = z
    t0 = (a[0] + c[0], a[1] + c[1])
    t1 = (a[0] - c[0], a[1] - c[1])
    t2 = (b[0] + d[0], b[1] + d[1])
    t3 = (b[0] - d[0], b[1] - d[1])
    o0 = (t0[0] + t2[0], t0[1] + t2[1])
    o2 = (t0[0] - t2[0], t0[1] - t2[1])
    p = (t1[0] + t3[1], t1[1] - t3[0])
    q = (t1[0] - t3[1], t1[1] + t3[0])
    return [o0, q, o2, p] if inv else [o0, p, o2, q]


def _tw16(z, e, inv):
    if e == 0:
        return z
    zr, zi = z
    if e == 4:
        return (-zi, zr) if inv else (zi, -zr)
    h = float(np.sqrt(0.5))
    if e == 2:
        return ((zr - zi) * h, (zr + zi) * h) if inv else ((zr + zi) * h, (zi - zr) * h)
    if e == 6:
        return ((-zr - zi) * h, (zr - zi) * h) if inv else ((zi - zr) * h, (-zr - zi) * h)
    sgn = 1.0 if inv else -1.0
    c = float(np.cos(2 * np.pi * e / 16))
    s = float(sgn * np.sin(2 * np.pi * e / 16))
    return (zr * c - zi * s, zr * s + zi * c)


def _fft16(z, inv):
    hh = [_dft4([z[a0 + 4 * a1] for a1 in range(4)], inv) for a0 in range(4)]
    out = [None] * 16
    for fa in range(4):
        o = _dft4([_tw16(hh[a0][fa], a0 * fa, inv) for a0 in range(4)], inv)
        for fb in range(4):
            out[fa + 4 * fb] = o[fb]
    return out


def _gwin(g):
    lo, hi = 80 * g, 80 * g + 79
    if lo // 128 == hi // 128:
        return ("nat", lo // 128, lo - 128 * (lo // 128))
    t = (lo - 64) // 128
    return ("shf", t, lo - 64 - 128 * t)


def _kernel(xa_hbm, wr_hbm, wi_hbm, xb_hbm, wqkv_hbm, wo_hbm, ff_hbm, gg_hbm, rr_hbm, out_hbm,
            xa32, wr32, wi32, wr_last, wi_last, ff32, gg32, rr32, ys_ref, zs_ref, ysc_ref, oa32,
            pin_ref, qw01_ref, xb32, wqkv32, wo32, wvt32, s_ref, p_ref, ob32, ot_ref, qw_ref, xz_ref, obo32,
            sem, osem, wsem, *groups):
    gs_refs = groups[0:4]
    kw_refs = groups[4:12]
    vt_refs = groups[12:20]

    def copy(src, dst, k):
        return pltpu.make_async_copy(src, dst, sem.at[k])

    xbh = xb_hbm.bitcast(i32)
    wqh = wqkv_hbm.bitcast(i32)
    xah = xa_hbm.bitcast(i32)
    oh32 = out_hbm.bitcast(i32)
    c_x0 = copy(xbh.at[pl.ds(0, 128)], xb32.at[pl.ds(0, 128)], 0)
    c_wk = copy(wqh.at[:, pl.ds(640, 640)], wqkv32.at[:, pl.ds(640, 640)], 1)
    c_wv = copy(wqh.at[:, pl.ds(1280, 640)], wqkv32.at[:, pl.ds(1280, 640)], 2)
    c_x1 = copy(xbh.at[pl.ds(128, 192)], xb32.at[pl.ds(128, 192)], 3)
    c_wq = copy(wqh.at[:, pl.ds(0, 640)], wqkv32.at[:, pl.ds(0, 640)], 4)
    c_ff = copy(ff_hbm, ff32, 5)
    c_xa = [copy(xah.at[:, pl.ds(128 * t, 128)], xa32.at[t], 6 + t) for t in range(5)]
    c_rr = copy(rr_hbm, rr32, 11)
    c_w = []
    for n, (src, dst, dst1) in enumerate(((wr_hbm, wr32, wr_last), (wi_hbm, wi32, wi_last))):
        w320 = src.at[pl.ds(0, 320)].bitcast(i32)
        for t in range(NB):
            c_w.append(pltpu.make_async_copy(w320.at[:, pl.ds(128 * t, 128)], dst.at[t], wsem.at[0]))
        c_w.append(copy(src.at[pl.ds(320, 1)], dst1, 13 + n))
    c_x2 = copy(xbh.at[pl.ds(320, 704)], xb32.at[pl.ds(320, 704)], 21)
    c_wo = copy(wo_hbm.bitcast(i32), wo32, 22)
    c_gg = copy(gg_hbm, gg32, 23)
    c_pin = copy(xbh.at[pl.ds(0, 8), pl.ds(0, 128)], pin_ref.at[0], 24)
    c_pin2 = copy(xbh.at[pl.ds(0, 8), pl.ds(0, 128)], pin_ref.at[1], 12)
    for cp in ([c_x0, c_wk, c_wv, c_x1, c_wq, c_wo, c_ff] + c_xa + [c_rr]
               + c_w + [c_x2, c_gg, c_pin, c_pin2]):
        cp.start()

    scale = float(DH ** -0.5 * np.log2(np.e))
    def _qpos(l):
        return (l & 16) + 4 * (l & 3) + ((l & 15) >> 2)
    rr_ = lax.broadcasted_iota(i32, (32, 128), 0)
    ll_ = _qpos(lax.broadcasted_iota(i32, (32, 128), 1))
    pos_ = rr_ & 15
    key_ = (rr_ & 16) + jnp.where(pos_ < 8, 2 * pos_, 2 * (pos_ - 8) + 1)
    le32 = key_ <= ll_
    wr_ = lax.broadcasted_iota(i32, (16, 128), 0)
    wq_ = _qpos(lax.broadcasted_iota(i32, (16, 128), 1))
    le_pk = (jnp.where(2 * wr_ <= wq_, jnp.int32(0xFFFF), jnp.int32(0))
             | jnp.where(2 * wr_ + 1 <= wq_, jnp.int32(-65536), jnp.int32(0)))
    lane8 = lax.broadcasted_iota(i32, (8, 128), 1)
    lane16 = lax.broadcasted_iota(i32, (16, 128), 1)
    bit0 = (lane16 & 32) != 0
    bit1 = (lane16 & 64) != 0
    bit0_8 = (lane8 & 32) != 0
    sub4 = lax.broadcasted_iota(i32, (8, 128), 0) < 4
    sub0 = lax.broadcasted_iota(i32, (8, 128), 0) == 0
    ones8 = jnp.ones((8, 128), f32)
    lo64 = lax.broadcasted_iota(i32, (64, 128), 1) < 64

    def rows_of(i):
        return i * 128 if isinstance(i, int) else pl.multiple_of(i * 128, 128)

    def wrows_of(i):
        return i * 64 if isinstance(i, int) else pl.multiple_of(i * 64, 64)

    def prep_wvt():
        for tr in range(5):
            wvt32[64 * tr:64 * tr + 64, :] = pltpu.bitcast(
                _b16(wqkv32[:, 1280 + tr * 128:1280 + (tr + 1) * 128]).T, i32)

    def prep_x(i):
        w = xb32[pl.ds(wrows_of(i), 64), :]
        z1 = _zip16(_b16(w).astype(f32))
        xz_ref[0] = z1
        xz_ref[1] = _zip16(_b16(z1).astype(f32))

    def win_ready(tiles, rolled, done, emit):
        for g in range(8):
            if g in done:
                continue
            kind, t, _ = _gwin(g)
            if kind == "nat":
                if t in tiles:
                    emit(g, tiles[t])
                    done.add(g)
            elif t in tiles and (t + 1) in tiles:
                for tt in (t, t + 1):
                    if tt not in rolled:
                        rolled[tt] = pltpu.roll(tiles[tt], 64, 1)
                emit(g, jnp.where(lo64, rolled[t], rolled[t + 1]))
                done.add(g)

    def proj_pieces(i, do_q=True, do_kv=True, qdst=None):
        qdst = qw_ref if qdst is None else qdst
        pieces = {}
        if do_kv:
            v8 = {}
            vdone = set()

            def vpiece(r):
                def f():
                    xb = _b16(xb32[pl.ds(wrows_of(i), 64), :])
                    vt = _dot_nt(_b16(wvt32[64 * r:64 * r + 64, :]), xb)
                    for j in range(16):
                        v8[16 * r + j] = vt[8 * j:8 * j + 8]
                    for p in range(16):
                        if p in vdone or any((5 * p + j) not in v8 for j in range(5)):
                            continue
                        v = [v8[5 * p + j] for j in range(5)]
                        h0, h1 = 2 * p, 2 * p + 1
                        vt_refs[h0 // 4][h0 % 4, i] = jnp.concatenate([v[0], v[1], v[2], ones8], 0).astype(bf)
                        vt_refs[h1 // 4][h1 % 4, i] = jnp.concatenate([v[2], v[3], v[4], ones8], 0).astype(bf)
                        vdone.add(p)
                return f

            kt, kr, kd = {}, {}, set()

            def kpiece(t):
                def f():
                    kt[t] = _zip16(_dot(_b16(xz_ref[1]), _b16(wqkv32[:, 640 + 128 * t:640 + 128 * t + 128])))

                    def emit(g, val):
                        kw_refs[g][pl.ds(wrows_of(i), 64), :] = val
                    win_ready(kt, kr, kd, emit)
                return f

            for r in range(5):
                pieces["v%d" % r] = vpiece(r)
                pieces["k%d" % r] = kpiece(r)
        if do_q:
            qt, qr, qd = {}, {}, set()

            def qpiece(t):
                def f():
                    qt[t] = _zip16(_dot(_b16(xz_ref[0]), _b16(wqkv32[:, 128 * t:128 * t + 128])) * scale)

                    def emit(g, val):
                        qdst[g] = val
                    win_ready(qt, qr, qd, emit)
                return f

            for t in range(5):
                pieces["q%d" % t] = qpiece(t)
        return pieces

    def out_pieces(i, slot=1):
        def opiece(t):
            def f():
                res = _dot(_b16(ob32[slot]), _b16(wo32[:, 128 * t:128 * t + 128]))
                obo32[pl.ds(wrows_of(i), 64), 128 * t:128 * t + 128] = _zip16(res)
            return f
        return {"o%d" % t: opiece(t) for t in range(5)}

    NSS = CFG.get('ss', 1)
    NSP = CFG.get('sp', 2)

    def key_tiles(i):
        return list(range(3)) if (not isinstance(i, int) or i >= 2) else list(range(2 - i, 3))

    pv_outs = {}
    last_pv = [None]

    def pv_group(g, i, es=(0, 1, 2, 3)):
        tiles = key_tiles(i)
        sl = g % NSP
        for e in es:
            P = _b16(p_ref[sl, e, 64 * tiles[0]:192, :])
            if len(tiles) > 1:
                vw = jnp.concatenate([vt_refs[g][e, i - 2 + j] for j in tiles], 1)
            else:
                vw = vt_refs[g][e, i]
            o = _dot(vw, P)
            rl = pltpu.reciprocal(o[24:32])
            res = [o[0:8] * rl, o[8:16] * rl, o[16:24] * rl]
            if e == 2:
                res = [pltpu.roll(r, 64, 1) for r in res]
            elif e == 1:
                res = [jnp.where(bit0_8, pltpu.roll(r, 32, 1), pltpu.roll(r, 96, 1)) for r in res]
            elif e == 3:
                res = [jnp.where(bit0_8, pltpu.roll(r, 96, 1), pltpu.roll(r, 32, 1)) for r in res]
            pv_outs[(g, e)] = res
            last_pv[0] = rl
            if (g, e ^ 1) in pv_outs:
                p = e // 2
                a, b = pv_outs.pop((g, 2 * p)), pv_outs.pop((g, 2 * p + 1))
                ot_ref[80 * g + 40 * p:80 * g + 40 * p + 40, :] = jnp.concatenate(
                    [a[0], a[1], jnp.where(sub4, a[2], b[0]), b[1], b[2]], 0)

    def fin_tile(t, slot):
        ob32[slot, :, 128 * t:128 * t + 128] = _zip16(ot_ref[128 * t:128 * t + 128, :].T)

    def ob_slot(i):
        return (0 if i in (0, 2) else (2 if i == 1 else 1)) if isinstance(i, int) else 1

    def finish(i):
        def f():
            pv_group(7, i)
            fin_tile(4, ob_slot(i))
        return f

    last_m = {}

    def token(n):
        kind = CFG.get("tok", {"0": "m", "1": "m", "2": "m", "3": "m"}).get(str(n))
        if kind == "m":
            g, u = max(last_m)
            return jnp.broadcast_to(last_m[(g, u)], (8, 128))
        if kind == "p":
            return last_pv[0]
        return None

    def attn(i, plan, head=None, qsrc=None, lazy=False):
        qsrc = qw_ref if qsrc is None else qsrc
        static = isinstance(i, int)
        lov = (lambda u: max(0, 8 - u - 4 * i)) if static else (lambda u: 0)
        tiles = key_tiles(i)
        ms = last_m

        def phase_a(g, us):
            sl = g % NSS
            _, _, off = _gwin(g)
            hm = [jnp.where((lane16 >= off + 20 * e) & (lane16 < off + 20 * e + 20), jnp.int32(-1), jnp.int32(0))
                  for e in range(4)]
            for u in us:
                lo = lov(u)
                nrow = 32 * (9 - lo)
                k0 = 64 * i - 128 + 16 * u + 16 * lo
                if not static:
                    k0 = pl.multiple_of(k0, 16)
                kw = _b16(kw_refs[g][pl.ds(k0, nrow // 2), :])
                qu = qsrc[g, 16 * u:16 * u + 16, :]
                qm = _b16(jnp.concatenate([qu & hm[lam ^ u] for lam in range(4)], 0))
                s = _dot_nt(kw, qm)
                sd = s[nrow - 32:nrow]
                if lo == 0:
                    T = jnp.where(le32, sd, s[0:32])
                    F = s[32:256]
                else:
                    T = jnp.where(le32, sd, NEG)
                    F = s[0:nrow - 32]
                m = jnp.max(T, axis=0, keepdims=True)
                s_ref[sl, u, 0:32] = T
                if F.shape[0] > 0:
                    m = jnp.maximum(m, jnp.max(F, axis=0, keepdims=True))
                    s_ref[sl, u, 32:32 + F.shape[0]] = F
                ms[(g, u)] = m

        def sel(m, a, b):
            if a is None and b is None:
                return None
            if a is None:
                a = jnp.zeros((16, 128), i32)
            if b is None:
                b = jnp.zeros((16, 128), i32)
            return jnp.where(m, a, b)

        def phase_b1(g):
            sl = g % NSS
            slp = g % NSP
            lo_ = [lov(u) for u in range(4)]
            nf = [7 if lo_[u] == 0 else 8 - lo_[u] for u in range(4)]

            def pblock(u, row0):
                p = jnp.exp2(s_ref[sl, u, row0:row0 + 32] - ms[(g, u)])
                return jnp.concatenate([_packi(p[16 * j:16 * j + 8], p[16 * j + 8:16 * j + 16]) for j in range(2)], 0)

            tri = {}

            def block(u, rel):
                if rel < 0 or rel > 8:
                    return None
                if rel == 0 or rel == 8:
                    if u not in tri:
                        pt = pblock(u, 0)
                        if lo_[u] == 0:
                            p8 = pt & le_pk
                            tri[u] = {8: p8, 0: pt ^ p8}
                        else:
                            tri[u] = {8: pt, 0: None}
                    return tri[u][rel]
                first = 8 - nf[u]
                if rel < first:
                    return None
                return pblock(u, 32 + 32 * (rel - first))

            for beta in range(4 * tiles[0], 12):
                src = [block(u, beta - u) for u in range(4)]
                a0 = sel(bit0, src[1], src[0])
                a1 = sel(bit0, src[0], src[1])
                c0 = sel(bit0, src[3], src[2])
                c1 = sel(bit0, src[2], src[3])
                o4 = [sel(bit1, c0, a0), sel(bit1, c1, a1), sel(bit1, a0, c0), sel(bit1, a1, c1)]
                for e in range(4):
                    p_ref[slp, e, 16 * beta:16 * beta + 16, :] = (
                        o4[e] if o4[e] is not None else jnp.zeros((16, 128), i32))

        okey = "order" if not static else ("order_pre" if i in (2, 3) else ("order_post" if i == NB - 1 else "order_01"))
        order = CFG.get(okey, {"order": "B P0 A0 A1 A2 A3 P1 P2 P3 X X Y",
                               "order_pre": "B A0 A1 P0 A2 P1 A3 X P2 X P3 Y",
                               "order_post": "B A0 A1 A2 P0 P1 P2 A3 P3 X X Y",
                               "order_01": "B P0 P1 A0 A1 A2 A3 P2 P3 X X Y"}[okey])

        def step(s):
            if s == -1 and head is not None:
                head()
            px = plan.get(s, [])
            todo = list(range(len(px)))
            for tok in order.split():
                if tok[0] == "A" and 0 <= s + 1 < 8:
                    phase_a(s + 1, [int(c) for c in tok[1:]])
                if tok[0] == "B" and 0 <= s < 8:
                    phase_b1(s)
                if tok[0] == "P" and 0 <= s - 1 < 8:
                    pv_group(s - 1, i, [int(c) for c in tok[1:]])
                if tok[0] == "X" and todo:
                    px[todo.pop(0)]()
                if tok[0] == "Y":
                    while todo:
                        px[todo.pop(0)]()
            while todo:
                px[todo.pop(0)]()
            if s == 7:
                for t in range(4):
                    fin_tile(t, ob_slot(i))

        steps = [(lambda s=s: step(s)) for s in range(-1, 8)]
        if lazy:
            return steps
        for f in steps:
            f()

    def a1_step(ax, ay, order):
        w = {}
        if ax is not None:
            j, par = ax // 2, ax % 2
            x = [_unpacki(xa32[t, pl.ds(j, 128, stride=8), :], par) for t in range(5)]
            t1 = x[1] + x[4]
            t2 = x[2] + x[3]
            t3 = x[1] - x[4]
            t4 = x[2] - x[3]
            p1 = x[0] + C1 * t1 + C2 * t2
            p2 = x[0] + C2 * t1 + C1 * t2
            q1 = S1 * t3 + S2 * t4
            q2 = S2 * t3 - S1 * t4
            ops = [x[0] + t1 + t2, p1 + q1, q1, p1, p2 + q2, q2, p2]
            w0s = [0, 80, 144, 208, 272, 336, 400, 464]
        for tok in order:
            if tok[0] == "x" and ax is not None:
                n = int(tok[1])
                w[tok] = _dot_nt(_b16(ff32[w0s[n]:w0s[n + 1]]), ops[n].astype(bf))
            if tok[0] == "y" and ay is not None:
                n = int(tok[1])
                w[tok] = _dot(ys_ref[ay % 2, n], _b16(rr32[ay, n]))
        if ay is not None:
            g_ = jnp.concatenate([w["y0"] - w["y1"], w["y0"] - w["y2"]], 1)
            for g in range(R // 8):
                gs_refs[g % 4][ay, 8 * (g // 4):8 * (g // 4) + 8, :] = g_[8 * g:8 * g + 8]
        if ax is not None:
            re, im = [w["x0"][0:80]], [w["x0"][80:160]]
            for n in (1, 4):
                t1, t2, t3 = w["x%d" % n], w["x%d" % (n + 1)], w["x%d" % (n + 2)]
                re.append(t1 - t2)
                im += [t3[0:64] - t1[0:64], t1[64:128] - t3[64:128]]
            yr = jnp.concatenate(re, 0)
            yi = jnp.concatenate(im, 0)
            ys_ref[ax % 2, 0] = (yr + yi).astype(bf)
            ys_ref[ax % 2, 1] = yi.astype(bf)
            ys_ref[ax % 2, 2] = yr.astype(bf)

    def a2_group(n, gq, token=None):
        g = 4 * gq + n
        special = isinstance(gq, int) and g == 8
        if isinstance(gq, int):
            w8 = g if g < 8 else (g - 10) % 8
            c10 = [0, 1, 4, 2, 3][0 if g < 8 else (g - 10) // 8 + 1] + 5 * (w8 // 4)
            r0 = 8 * gq
        else:
            w8 = jnp.where(g < 8, g, (g - 10) & 7)
            blk = jnp.minimum(jnp.where(g < 10, 0, ((g - 10) >> 3) + 1), 4)
            c10 = jnp.where(blk == 2, 4, jnp.where(blk > 2, blk - 1, blk)) + 5 * (w8 >> 2)
            r0 = 8 * gq
            if n == 0:
                r0 = jnp.where(g == 8, 96, r0)
            r0 = pl.multiple_of(r0, 8)
        w0 = (c10 >> 1) + 40 * (w8 & 3)
        sh = 16 * (1 - (c10 & 1))

        def wload(ref, last, f1):
            if special:
                return jnp.broadcast_to(last[0:1, 128 * f1:128 * f1 + 128].astype(f32), (8, 128))
            return pltpu.bitcast((ref[f1, pl.ds(w0, 8, stride=5), :] << sh) & jnp.int32(-65536), f32)

        gref = gs_refs[n]
        if token is not None:
            gref[16, pl.ds(pl.multiple_of(8 * (gq & 15), 8), 8), 0:128] = token
        z = [(gref[a, pl.ds(r0, 8), 0:128], gref[a, pl.ds(r0, 8), 128:256]) for a in range(16)]
        X = _fft16(z, False)
        V = []
        for f1 in range(16):
            wr = wload(wr32, wr_last, f1)
            wi = wload(wi32, wi_last, f1)
            V.append((X[f1][0] * wr - X[f1][1] * wi, X[f1][0] * wi + X[f1][1] * wr))
        U = _fft16(V, True)
        for a in range(16):
            gref[a, pl.ds(r0, 8), 0:128] = U[a][0]
            gref[a, pl.ds(r0, 8), 128:256] = U[a][1]

    def a3_step(az, ad, order, extra=()):
        w = {}
        if az is not None:
            u = jnp.concatenate([gs_refs[g % 4][az, 8 * (g // 4):8 * (g // 4) + 8, :] for g in range(R // 8)], 0)
            ur = u[:, 0:128]
            ui = u[:, 128:256]
            zops = [(ur + ui, 0), (ui, 2), (ur, 1)]
        for tok in order:
            if tok[0] == "z" and az is not None:
                v, n = zops[int(tok[1])]
                w[tok] = _dot_nt(v.astype(bf), _b16(rr32[az, n]))
            if tok[0] == "d" and ad is not None:
                n = int(tok[1])
                w[tok] = _dot(zs_ref[ad % 2, n], _b16(gg32[64 * n:64 * n + 64]))
            if tok == "E":
                for f in extra:
                    f()
        if ad is not None:
            v0 = w["d0"]
            v1r, v1i = w["d1"] - w["d2"], w["d1"] + w["d3"]
            v2r, v2i = w["d4"] - w["d5"], w["d4"] + w["d6"]
            A1 = v0 + C1 * v1r + C2 * v2r
            A2 = v0 + C2 * v1r + C1 * v2r
            B1 = S1 * v1i + S2 * v2i
            B2 = S2 * v1i - S1 * v2i
            y = [v0 + v1r + v2r, A1 - B1, A2 - B2, A2 + B2, A1 + B1]
            for t in range(5):
                if ad % 2 == 0:
                    ysc_ref[t] = y[t]
                else:
                    oa32[t, pl.ds(ad // 2, 128, stride=8), :] = _packi(ysc_ref[t], y[t])
        if az is not None:
            zr = w["z0"] - w["z1"]
            zi = w["z0"] - w["z2"]
            kop = [jnp.concatenate([zr[0:64], jnp.where(sub0, zr[64:72], zi[0:8]), zi[8:64]], 0)]
            for r0 in (80, 208):
                kop += [jnp.concatenate([zr[r0:r0 + 64] + zi[r0:r0 + 64], zr[r0 + 64:r0 + 128] - zi[r0 + 64:r0 + 128]], 0),
                        zi[r0:r0 + 128], zr[r0:r0 + 128]]
            for n in range(7):
                zs_ref[az % 2, n] = kop[n].T.astype(bf)

    def run(pieces, order=None):
        for k in (order or list(pieces)):
            if k in pieces:
                pieces[k]()

    PLAN = {-1: ["v0", "v1"], 0: ["q0", "k0"], 1: ["k1", "q1", "a3"], 2: ["k2", "q2"], 3: ["o0", "o1", "a1"],
            4: ["k3", "q3"], 5: ["o2", "o3", "a0"], 6: ["v2", "o4", "a2"], 7: ["k4", "q4", "v3", "v4"]}

    if 'plan' in CFG:
        PLAN = {int(k): v for k, v in CFG['plan'].items()}

    def mkplan(pieces):
        return {s_: [pieces[k] for k in ks if k in pieces] for s_, ks in PLAN.items()}

    ORD = ["v0", "v1", "v2", "v3", "v4", "k0", "k1", "k2", "k3", "k4", "q0", "q1", "q2", "q3", "q4"]

    def out_b_copy(i):
        return pltpu.make_async_copy(obo32.at[pl.ds(wrows_of(i), 64)],
                                     oh32.at[pl.ds(wrows_of(i), 64), pl.ds(D, D)], osem.at[0])

    for g in range(R // 8, 44):
        gs_refs[g % 4][0:16, 8 * (g // 4):8 * (g // 4) + 8, :] = jnp.zeros((16, 8, 256), f32)
    gs_refs[0][0:16, 96:104, :] = jnp.zeros((16, 8, 256), f32)
    c_x0.wait()
    c_wk.wait()
    prep_x(0)
    P0 = proj_pieces(0, do_q=False)
    run(P0, ["k0", "k1", "k2", "k3", "k4"])
    prep_x(1)
    P1 = proj_pieces(1, do_q=False)
    run(P1, ["k0", "k1", "k2", "k3", "k4"])
    c_wv.wait()
    prep_wvt()
    run(P0, ["v0", "v1", "v2", "v3", "v4"])
    run(P1, ["v0", "v1", "v2", "v3", "v4"])
    c_x1.wait()
    c_wq.wait()
    prep_x(2)
    run(proj_pieces(2), ORD)
    prep_x(3)
    attn(2, mkplan(proj_pieces(3)))
    prep_x(4)
    attn(3, mkplan(proj_pieces(4)), head=finish(2))
    for i_ in range(2):
        prep_x(i_)
        run(proj_pieces(i_, do_kv=False, qdst=qw01_ref.at[i_]), ORD)

    for cp in [c_wo, c_ff] + c_xa + [c_rr]:
        cp.wait()
    P2 = out_pieces(2, slot=0)
    run(P2, ["o0", "o1", "o2"])
    a1o = CFG.get("a1", "x0 x1 x2 x3 y0 x4 y1 x5 y2 x6").split()
    a1_step(0, None, a1o)
    run(P2, ["o3", "o4"])
    for a in range(16):
        a1_step(a + 1 if a < 15 else None, a, a1o)
    for cp in c_w:
        cp.wait()
    c_x2.wait()
    c_gg.wait()

    def one_block(i):
        nxt = jnp.minimum(i + 1, NB - 1)
        prep_x(nxt)
        P = proj_pieces(nxt)
        P.update(out_pieces(i - 1))
        for n in range(4):
            P["a%d" % n] = (lambda n=n: a2_group(n, i - 4, token(n)))
        last_m.clear()
        attn(i, mkplan(P), head=finish(i - 1))

    UNR = CFG.get("unroll", 1)

    def body(it, carry):
        for u_ in range(UNR):
            i = 4 + UNR * it + u_
            one_block(i)
            out_b_copy(i - 1).start()
        return carry

    out_b_copy(2).start()
    lax.fori_loop(0, NB - 5, body, 0)

    finish(NB - 2)()
    a2_group(0, 2)

    extra = attn(0, {}, qsrc=qw01_ref.at[0], lazy=True) + attn(1, {}, head=finish(0), qsrc=qw01_ref.at[1], lazy=True)
    extra += [lambda: pv_group(7, 1), lambda: fin_tile(4, 2)]
    a3o = CFG.get("a3", "z0 E z1 z2 d0 d1 d2 d3 d4 d5 d6").split()
    a3_step(0, None, a3o)
    for a in range(16):
        cut = CFG.get("cut", [0, 1, 2, 2, 5, 5, 7, 8, 10, 11, 12, 13, 15, 16, 18, 18, 20])
        a3_step(a + 1 if a < 15 else None, a, a3o, extra[cut[a]:cut[a + 1]])
    c_oa = [pltpu.make_async_copy(oa32.at[t], oh32.at[:, pl.ds(128 * t, 128)], osem.at[1 + t]) for t in range(5)]
    for cp in c_oa:
        cp.start()
    c_pin.wait()

    fill = []
    for t in range(5):
        fill += [out_pieces(0, slot=0)["o%d" % t], out_pieces(1, slot=2)["o%d" % t], out_pieces(NB - 2)["o%d" % t]]
    last_m.clear()
    fc = CFG.get("fc", [0, 2, 4, 4, 6, 8, 10, 11, 13, 15])
    attn(NB - 1, {s_: fill[fc[s_ + 1]:fc[s_ + 2]] for s_ in range(-1, 8)})
    for i_ in (0, 1, NB - 2):
        out_b_copy(i_).start()
    c_pin2.wait()
    finish(NB - 1)()
    run(out_pieces(NB - 1))
    out_b_copy(NB - 1).start()

    for cp in c_oa:
        cp.wait()
    for i in range(NB):
        out_b_copy(i).wait()


def _build(FF32, GG32, RR32):
    scratch = [
        pltpu.VMEM((5, S // 2, 128), i32),
        pltpu.VMEM((NB, 160, 128), i32), pltpu.VMEM((NB, 160, 128), i32),
        pltpu.VMEM((1, S), bf), pltpu.VMEM((1, S), bf),
        pltpu.VMEM(FF32.shape, i32), pltpu.VMEM(GG32.shape, i32), pltpu.VMEM(RR32.shape, i32),
        pltpu.VMEM((2, 3, R, 128), bf),
        pltpu.VMEM((2, 7, 128, 128), bf),
        pltpu.VMEM((5, 128, 128), f32),
        pltpu.VMEM((5, S // 2, 128), i32),
        pltpu.VMEM((2, 8, 128), i32),
        pltpu.VMEM((2, 8, 64, 128), i32),
        pltpu.VMEM((S // 2, D), i32),
        pltpu.VMEM((D // 2, 3 * D), i32),
        pltpu.VMEM((D // 2, D), i32),
        pltpu.VMEM((D // 2, D), i32),
        pltpu.VMEM((CFG.get('ss', 1), 4, 256, 128), f32),
        pltpu.VMEM((CFG.get('sp', 2), 4, 192, 128), i32),
        pltpu.VMEM((3, 64, D), i32),
        pltpu.VMEM((D, 128), f32),
        pltpu.VMEM((8, 64, 128), i32),
        pltpu.VMEM((2, 64, D), i32),
        pltpu.VMEM((S // 2, D), i32),
        pltpu.SemaphoreType.DMA((25,)),
        pltpu.SemaphoreType.DMA((6,)),
        pltpu.SemaphoreType.DMA((1,)),
    ]
    scratch += [pltpu.VMEM((17, 104, 256), f32)] * 4
    scratch += [pltpu.VMEM((S // 2, 128), i32)] * 8
    scratch += [pltpu.VMEM((4, NB, 32, 128), bf)] * 8
    return pl.pallas_call(
        _kernel,
        out_shape=jax.ShapeDtypeStruct((S, 2 * D), bf),
        in_specs=[pl.BlockSpec(memory_space=pl.ANY)] * 9,
        out_specs=pl.BlockSpec(memory_space=pl.ANY),
        scratch_shapes=scratch,
        compiler_params=pltpu.CompilerParams(vmem_limit_bytes=110 * 2 ** 20),
    )


@jax.jit
def pallas_concat_heads__spectral_gfnet__sliding_block__prompt_kernel(
    A_x: jax.Array,
    A_w_r: jax.Array,
    A_w_i: jax.Array,
    B_x: jax.Array,
    B_wqkv: jax.Array,
    B_wo: jax.Array,
):
    FF32, GG32, RR32 = _make_consts()
    out = _build(FF32, GG32, RR32)(
        A_x.reshape(S, D), A_w_r.T, A_w_i.T, B_x.reshape(S, D), B_wqkv, B_wo,
        jnp.asarray(FF32), jnp.asarray(GG32), jnp.asarray(RR32))
    return out.reshape(1, S, 2 * D)
```

```python
import numpy as np
import ml_dtypes
import jax
import jax.numpy as jnp
from jax import lax
import jax.experimental.pallas as pl
import jax.experimental.pallas.tpu as pltpu

S = 2048
D = 640
DF = 321
H = 32
DH = 20
NB = S // 128
R = 336
NEG = -1e30
CFG = {}
f32 = jnp.float32
bf = jnp.bfloat16
i32 = jnp.int32

C1 = float(np.cos(2 * np.pi / 5))
C2 = float(np.cos(4 * np.pi / 5))
S1 = float(np.sin(2 * np.pi / 5))
S2 = float(np.sin(4 * np.pi / 5))


def _pack_rows(a):
    u = np.ascontiguousarray(a.astype(ml_dtypes.bfloat16)).view(np.uint16).astype(np.uint32)
    return (u[..., 0::2, :] | (u[..., 1::2, :] << 16)).astype(np.uint32).view(np.int32)


def _make_consts():
    b5 = np.arange(128)

    def cs(k):
        th = 2 * np.pi * np.outer(k, b5) / D
        return np.cos(th), np.sin(th)

    m32 = np.arange(32)
    k0 = np.concatenate([10 * m32, 5 + 10 * m32, [320]])
    c, s = cs(k0)
    F0 = np.zeros((160, 128))
    F0[0:65] = c
    F0[80:145] = -s

    def kpair(j):
        return (np.concatenate([j + 10 * m32, j + 5 + 10 * m32]),
                np.concatenate([5 - j + 10 * m32, 10 - j + 10 * m32]))

    def fwd(j):
        ka, kb = kpair(j)
        (ca, sa), (cb, sb) = cs(ka), cs(kb)
        return np.concatenate([ca, cb, ca + sa, cb - sb, ca - sa, cb + sb], 0)

    FF = np.concatenate([F0, fwd(1), fwd(2)], 0)

    b = np.arange(128)
    f2 = np.arange(128)
    RR = np.zeros((16, 3, 128, 128))
    for a in range(16):
        th = -2 * np.pi * (np.outer(b, f2) / 128.0 + a * f2[None, :] / float(S))
        Mr, Mi = np.cos(th), np.sin(th)
        RR[a, 0] = Mr
        RR[a, 1] = Mr + Mi
        RR[a, 2] = Mr - Mi

    sc = 1.0 / (S * D)
    G0 = np.zeros((128, 128))
    al = np.full(65, 2.0)
    al[0] = 1.0
    al[64] = 1.0
    G0[:, 0:64] = (al[0:64, None] * c[0:64]).T
    G0[:, 64:128] = (-al[0:64, None] * s[0:64]).T
    G0[:, 64] = al[64] * c[64]

    def inv(j):
        ka, kb = kpair(j)
        (ca, sa), (cb, sb) = cs(ka), cs(kb)
        return 2 * np.concatenate([np.concatenate([ca, cb], 0).T,
                                   np.concatenate([ca + sa, sb - cb], 0).T,
                                   np.concatenate([sa - ca, -sb - cb], 0).T], 0)

    GG = np.concatenate([G0, inv(1), inv(2)], 0) * sc
    GG = GG.reshape(7, 128, 128).transpose(0, 2, 1).reshape(896, 128)
    return _pack_rows(FF), _pack_rows(GG), _pack_rows(RR)


_NT = (((1,), (1,)), ((), ()))


def _dot(a, b):
    return jnp.dot(a, b, preferred_element_type=f32)


def _dot_nt(a, b):
    return lax.dot_general(a, b, _NT, preferred_element_type=f32)


def _b16(x):
    return pltpu.bitcast(x, bf)


def _packi(a, b):
    return pltpu.pack_elementwise([a, b], packed_dtype=bf)


def _unpacki(x, idx):
    return pltpu.unpack_elementwise(x, index=idx, packed_dtype=bf, unpacked_dtype=f32)


def _zip16(x):
    n = x.shape[0] // 16
    return jnp.concatenate([_packi(x[16 * j:16 * j + 8], x[16 * j + 8:16 * j + 16]) for j in range(n)], 0)


def _dft4(z, inv):
    (a, b, c, d) = z
    t0 = (a[0] + c[0], a[1] + c[1])
    t1 = (a[0] - c[0], a[1] - c[1])
    t2 = (b[0] + d[0], b[1] + d[1])
    t3 = (b[0] - d[0], b[1] - d[1])
    o0 = (t0[0] + t2[0], t0[1] + t2[1])
    o2 = (t0[0] - t2[0], t0[1] - t2[1])
    p = (t1[0] + t3[1], t1[1] - t3[0])
    q = (t1[0] - t3[1], t1[1] + t3[0])
    return [o0, q, o2, p] if inv else [o0, p, o2, q]


def _tw16(z, e, inv):
    if e == 0:
        return z
    zr, zi = z
    if e == 4:
        return (-zi, zr) if inv else (zi, -zr)
    h = float(np.sqrt(0.5))
    if e == 2:
        return ((zr - zi) * h, (zr + zi) * h) if inv else ((zr + zi) * h, (zi - zr) * h)
    if e == 6:
        return ((-zr - zi) * h, (zr - zi) * h) if inv else ((zi - zr) * h, (-zr - zi) * h)
    sgn = 1.0 if inv else -1.0
    c = float(np.cos(2 * np.pi * e / 16))
    s = float(sgn * np.sin(2 * np.pi * e / 16))
    return (zr * c - zi * s, zr * s + zi * c)


def _fft16(z, inv):
    hh = [_dft4([z[a0 + 4 * a1] for a1 in range(4)], inv) for a0 in range(4)]
    out = [None] * 16
    for fa in range(4):
        o = _dft4([_tw16(hh[a0][fa], a0 * fa, inv) for a0 in range(4)], inv)
        for fb in range(4):
            out[fa + 4 * fb] = o[fb]
    return out


def _gwin(g):
    lo, hi = 80 * g, 80 * g + 79
    if lo // 128 == hi // 128:
        return ("nat", lo // 128, lo - 128 * (lo // 128))
    t = (lo - 64) // 128
    return ("shf", t, lo - 64 - 128 * t)


def _kernel(xa_hbm, wr_hbm, wi_hbm, xb_hbm, wqkv_hbm, wo_hbm, ff_hbm, gg_hbm, rr_hbm, out_hbm,
            xa32, wr32, wi32, wr_last, wi_last, ff32, gg32, rr32, ys_ref, zs_ref, ysc_ref, oa32,
            pin_ref, qw01_ref, xq_ref, xb32, wqkv32, wo32, wvt32, s_ref, p_ref, ob32, ot_ref, qw_ref, xz_ref, obo32,
            sem, osem, wsem, *groups):
    gs_refs = groups[0:4]
    kw_refs = groups[4:12]
    vt_refs = groups[12:20]

    def copy(src, dst, k):
        return pltpu.make_async_copy(src, dst, sem.at[k])

    xbh = xb_hbm.bitcast(i32)
    wqh = wqkv_hbm.bitcast(i32)
    xah = xa_hbm.bitcast(i32)
    oh32 = out_hbm.bitcast(i32)
    c_x0 = copy(xbh.at[pl.ds(0, 128)], xb32.at[pl.ds(0, 128)], 0)
    c_wk = copy(wqh.at[:, pl.ds(640, 640)], wqkv32.at[:, pl.ds(640, 640)], 1)
    c_wv = copy(wqh.at[:, pl.ds(1280, 640)], wqkv32.at[:, pl.ds(1280, 640)], 2)
    c_x1 = copy(xbh.at[pl.ds(128, 192)], xb32.at[pl.ds(128, 192)], 3)
    c_wq = copy(wqh.at[:, pl.ds(0, 640)], wqkv32.at[:, pl.ds(0, 640)], 4)
    c_ff = copy(ff_hbm, ff32, 5)
    c_xa = [copy(xah.at[:, pl.ds(128 * t, 128)], xa32.at[t], 6 + t) for t in range(5)]
    c_rr = copy(rr_hbm, rr32, 11)
    c_w = []
    for n, (src, dst, dst1) in enumerate(((wr_hbm, wr32, wr_last), (wi_hbm, wi32, wi_last))):
        w320 = src.at[pl.ds(0, 320)].bitcast(i32)
        for t in range(NB):
            c_w.append(pltpu.make_async_copy(w320.at[:, pl.ds(128 * t, 128)], dst.at[t], wsem.at[0]))
        c_w.append(copy(src.at[pl.ds(320, 1)], dst1, 13 + n))
    c_x2 = copy(xbh.at[pl.ds(320, 704)], xb32.at[pl.ds(320, 704)], 21)
    c_wo = copy(wo_hbm.bitcast(i32), wo32, 22)
    c_gg = copy(gg_hbm, gg32, 23)
    c_pin = copy(xbh.at[pl.ds(0, 8), pl.ds(0, 128)], pin_ref.at[0], 24)
    c_pin2 = copy(xbh.at[pl.ds(0, 8), pl.ds(0, 128)], pin_ref.at[1], 12)
    for cp in ([c_x0, c_wk, c_wv, c_x1, c_wq, c_ff] + c_xa + [c_rr]
               + c_w + [c_x2, c_wo, c_gg, c_pin, c_pin2]):
        cp.start()

    scale = float(DH ** -0.5 * np.log2(np.e))
    def _qpos(l):
        return (l & 16) + 4 * (l & 3) + ((l & 15) >> 2)
    rr_ = lax.broadcasted_iota(i32, (32, 128), 0)
    ll_ = _qpos(lax.broadcasted_iota(i32, (32, 128), 1))
    pos_ = rr_ & 15
    key_ = (rr_ & 16) + jnp.where(pos_ < 8, 2 * pos_, 2 * (pos_ - 8) + 1)
    le32 = key_ <= ll_
    wr_ = lax.broadcasted_iota(i32, (16, 128), 0)
    wq_ = _qpos(lax.broadcasted_iota(i32, (16, 128), 1))
    le_pk = (jnp.where(2 * wr_ <= wq_, jnp.int32(0xFFFF), jnp.int32(0))
             | jnp.where(2 * wr_ + 1 <= wq_, jnp.int32(-65536), jnp.int32(0)))
    lane8 = lax.broadcasted_iota(i32, (8, 128), 1)
    lane16 = lax.broadcasted_iota(i32, (16, 128), 1)
    bit0 = (lane16 & 32) != 0
    bit1 = (lane16 & 64) != 0
    bit0_8 = (lane8 & 32) != 0
    sub4 = lax.broadcasted_iota(i32, (8, 128), 0) < 4
    sub0 = lax.broadcasted_iota(i32, (8, 128), 0) == 0
    ones8 = jnp.ones((8, 128), f32)
    lo64 = lax.broadcasted_iota(i32, (64, 128), 1) < 64

    def rows_of(i):
        return i * 128 if isinstance(i, int) else pl.multiple_of(i * 128, 128)

    def wrows_of(i):
        return i * 64 if isinstance(i, int) else pl.multiple_of(i * 64, 64)

    def prep_wvt():
        for tr in range(5):
            wvt32[64 * tr:64 * tr + 64, :] = pltpu.bitcast(
                _b16(wqkv32[:, 1280 + tr * 128:1280 + (tr + 1) * 128]).T, i32)

    def prep_x(i):
        w = xb32[pl.ds(wrows_of(i), 64), :]
        z1 = _zip16(_b16(w).astype(f32))
        xz_ref[0] = z1
        xz_ref[1] = _zip16(_b16(z1).astype(f32))

    def win_ready(tiles, rolled, done, emit):
        for g in range(8):
            if g in done:
                continue
            kind, t, _ = _gwin(g)
            if kind == "nat":
                if t in tiles:
                    emit(g, tiles[t])
                    done.add(g)
            elif t in tiles and (t + 1) in tiles:
                for tt in (t, t + 1):
                    if tt not in rolled:
                        rolled[tt] = pltpu.roll(tiles[tt], 64, 1)
                emit(g, jnp.where(lo64, rolled[t], rolled[t + 1]))
                done.add(g)

    def proj_pieces(i, do_q=True, do_kv=True, qdst=None, xz=None):
        qdst = qw_ref if qdst is None else qdst
        xz = xz_ref.at[0] if xz is None else xz
        pieces = {}
        if do_kv:
            v8 = {}
            vdone = set()

            def vpiece(r):
                def f():
                    xb = _b16(xb32[pl.ds(wrows_of(i), 64), :])
                    vt = _dot_nt(_b16(wvt32[64 * r:64 * r + 64, :]), xb)
                    for j in range(16):
                        v8[16 * r + j] = vt[8 * j:8 * j + 8]
                    for p in range(16):
                        if p in vdone or any((5 * p + j) not in v8 for j in range(5)):
                            continue
                        v = [v8[5 * p + j] for j in range(5)]
                        h0, h1 = 2 * p, 2 * p + 1
                        vt_refs[h0 // 4][h0 % 4, i] = jnp.concatenate([v[0], v[1], v[2], ones8], 0).astype(bf)
                        vt_refs[h1 // 4][h1 % 4, i] = jnp.concatenate([v[2], v[3], v[4], ones8], 0).astype(bf)
                        vdone.add(p)
                return f

            kt, kr, kd = {}, {}, set()

            def kpiece(t):
                def f():
                    kt[t] = _zip16(_dot(_b16(xz_ref[1]), _b16(wqkv32[:, 640 + 128 * t:640 + 128 * t + 128])))

                    def emit(g, val):
                        kw_refs[g][pl.ds(wrows_of(i), 64), :] = val
                    win_ready(kt, kr, kd, emit)
                return f

            for r in range(5):
                pieces["v%d" % r] = vpiece(r)
                pieces["k%d" % r] = kpiece(r)
        if do_q:
            qt, qr, qd = {}, {}, set()

            def qpiece(t):
                def f():
                    qt[t] = _zip16(_dot(_b16(xz[...]), _b16(wqkv32[:, 128 * t:128 * t + 128])) * scale)

                    def emit(g, val):
                        qdst[g] = val
                    win_ready(qt, qr, qd, emit)
                return f

            for t in range(5):
                pieces["q%d" % t] = qpiece(t)
        return pieces

    def out_pieces(i, slot=1):
        def opiece(t):
            def f():
                res = _dot(_b16(ob32[slot]), _b16(wo32[:, 128 * t:128 * t + 128]))
                obo32[pl.ds(wrows_of(i), 64), 128 * t:128 * t + 128] = _zip16(res)
            return f
        return {"o%d" % t: opiece(t) for t in range(5)}

    NSS = CFG.get('ss', 1)
    NSP = CFG.get('sp', 2)

    def key_tiles(i):
        return list(range(3)) if (not isinstance(i, int) or i >= 2) else list(range(2 - i, 3))

    pv_outs = {}
    last_pv = [None]

    def pv_group(g, i, es=(0, 1, 2, 3)):
        tiles = key_tiles(i)
        sl = g % NSP
        for e in es:
            P = _b16(p_ref[sl, e, 64 * tiles[0]:192, :])
            if len(tiles) > 1:
                vw = jnp.concatenate([vt_refs[g][e, i - 2 + j] for j in tiles], 1)
            else:
                vw = vt_refs[g][e, i]
            o = _dot(vw, P)
            rl = pltpu.reciprocal(o[24:32])
            res = [o[0:8] * rl, o[8:16] * rl, o[16:24] * rl]
            if e == 2:
                res = [pltpu.roll(r, 64, 1) for r in res]
            elif e == 1:
                res = [jnp.where(bit0_8, pltpu.roll(r, 32, 1), pltpu.roll(r, 96, 1)) for r in res]
            elif e == 3:
                res = [jnp.where(bit0_8, pltpu.roll(r, 96, 1), pltpu.roll(r, 32, 1)) for r in res]
            pv_outs[(g, e)] = res
            last_pv[0] = rl
            if (g, e ^ 1) in pv_outs:
                p = e // 2
                a, b = pv_outs.pop((g, 2 * p)), pv_outs.pop((g, 2 * p + 1))
                ot_ref[80 * g + 40 * p:80 * g + 40 * p + 40, :] = jnp.concatenate(
                    [a[0], a[1], jnp.where(sub4, a[2], b[0]), b[1], b[2]], 0)

    def fin_tile(t, slot):
        ob32[slot, :, 128 * t:128 * t + 128] = _zip16(ot_ref[128 * t:128 * t + 128, :].T)

    def ob_slot(i):
        return {0: 0, 1: 2, 2: 3}.get(i, 1) if isinstance(i, int) else 1

    def finish(i):
        def f():
            pv_group(7, i)
            fin_tile(4, ob_slot(i))
        return f

    last_m = {}

    def token(n):
        kind = CFG.get("tok", {"0": "m", "1": "m", "2": "m", "3": "m"}).get(str(n))
        if kind == "m":
            g, u = max(last_m)
            return jnp.broadcast_to(last_m[(g, u)], (8, 128))
        if kind == "p":
            return last_pv[0]
        return None

    def attn(i, plan, head=None, qsrc=None, lazy=False):
        qsrc = qw_ref if qsrc is None else qsrc
        static = isinstance(i, int)
        lov = (lambda u: max(0, 8 - u - 4 * i)) if static else (lambda u: 0)
        tiles = key_tiles(i)
        ms = last_m

        def phase_a(g, us):
            sl = g % NSS
            _, _, off = _gwin(g)
            hm = [jnp.where((lane16 >= off + 20 * e) & (lane16 < off + 20 * e + 20), jnp.int32(-1), jnp.int32(0))
                  for e in range(4)]
            for u in us:
                lo = lov(u)
                nrow = 32 * (9 - lo)
                k0 = 64 * i - 128 + 16 * u + 16 * lo
                if not static:
                    k0 = pl.multiple_of(k0, 16)
                kw = _b16(kw_refs[g][pl.ds(k0, nrow // 2), :])
                qu = qsrc[g, 16 * u:16 * u + 16, :]
                qm = _b16(jnp.concatenate([qu & hm[lam ^ u] for lam in range(4)], 0))
                s = _dot_nt(kw, qm)
                sd = s[nrow - 32:nrow]
                if lo == 0:
                    T = jnp.where(le32, sd, s[0:32])
                    F = s[32:256]
                else:
                    T = jnp.where(le32, sd, NEG)
                    F = s[0:nrow - 32]
                m = jnp.max(T, axis=0, keepdims=True)
                s_ref[sl, u, 0:32] = T
                if F.shape[0] > 0:
                    m = jnp.maximum(m, jnp.max(F, axis=0, keepdims=True))
                    s_ref[sl, u, 32:32 + F.shape[0]] = F
                ms[(g, u)] = m

        def sel(m, a, b):
            if a is None and b is None:
                return None
            if a is None:
                a = jnp.zeros((16, 128), i32)
            if b is None:
                b = jnp.zeros((16, 128), i32)
            return jnp.where(m, a, b)

        def phase_b1(g):
            sl = g % NSS
            slp = g % NSP
            lo_ = [lov(u) for u in range(4)]
            nf = [7 if lo_[u] == 0 else 8 - lo_[u] for u in range(4)]

            def pblock(u, row0):
                p = jnp.exp2(s_ref[sl, u, row0:row0 + 32] - ms[(g, u)])
                return jnp.concatenate([_packi(p[16 * j:16 * j + 8], p[16 * j + 8:16 * j + 16]) for j in range(2)], 0)

            tri = {}

            def block(u, rel):
                if rel < 0 or rel > 8:
                    return None
                if rel == 0 or rel == 8:
                    if u not in tri:
                        pt = pblock(u, 0)
                        if lo_[u] == 0:
                            p8 = pt & le_pk
                            tri[u] = {8: p8, 0: pt ^ p8}
                        else:
                            tri[u] = {8: pt, 0: None}
                    return tri[u][rel]
                first = 8 - nf[u]
                if rel < first:
                    return None
                return pblock(u, 32 + 32 * (rel - first))

            for beta in range(4 * tiles[0], 12):
                src = [block(u, beta - u) for u in range(4)]
                a0 = sel(bit0, src[1], src[0])
                a1 = sel(bit0, src[0], src[1])
                c0 = sel(bit0, src[3], src[2])
                c1 = sel(bit0, src[2], src[3])
                o4 = [sel(bit1, c0, a0), sel(bit1, c1, a1), sel(bit1, a0, c0), sel(bit1, a1, c1)]
                for e in range(4):
                    p_ref[slp, e, 16 * beta:16 * beta + 16, :] = (
                        o4[e] if o4[e] is not None else jnp.zeros((16, 128), i32))

        okey = "order" if not static else ("order_pre" if i in (2, 3) else ("order_post" if i == NB - 1 else "order_01"))
        order = CFG.get(okey, {"order": "B P0 A0 A1 A2 A3 P1 P2 P3 X X Y",
                               "order_pre": "B A0 A1 P0 A2 P1 A3 P2 P3 X X Y",
                               "order_post": "B A0 A1 A2 P0 P1 P2 A3 P3 X X Y",
                               "order_01": "B P0 P1 A0 A1 A2 A3 P2 P3 X X Y"}[okey])

        def step(s):
            if s == -1 and head is not None:
                head()
            px = plan.get(s, [])
            todo = list(range(len(px)))
            for tok in order.split():
                if tok[0] == "A" and 0 <= s + 1 < 8:
                    phase_a(s + 1, [int(c) for c in tok[1:]])
                if tok[0] == "B" and 0 <= s < 8:
                    phase_b1(s)
                if tok[0] == "P" and 0 <= s - 1 < 8:
                    pv_group(s - 1, i, [int(c) for c in tok[1:]])
                if tok[0] == "X" and todo:
                    px[todo.pop(0)]()
                if tok[0] == "Y":
                    while todo:
                        px[todo.pop(0)]()
            while todo:
                px[todo.pop(0)]()
            if s == 7:
                for t in range(4):
                    fin_tile(t, ob_slot(i))

        steps = [(lambda s=s: step(s)) for s in range(-1, 8)]
        if lazy:
            return steps
        for f in steps:
            f()

    def a1_step(ax, ay, order):
        w = {}
        if ax is not None:
            j, par = ax // 2, ax % 2
            x = [_unpacki(xa32[t, pl.ds(j, 128, stride=8), :], par) for t in range(5)]
            t1 = x[1] + x[4]
            t2 = x[2] + x[3]
            t3 = x[1] - x[4]
            t4 = x[2] - x[3]
            p1 = x[0] + C1 * t1 + C2 * t2
            p2 = x[0] + C2 * t1 + C1 * t2
            q1 = S1 * t3 + S2 * t4
            q2 = S2 * t3 - S1 * t4
            ops = [x[0] + t1 + t2, p1 + q1, q1, p1, p2 + q2, q2, p2]
            w0s = [0, 80, 144, 208, 272, 336, 400, 464]
        for tok in order:
            if tok[0] == "x" and ax is not None:
                n = int(tok[1])
                w[tok] = _dot_nt(_b16(ff32[w0s[n]:w0s[n + 1]]), ops[n].astype(bf))
            if tok[0] == "y" and ay is not None:
                n = int(tok[1])
                w[tok] = _dot(ys_ref[ay % 2, n], _b16(rr32[ay, n]))
        if ay is not None:
            g_ = jnp.concatenate([w["y0"] - w["y1"], w["y0"] - w["y2"]], 1)
            for g in range(R // 8):
                gs_refs[g % 4][ay, 8 * (g // 4):8 * (g // 4) + 8, :] = g_[8 * g:8 * g + 8]
        if ax is not None:
            re, im = [w["x0"][0:80]], [w["x0"][80:160]]
            for n in (1, 4):
                t1, t2, t3 = w["x%d" % n], w["x%d" % (n + 1)], w["x%d" % (n + 2)]
                re.append(t1 - t2)
                im += [t3[0:64] - t1[0:64], t1[64:128] - t3[64:128]]
            yr = jnp.concatenate(re, 0)
            yi = jnp.concatenate(im, 0)
            ys_ref[ax % 2, 0] = (yr + yi).astype(bf)
            ys_ref[ax % 2, 1] = yi.astype(bf)
            ys_ref[ax % 2, 2] = yr.astype(bf)

    def a2_group(n, gq, token=None):
        g = 4 * gq + n
        special = isinstance(gq, int) and g == 8
        if isinstance(gq, int):
            w8 = g if g < 8 else (g - 10) % 8
            c10 = [0, 1, 4, 2, 3][0 if g < 8 else (g - 10) // 8 + 1] + 5 * (w8 // 4)
            r0 = 8 * gq
        else:
            w8 = jnp.where(g < 8, g, (g - 10) & 7)
            blk = jnp.minimum(jnp.where(g < 10, 0, ((g - 10) >> 3) + 1), 4)
            c10 = jnp.where(blk == 2, 4, jnp.where(blk > 2, blk - 1, blk)) + 5 * (w8 >> 2)
            r0 = 8 * gq
            if n == 0:
                r0 = jnp.where(g == 8, 96, r0)
            r0 = pl.multiple_of(r0, 8)
        w0 = (c10 >> 1) + 40 * (w8 & 3)
        sh = 16 * (1 - (c10 & 1))

        def wload(ref, last, f1):
            if special:
                return jnp.broadcast_to(last[0:1, 128 * f1:128 * f1 + 128].astype(f32), (8, 128))
            return pltpu.bitcast((ref[f1, pl.ds(w0, 8, stride=5), :] << sh) & jnp.int32(-65536), f32)

        gref = gs_refs[n]
        if token is not None:
            gref[16, pl.ds(pl.multiple_of(8 * (gq & 15), 8), 8), 0:128] = token
        z = [(gref[a, pl.ds(r0, 8), 0:128], gref[a, pl.ds(r0, 8), 128:256]) for a in range(16)]
        X = _fft16(z, False)
        V = []
        for f1 in range(16):
            wr = wload(wr32, wr_last, f1)
            wi = wload(wi32, wi_last, f1)
            V.append((X[f1][0] * wr - X[f1][1] * wi, X[f1][0] * wi + X[f1][1] * wr))
        U = _fft16(V, True)
        for a in range(16):
            gref[a, pl.ds(r0, 8), 0:128] = U[a][0]
            gref[a, pl.ds(r0, 8), 128:256] = U[a][1]

    def a3_step(az, ad, order, extra=()):
        w = {}
        if az is not None:
            u = jnp.concatenate([gs_refs[g % 4][az, 8 * (g // 4):8 * (g // 4) + 8, :] for g in range(R // 8)], 0)
            ur = u[:, 0:128]
            ui = u[:, 128:256]
            zops = [(ur + ui, 0), (ui, 2), (ur, 1)]
        for tok in order:
            if tok[0] == "z" and az is not None:
                v, n = zops[int(tok[1])]
                w[tok] = _dot_nt(v.astype(bf), _b16(rr32[az, n]))
            if tok[0] == "d" and ad is not None:
                n = int(tok[1])
                w[tok] = _dot(zs_ref[ad % 2, n], _b16(gg32[64 * n:64 * n + 64]))
            if tok == "E":
                for f in extra:
                    f()
        if ad is not None:
            v0 = w["d0"]
            v1r, v1i = w["d1"] - w["d2"], w["d1"] + w["d3"]
            v2r, v2i = w["d4"] - w["d5"], w["d4"] + w["d6"]
            A1 = v0 + C1 * v1r + C2 * v2r
            A2 = v0 + C2 * v1r + C1 * v2r
            B1 = S1 * v1i + S2 * v2i
            B2 = S2 * v1i - S1 * v2i
            y = [v0 + v1r + v2r, A1 - B1, A2 - B2, A2 + B2, A1 + B1]
            for t in range(5):
                if ad % 2 == 0:
                    ysc_ref[t] = y[t]
                else:
                    oa32[t, pl.ds(ad // 2, 128, stride=8), :] = _packi(ysc_ref[t], y[t])
        if az is not None:
            zr = w["z0"] - w["z1"]
            zi = w["z0"] - w["z2"]
            kop = [jnp.concatenate([zr[0:64], jnp.where(sub0, zr[64:72], zi[0:8]), zi[8:64]], 0)]
            for r0 in (80, 208):
                kop += [jnp.concatenate([zr[r0:r0 + 64] + zi[r0:r0 + 64], zr[r0 + 64:r0 + 128] - zi[r0 + 64:r0 + 128]], 0),
                        zi[r0:r0 + 128], zr[r0:r0 + 128]]
            for n in range(7):
                zs_ref[az % 2, n] = kop[n].T.astype(bf)

    def run(pieces, order=None):
        for k in (order or list(pieces)):
            if k in pieces:
                pieces[k]()

    PLAN = {-1: ["v0", "v1"], 0: ["q0", "k0"], 1: ["k1", "q1", "a3"], 2: ["k2", "q2"], 3: ["o0", "o1", "a1"],
            4: ["k3", "q3"], 5: ["o2", "o3", "a0"], 6: ["v2", "o4", "a2"], 7: ["k4", "q4", "v3", "v4"]}

    if 'plan' in CFG:
        PLAN = {int(k): v for k, v in CFG['plan'].items()}

    def mkplan(pieces):
        return {s_: [pieces[k] for k in ks if k in pieces] for s_, ks in PLAN.items()}

    ORD = ["v0", "v1", "v2", "v3", "v4", "k0", "k1", "k2", "k3", "k4", "q0", "q1", "q2", "q3", "q4"]

    def out_b_copy(i):
        return pltpu.make_async_copy(obo32.at[pl.ds(wrows_of(i), 64)],
                                     oh32.at[pl.ds(wrows_of(i), 64), pl.ds(D, D)], osem.at[0])

    for g in range(R // 8, 44):
        gs_refs[g % 4][0:16, 8 * (g // 4):8 * (g // 4) + 8, :] = jnp.zeros((16, 8, 256), f32)
    gs_refs[0][0:16, 96:104, :] = jnp.zeros((16, 8, 256), f32)
    c_x0.wait()
    c_wk.wait()
    prep_x(0)
    P0 = proj_pieces(0, do_q=False)
    run(P0, ["k0", "k1", "k2", "k3", "k4"])
    prep_x(1)
    P1 = proj_pieces(1, do_q=False)
    nk = CFG.get("nk", 3)
    KS = ["k0", "k1", "k2", "k3", "k4"]
    VS = ["v0", "v1", "v2", "v3", "v4"]
    run(P1, KS[:nk])
    c_wv.wait()
    prep_wvt()
    run(P1, KS[nk:])
    run(P0, VS)
    nv = CFG.get("nv", 5)
    run(P1, VS[:nv])
    c_x1.wait()
    c_wq.wait()
    run(P1, VS[nv:])
    prep_x(2)
    run(proj_pieces(2), CFG.get("ord2", ["q0", "k0", "q1", "k1", "q2", "k2", "q3", "k3", "q4", "k4"] + VS))
    for i_ in range(2):
        xq_ref[i_] = _zip16(_b16(xb32[64 * i_:64 * i_ + 64, :]).astype(f32))

    def with_q(P, i_):
        Pq = proj_pieces(i_, do_kv=False, qdst=qw01_ref.at[i_], xz=xq_ref.at[i_])
        P.update({"o%d" % t: Pq["q%d" % t] for t in range(5)})
        return P

    prep_x(3)
    attn(2, mkplan(with_q(proj_pieces(3), 0)))
    prep_x(4)
    attn(3, mkplan(with_q(proj_pieces(4), 1)), head=finish(2))

    for cp in [c_ff] + c_xa + [c_rr]:
        cp.wait()
    a1o = CFG.get("a1", "x0 x1 x2 x3 y0 x4 y1 x5 y2 x6").split()
    a1_step(0, None, a1o)
    for a in range(16):
        a1_step(a + 1 if a < 15 else None, a, a1o)
    for cp in c_w:
        cp.wait()
    c_x2.wait()
    c_wo.wait()
    c_gg.wait()

    def one_block(i):
        nxt = jnp.minimum(i + 1, NB - 1)
        prep_x(nxt)
        P = proj_pieces(nxt)
        P.update(out_pieces(i - 1))
        for n in range(4):
            P["a%d" % n] = (lambda n=n: a2_group(n, i - 4, token(n)))
        last_m.clear()
        attn(i, mkplan(P), head=finish(i - 1))

    UNR = CFG.get("unroll", 1)

    def body(it, carry):
        for u_ in range(UNR):
            i = 4 + UNR * it + u_
            one_block(i)
            out_b_copy(i - 1).start()
        return carry

    lax.fori_loop(0, NB - 5, body, 0)

    finish(NB - 2)()
    a2_group(0, 2)

    extra = attn(0, {}, qsrc=qw01_ref.at[0], lazy=True) + attn(1, {}, head=finish(0), qsrc=qw01_ref.at[1], lazy=True)
    extra += [lambda: pv_group(7, 1), lambda: fin_tile(4, 2)]
    a3o = CFG.get("a3", "z0 E z1 z2 d0 d1 d2 d3 d4 d5 d6").split()
    a3_step(0, None, a3o)
    for a in range(16):
        cut = CFG.get("cut", [0, 1, 2, 2, 5, 5, 7, 8, 10, 11, 12, 13, 15, 16, 18, 18, 20])
        a3_step(a + 1 if a < 15 else None, a, a3o, extra[cut[a]:cut[a + 1]])
    c_oa = [pltpu.make_async_copy(oa32.at[t], oh32.at[:, pl.ds(128 * t, 128)], osem.at[1 + t]) for t in range(5)]
    for cp in c_oa:
        cp.start()
    c_pin.wait()

    fill = []
    for t in range(5):
        fill += [out_pieces(0, slot=0)["o%d" % t], out_pieces(1, slot=2)["o%d" % t],
                 out_pieces(2, slot=3)["o%d" % t], out_pieces(NB - 2)["o%d" % t]]
    last_m.clear()
    fc = CFG.get("fc", [0, 3, 5, 7, 9, 11, 13, 15, 17, 20])
    attn(NB - 1, {s_: fill[fc[s_ + 1]:fc[s_ + 2]] for s_ in range(-1, 8)})
    for i_ in (0, 1, 2, NB - 2):
        out_b_copy(i_).start()
    c_pin2.wait()
    finish(NB - 1)()
    run(out_pieces(NB - 1))
    out_b_copy(NB - 1).start()

    for cp in c_oa:
        cp.wait()
    for i in range(NB):
        out_b_copy(i).wait()


def _build(FF32, GG32, RR32):
    scratch = [
        pltpu.VMEM((5, S // 2, 128), i32),
        pltpu.VMEM((NB, 160, 128), i32), pltpu.VMEM((NB, 160, 128), i32),
        pltpu.VMEM((1, S), bf), pltpu.VMEM((1, S), bf),
        pltpu.VMEM(FF32.shape, i32), pltpu.VMEM(GG32.shape, i32), pltpu.VMEM(RR32.shape, i32),
        pltpu.VMEM((2, 3, R, 128), bf),
        pltpu.VMEM((2, 7, 128, 128), bf),
        pltpu.VMEM((5, 128, 128), f32),
        pltpu.VMEM((5, S // 2, 128), i32),
        pltpu.VMEM((2, 8, 128), i32),
        pltpu.VMEM((2, 8, 64, 128), i32),
        pltpu.VMEM((2, 64, D), i32),
        pltpu.VMEM((S // 2, D), i32),
        pltpu.VMEM((D // 2, 3 * D), i32),
        pltpu.VMEM((D // 2, D), i32),
        pltpu.VMEM((D // 2, D), i32),
        pltpu.VMEM((CFG.get('ss', 1), 4, 256, 128), f32),
        pltpu.VMEM((CFG.get('sp', 2), 4, 192, 128), i32),
        pltpu.VMEM((4, 64, D), i32),
        pltpu.VMEM((D, 128), f32),
        pltpu.VMEM((8, 64, 128), i32),
        pltpu.VMEM((2, 64, D), i32),
        pltpu.VMEM((S // 2, D), i32),
        pltpu.SemaphoreType.DMA((25,)),
        pltpu.SemaphoreType.DMA((6,)),
        pltpu.SemaphoreType.DMA((1,)),
    ]
    scratch += [pltpu.VMEM((17, 104, 256), f32)] * 4
    scratch += [pltpu.VMEM((S // 2, 128), i32)] * 8
    scratch += [pltpu.VMEM((4, NB, 32, 128), bf)] * 8
    return pl.pallas_call(
        _kernel,
        out_shape=jax.ShapeDtypeStruct((S, 2 * D), bf),
        in_specs=[pl.BlockSpec(memory_space=pl.ANY)] * 9,
        out_specs=pl.BlockSpec(memory_space=pl.ANY),
        scratch_shapes=scratch,
        compiler_params=pltpu.CompilerParams(vmem_limit_bytes=110 * 2 ** 20),
    )


@jax.jit
def pallas_concat_heads__spectral_gfnet__sliding_block__prompt_kernel(
    A_x: jax.Array,
    A_w_r: jax.Array,
    A_w_i: jax.Array,
    B_x: jax.Array,
    B_wqkv: jax.Array,
    B_wo: jax.Array,
):
    FF32, GG32, RR32 = _make_consts()
    out = _build(FF32, GG32, RR32)(
        A_x.reshape(S, D), A_w_r.T, A_w_i.T, B_x.reshape(S, D), B_wqkv, B_wo,
        jnp.asarray(FF32), jnp.asarray(GG32), jnp.asarray(RR32))
    return out.reshape(1, S, 2 * D)
```

```python
import numpy as np
import ml_dtypes
import jax
import jax.numpy as jnp
from jax import lax
import jax.experimental.pallas as pl
import jax.experimental.pallas.tpu as pltpu

S = 2048
D = 640
DF = 321
H = 32
DH = 20
NB = S // 128
R = 336
NEG = -1e30
f32 = jnp.float32
bf = jnp.bfloat16
i32 = jnp.int32

C1 = float(np.cos(2 * np.pi / 5))
C2 = float(np.cos(4 * np.pi / 5))
S1 = float(np.sin(2 * np.pi / 5))
S2 = float(np.sin(4 * np.pi / 5))


def _pack_rows(a):
    u = np.ascontiguousarray(a.astype(ml_dtypes.bfloat16)).view(np.uint16).astype(np.uint32)
    return (u[..., 0::2, :] | (u[..., 1::2, :] << 16)).astype(np.uint32).view(np.int32)


def _make_consts():
    b5 = np.arange(128)

    def cs(k):
        th = 2 * np.pi * np.outer(k, b5) / D
        return np.cos(th), np.sin(th)

    m32 = np.arange(32)
    k0 = np.concatenate([10 * m32, 5 + 10 * m32, [320]])
    c, s = cs(k0)
    F0 = np.zeros((160, 128))
    F0[0:65] = c
    F0[80:145] = -s

    def kpair(j):
        return (np.concatenate([j + 10 * m32, j + 5 + 10 * m32]),
                np.concatenate([5 - j + 10 * m32, 10 - j + 10 * m32]))

    def fwd(j):
        ka, kb = kpair(j)
        (ca, sa), (cb, sb) = cs(ka), cs(kb)
        return np.concatenate([ca, cb, ca + sa, cb - sb, ca - sa, cb + sb], 0)

    FF = np.concatenate([F0, fwd(1), fwd(2)], 0)

    b = np.arange(128)
    f2 = np.arange(128)
    RR = np.zeros((16, 3, 128, 128))
    for a in range(16):
        th = -2 * np.pi * (np.outer(b, f2) / 128.0 + a * f2[None, :] / float(S))
        Mr, Mi = np.cos(th), np.sin(th)
        RR[a, 0] = Mr
        RR[a, 1] = Mr + Mi
        RR[a, 2] = Mr - Mi

    sc = 1.0 / (S * D)
    G0 = np.zeros((128, 128))
    al = np.full(65, 2.0)
    al[0] = 1.0
    al[64] = 1.0
    G0[:, 0:64] = (al[0:64, None] * c[0:64]).T
    G0[:, 64:128] = (-al[0:64, None] * s[0:64]).T
    G0[:, 64] = al[64] * c[64]

    def inv(j):
        ka, kb = kpair(j)
        (ca, sa), (cb, sb) = cs(ka), cs(kb)
        return 2 * np.concatenate([np.concatenate([ca, cb], 0).T,
                                   np.concatenate([ca + sa, sb - cb], 0).T,
                                   np.concatenate([sa - ca, -sb - cb], 0).T], 0)

    GG = np.concatenate([G0, inv(1), inv(2)], 0) * sc
    GG = GG.reshape(7, 128, 128).transpose(0, 2, 1).reshape(896, 128)
    return _pack_rows(FF), _pack_rows(GG), _pack_rows(RR)


_NT = (((1,), (1,)), ((), ()))


def _dot(a, b):
    return jnp.dot(a, b, preferred_element_type=f32)


def _dot_nt(a, b):
    return lax.dot_general(a, b, _NT, preferred_element_type=f32)


def _b16(x):
    return pltpu.bitcast(x, bf)


def _packi(a, b):
    return pltpu.pack_elementwise([a, b], packed_dtype=bf)


def _unpacki(x, idx):
    return pltpu.unpack_elementwise(x, index=idx, packed_dtype=bf, unpacked_dtype=f32)


def _zip16(x):
    n = x.shape[0] // 16
    return jnp.concatenate([_packi(x[16 * j:16 * j + 8], x[16 * j + 8:16 * j + 16]) for j in range(n)], 0)


def _dft4(z, inv):
    (a, b, c, d) = z
    t0 = (a[0] + c[0], a[1] + c[1])
    t1 = (a[0] - c[0], a[1] - c[1])
    t2 = (b[0] + d[0], b[1] + d[1])
    t3 = (b[0] - d[0], b[1] - d[1])
    o0 = (t0[0] + t2[0], t0[1] + t2[1])
    o2 = (t0[0] - t2[0], t0[1] - t2[1])
    p = (t1[0] + t3[1], t1[1] - t3[0])
    q = (t1[0] - t3[1], t1[1] + t3[0])
    return [o0, q, o2, p] if inv else [o0, p, o2, q]


def _tw16(z, e, inv):
    if e == 0:
        return z
    zr, zi = z
    if e == 4:
        return (-zi, zr) if inv else (zi, -zr)
    h = float(np.sqrt(0.5))
    if e == 2:
        return ((zr - zi) * h, (zr + zi) * h) if inv else ((zr + zi) * h, (zi - zr) * h)
    if e == 6:
        return ((-zr - zi) * h, (zr - zi) * h) if inv else ((zi - zr) * h, (-zr - zi) * h)
    sgn = 1.0 if inv else -1.0
    c = float(np.cos(2 * np.pi * e / 16))
    s = float(sgn * np.sin(2 * np.pi * e / 16))
    return (zr * c - zi * s, zr * s + zi * c)


def _fft16(z, inv):
    hh = [_dft4([z[a0 + 4 * a1] for a1 in range(4)], inv) for a0 in range(4)]
    out = [None] * 16
    for fa in range(4):
        o = _dft4([_tw16(hh[a0][fa], a0 * fa, inv) for a0 in range(4)], inv)
        for fb in range(4):
            out[fa + 4 * fb] = o[fb]
    return out


def _gwin(g):
    lo, hi = 80 * g, 80 * g + 79
    if lo // 128 == hi // 128:
        return ("nat", lo // 128, lo - 128 * (lo // 128))
    t = (lo - 64) // 128
    return ("shf", t, lo - 64 - 128 * t)


def _kernel(xa_hbm, wr_hbm, wi_hbm, xb_hbm, wqkv_hbm, wo_hbm, ff_hbm, gg_hbm, rr_hbm, out_hbm,
            xa32, wr32, wi32, wr_last, wi_last, ff32, gg32, rr32, ys_ref, zs_ref, ysc_ref, oa32,
            pin_ref, qw01_ref, xq_ref, xb32, wqkv32, wo32, wvt32, s_ref, p_ref, ob32, ot_ref, qw_ref, xz_ref, obo32,
            sem, osem, wsem, *groups):
    gs_refs = groups[0:4]
    kw_refs = groups[4:12]
    vt_refs = groups[12:20]

    def copy(src, dst, k):
        return pltpu.make_async_copy(src, dst, sem.at[k])

    xbh = xb_hbm.bitcast(i32)
    wqh = wqkv_hbm.bitcast(i32)
    xah = xa_hbm.bitcast(i32)
    oh32 = out_hbm.bitcast(i32)
    c_x0 = copy(xbh.at[pl.ds(0, 128)], xb32.at[pl.ds(0, 128)], 0)
    c_wk = copy(wqh.at[:, pl.ds(640, 640)], wqkv32.at[:, pl.ds(640, 640)], 1)
    c_wv = copy(wqh.at[:, pl.ds(1280, 640)], wqkv32.at[:, pl.ds(1280, 640)], 2)
    c_x1 = copy(xbh.at[pl.ds(128, 192)], xb32.at[pl.ds(128, 192)], 3)
    c_wq = copy(wqh.at[:, pl.ds(0, 640)], wqkv32.at[:, pl.ds(0, 640)], 4)
    c_ff = copy(ff_hbm, ff32, 5)
    c_xa = [copy(xah.at[:, pl.ds(128 * t, 128)], xa32.at[t], 6 + t) for t in range(5)]
    c_rr = copy(rr_hbm, rr32, 11)
    c_w = []
    for n, (src, dst, dst1) in enumerate(((wr_hbm, wr32, wr_last), (wi_hbm, wi32, wi_last))):
        w320 = src.at[pl.ds(0, 320)].bitcast(i32)
        for t in range(NB):
            c_w.append(pltpu.make_async_copy(w320.at[:, pl.ds(128 * t, 128)], dst.at[t], wsem.at[0]))
        c_w.append(copy(src.at[pl.ds(320, 1)], dst1, 13 + n))
    c_x2 = copy(xbh.at[pl.ds(320, 704)], xb32.at[pl.ds(320, 704)], 21)
    c_wo = copy(wo_hbm.bitcast(i32), wo32, 22)
    c_gg = copy(gg_hbm, gg32, 23)
    c_pin = copy(xbh.at[pl.ds(0, 8), pl.ds(0, 128)], pin_ref.at[0], 24)
    c_pin2 = copy(xbh.at[pl.ds(0, 8), pl.ds(0, 128)], pin_ref.at[1], 12)
    for cp in ([c_x0, c_wk, c_wv, c_x1, c_wq, c_ff] + c_xa + [c_rr]
               + c_w + [c_x2, c_wo, c_gg, c_pin, c_pin2]):
        cp.start()

    scale = float(DH ** -0.5 * np.log2(np.e))
    def _qpos(l):
        return (l & 16) + 4 * (l & 3) + ((l & 15) >> 2)
    rr_ = lax.broadcasted_iota(i32, (32, 128), 0)
    ll_ = _qpos(lax.broadcasted_iota(i32, (32, 128), 1))
    pos_ = rr_ & 15
    key_ = (rr_ & 16) + jnp.where(pos_ < 8, 2 * pos_, 2 * (pos_ - 8) + 1)
    le32 = key_ <= ll_
    wr_ = lax.broadcasted_iota(i32, (16, 128), 0)
    wq_ = _qpos(lax.broadcasted_iota(i32, (16, 128), 1))
    le_pk = (jnp.where(2 * wr_ <= wq_, jnp.int32(0xFFFF), jnp.int32(0))
             | jnp.where(2 * wr_ + 1 <= wq_, jnp.int32(-65536), jnp.int32(0)))
    lane8 = lax.broadcasted_iota(i32, (8, 128), 1)
    lane16 = lax.broadcasted_iota(i32, (16, 128), 1)
    bit0 = (lane16 & 32) != 0
    bit1 = (lane16 & 64) != 0
    bit0_8 = (lane8 & 32) != 0
    sub4 = lax.broadcasted_iota(i32, (8, 128), 0) < 4
    sub0 = lax.broadcasted_iota(i32, (8, 128), 0) == 0
    ones8 = jnp.ones((8, 128), f32)
    lo64 = lax.broadcasted_iota(i32, (64, 128), 1) < 64

    def wrows_of(i):
        return i * 64 if isinstance(i, int) else pl.multiple_of(i * 64, 64)

    def prep_wvt():
        for tr in range(5):
            wvt32[64 * tr:64 * tr + 64, :] = pltpu.bitcast(
                _b16(wqkv32[:, 1280 + tr * 128:1280 + (tr + 1) * 128]).T, i32)

    def prep_x(i):
        w = xb32[pl.ds(wrows_of(i), 64), :]
        z1 = _zip16(_b16(w).astype(f32))
        xz_ref[0] = z1
        xz_ref[1] = _zip16(_b16(z1).astype(f32))

    def win_ready(tiles, rolled, done, emit):
        for g in range(8):
            if g in done:
                continue
            kind, t, _ = _gwin(g)
            if kind == "nat":
                if t in tiles:
                    emit(g, tiles[t])
                    done.add(g)
            elif t in tiles and (t + 1) in tiles:
                for tt in (t, t + 1):
                    if tt not in rolled:
                        rolled[tt] = pltpu.roll(tiles[tt], 64, 1)
                emit(g, jnp.where(lo64, rolled[t], rolled[t + 1]))
                done.add(g)

    def proj_pieces(i, do_q=True, do_kv=True, qdst=None, xz=None):
        qdst = qw_ref if qdst is None else qdst
        xz = xz_ref.at[0] if xz is None else xz
        pieces = {}
        if do_kv:
            v8 = {}
            vdone = set()

            def vpiece(r):
                def f():
                    xb = _b16(xb32[pl.ds(wrows_of(i), 64), :])
                    vt = _dot_nt(_b16(wvt32[64 * r:64 * r + 64, :]), xb)
                    for j in range(16):
                        v8[16 * r + j] = vt[8 * j:8 * j + 8]
                    for p in range(16):
                        if p in vdone or any((5 * p + j) not in v8 for j in range(5)):
                            continue
                        v = [v8[5 * p + j] for j in range(5)]
                        h0, h1 = 2 * p, 2 * p + 1
                        vt_refs[h0 // 4][h0 % 4, i] = jnp.concatenate([v[0], v[1], v[2], ones8], 0).astype(bf)
                        vt_refs[h1 // 4][h1 % 4, i] = jnp.concatenate([v[2], v[3], v[4], ones8], 0).astype(bf)
                        vdone.add(p)
                return f

            kt, kr, kd = {}, {}, set()

            def kpiece(t):
                def f():
                    kt[t] = _zip16(_dot(_b16(xz_ref[1]), _b16(wqkv32[:, 640 + 128 * t:640 + 128 * t + 128])))

                    def emit(g, val):
                        kw_refs[g][pl.ds(wrows_of(i), 64), :] = val
                    win_ready(kt, kr, kd, emit)
                return f

            for r in range(5):
                pieces["v%d" % r] = vpiece(r)
                pieces["k%d" % r] = kpiece(r)
        if do_q:
            qt, qr, qd = {}, {}, set()

            def qpiece(t):
                def f():
                    qt[t] = _zip16(_dot(_b16(xz[...]), _b16(wqkv32[:, 128 * t:128 * t + 128])) * scale)

                    def emit(g, val):
                        qdst[g] = val
                    win_ready(qt, qr, qd, emit)
                return f

            for t in range(5):
                pieces["q%d" % t] = qpiece(t)
        return pieces

    def out_pieces(i, slot=1):
        def opiece(t):
            def f():
                res = _dot(_b16(ob32[slot]), _b16(wo32[:, 128 * t:128 * t + 128]))
                obo32[pl.ds(wrows_of(i), 64), 128 * t:128 * t + 128] = _zip16(res)
            return f
        return {"o%d" % t: opiece(t) for t in range(5)}

    def key_tiles(i):
        return list(range(3)) if (not isinstance(i, int) or i >= 2) else list(range(2 - i, 3))

    pv_outs = {}

    def pv_group(g, i, es=(0, 1, 2, 3)):
        tiles = key_tiles(i)
        sl = g % 2
        for e in es:
            P = _b16(p_ref[sl, e, 64 * tiles[0]:192, :])
            if len(tiles) > 1:
                vw = jnp.concatenate([vt_refs[g][e, i - 2 + j] for j in tiles], 1)
            else:
                vw = vt_refs[g][e, i]
            o = _dot(vw, P)
            rl = pltpu.reciprocal(o[24:32])
            res = [o[0:8] * rl, o[8:16] * rl, o[16:24] * rl]
            if e == 2:
                res = [pltpu.roll(r, 64, 1) for r in res]
            elif e == 1:
                res = [jnp.where(bit0_8, pltpu.roll(r, 32, 1), pltpu.roll(r, 96, 1)) for r in res]
            elif e == 3:
                res = [jnp.where(bit0_8, pltpu.roll(r, 96, 1), pltpu.roll(r, 32, 1)) for r in res]
            pv_outs[(g, e)] = res
            if (g, e ^ 1) in pv_outs:
                p = e // 2
                a, b = pv_outs.pop((g, 2 * p)), pv_outs.pop((g, 2 * p + 1))
                ot_ref[80 * g + 40 * p:80 * g + 40 * p + 40, :] = jnp.concatenate(
                    [a[0], a[1], jnp.where(sub4, a[2], b[0]), b[1], b[2]], 0)

    def fin_tile(t, slot):
        ob32[slot, :, 128 * t:128 * t + 128] = _zip16(ot_ref[128 * t:128 * t + 128, :].T)

    def ob_slot(i):
        return {0: 0, 1: 2, 2: 3}.get(i, 1) if isinstance(i, int) else 1

    def finish(i):
        def f():
            pv_group(7, i)
            fin_tile(4, ob_slot(i))
        return f

    last_m = {}

    def token():
        return jnp.broadcast_to(last_m[max(last_m)], (8, 128))

    def attn(i, plan, head=None, qsrc=None, lazy=False):
        qsrc = qw_ref if qsrc is None else qsrc
        static = isinstance(i, int)
        lov = (lambda u: max(0, 8 - u - 4 * i)) if static else (lambda u: 0)
        tiles = key_tiles(i)
        ms = last_m

        def phase_a(g, us):
            _, _, off = _gwin(g)
            hm = [jnp.where((lane16 >= off + 20 * e) & (lane16 < off + 20 * e + 20), jnp.int32(-1), jnp.int32(0))
                  for e in range(4)]
            for u in us:
                lo = lov(u)
                nrow = 32 * (9 - lo)
                k0 = 64 * i - 128 + 16 * u + 16 * lo
                if not static:
                    k0 = pl.multiple_of(k0, 16)
                kw = _b16(kw_refs[g][pl.ds(k0, nrow // 2), :])
                qu = qsrc[g, 16 * u:16 * u + 16, :]
                qm = _b16(jnp.concatenate([qu & hm[lam ^ u] for lam in range(4)], 0))
                s = _dot_nt(kw, qm)
                sd = s[nrow - 32:nrow]
                if lo == 0:
                    T = jnp.where(le32, sd, s[0:32])
                    F = s[32:256]
                else:
                    T = jnp.where(le32, sd, NEG)
                    F = s[0:nrow - 32]
                m = jnp.max(T, axis=0, keepdims=True)
                s_ref[u, 0:32] = T
                if F.shape[0] > 0:
                    m = jnp.maximum(m, jnp.max(F, axis=0, keepdims=True))
                    s_ref[u, 32:32 + F.shape[0]] = F
                ms[(g, u)] = m

        def sel(m, a, b):
            if a is None and b is None:
                return None
            if a is None:
                a = jnp.zeros((16, 128), i32)
            if b is None:
                b = jnp.zeros((16, 128), i32)
            return jnp.where(m, a, b)

        def phase_b1(g):
            slp = g % 2
            lo_ = [lov(u) for u in range(4)]
            nf = [7 if lo_[u] == 0 else 8 - lo_[u] for u in range(4)]

            def pblock(u, row0):
                p = jnp.exp2(s_ref[u, row0:row0 + 32] - ms[(g, u)])
                return jnp.concatenate([_packi(p[16 * j:16 * j + 8], p[16 * j + 8:16 * j + 16]) for j in range(2)], 0)

            tri = {}

            def block(u, rel):
                if rel < 0 or rel > 8:
                    return None
                if rel == 0 or rel == 8:
                    if u not in tri:
                        pt = pblock(u, 0)
                        if lo_[u] == 0:
                            p8 = pt & le_pk
                            tri[u] = {8: p8, 0: pt ^ p8}
                        else:
                            tri[u] = {8: pt, 0: None}
                    return tri[u][rel]
                first = 8 - nf[u]
                if rel < first:
                    return None
                return pblock(u, 32 + 32 * (rel - first))

            for beta in range(4 * tiles[0], 12):
                src = [block(u, beta - u) for u in range(4)]
                a0 = sel(bit0, src[1], src[0])
                a1 = sel(bit0, src[0], src[1])
                c0 = sel(bit0, src[3], src[2])
                c1 = sel(bit0, src[2], src[3])
                o4 = [sel(bit1, c0, a0), sel(bit1, c1, a1), sel(bit1, a0, c0), sel(bit1, a1, c1)]
                for e in range(4):
                    p_ref[slp, e, 16 * beta:16 * beta + 16, :] = (
                        o4[e] if o4[e] is not None else jnp.zeros((16, 128), i32))

        okey = "order" if not static else ("order_pre" if i in (2, 3) else ("order_post" if i == NB - 1 else "order_01"))
        order = {"order": "B P0 A0 A1 A2 A3 P1 P2 P3 X X Y",
                 "order_pre": "B A0 A1 P0 A2 P1 A3 P2 P3 X X Y",
                 "order_post": "B A0 A1 A2 P0 P1 P2 A3 P3 X X Y",
                 "order_01": "B P0 P1 A0 A1 A2 A3 P2 P3 X X Y"}[okey]

        def step(s):
            if s == -1 and head is not None:
                head()
            px = plan.get(s, [])
            todo = list(range(len(px)))
            for tok in order.split():
                if tok[0] == "A" and 0 <= s + 1 < 8:
                    phase_a(s + 1, [int(c) for c in tok[1:]])
                if tok[0] == "B" and 0 <= s < 8:
                    phase_b1(s)
                if tok[0] == "P" and 0 <= s - 1 < 8:
                    pv_group(s - 1, i, [int(c) for c in tok[1:]])
                if tok[0] == "X" and todo:
                    px[todo.pop(0)]()
                if tok[0] == "Y":
                    while todo:
                        px[todo.pop(0)]()
            while todo:
                px[todo.pop(0)]()
            if s == 7:
                for t in range(4):
                    fin_tile(t, ob_slot(i))

        steps = [(lambda s=s: step(s)) for s in range(-1, 8)]
        if lazy:
            return steps
        for f in steps:
            f()

    def a1_step(ax, ay, order):
        w = {}
        if ax is not None:
            j, par = ax // 2, ax % 2
            x = [_unpacki(xa32[t, pl.ds(j, 128, stride=8), :], par) for t in range(5)]
            t1 = x[1] + x[4]
            t2 = x[2] + x[3]
            t3 = x[1] - x[4]
            t4 = x[2] - x[3]
            p1 = x[0] + C1 * t1 + C2 * t2
            p2 = x[0] + C2 * t1 + C1 * t2
            q1 = S1 * t3 + S2 * t4
            q2 = S2 * t3 - S1 * t4
            ops = [x[0] + t1 + t2, p1 + q1, q1, p1, p2 + q2, q2, p2]
            w0s = [0, 80, 144, 208, 272, 336, 400, 464]
        for tok in order:
            if tok[0] == "x" and ax is not None:
                n = int(tok[1])
                w[tok] = _dot_nt(_b16(ff32[w0s[n]:w0s[n + 1]]), ops[n].astype(bf))
            if tok[0] == "y" and ay is not None:
                n = int(tok[1])
                w[tok] = _dot(ys_ref[ay % 2, n], _b16(rr32[ay, n]))
        if ay is not None:
            g_ = jnp.concatenate([w["y0"] - w["y1"], w["y0"] - w["y2"]], 1)
            for g in range(R // 8):
                gs_refs[g % 4][ay, 8 * (g // 4):8 * (g // 4) + 8, :] = g_[8 * g:8 * g + 8]
        if ax is not None:
            re, im = [w["x0"][0:80]], [w["x0"][80:160]]
            for n in (1, 4):
                t1, t2, t3 = w["x%d" % n], w["x%d" % (n + 1)], w["x%d" % (n + 2)]
                re.append(t1 - t2)
                im += [t3[0:64] - t1[0:64], t1[64:128] - t3[64:128]]
            yr = jnp.concatenate(re, 0)
            yi = jnp.concatenate(im, 0)
            ys_ref[ax % 2, 0] = (yr + yi).astype(bf)
            ys_ref[ax % 2, 1] = yi.astype(bf)
            ys_ref[ax % 2, 2] = yr.astype(bf)

    def a2_group(n, gq, token=None):
        g = 4 * gq + n
        special = isinstance(gq, int) and g == 8
        if isinstance(gq, int):
            w8 = g if g < 8 else (g - 10) % 8
            c10 = [0, 1, 4, 2, 3][0 if g < 8 else (g - 10) // 8 + 1] + 5 * (w8 // 4)
            r0 = 8 * gq
        else:
            w8 = jnp.where(g < 8, g, (g - 10) & 7)
            blk = jnp.minimum(jnp.where(g < 10, 0, ((g - 10) >> 3) + 1), 4)
            c10 = jnp.where(blk == 2, 4, jnp.where(blk > 2, blk - 1, blk)) + 5 * (w8 >> 2)
            r0 = 8 * gq
            if n == 0:
                r0 = jnp.where(g == 8, 96, r0)
            r0 = pl.multiple_of(r0, 8)
        w0 = (c10 >> 1) + 40 * (w8 & 3)
        sh = 16 * (1 - (c10 & 1))

        def wload(ref, last, f1):
            if special:
                return jnp.broadcast_to(last[0:1, 128 * f1:128 * f1 + 128].astype(f32), (8, 128))
            return pltpu.bitcast((ref[f1, pl.ds(w0, 8, stride=5), :] << sh) & jnp.int32(-65536), f32)

        gref = gs_refs[n]
        if token is not None:
            gref[16, pl.ds(pl.multiple_of(8 * (gq & 15), 8), 8), 0:128] = token
        z = [(gref[a, pl.ds(r0, 8), 0:128], gref[a, pl.ds(r0, 8), 128:256]) for a in range(16)]
        X = _fft16(z, False)
        V = []
        for f1 in range(16):
            wr = wload(wr32, wr_last, f1)
            wi = wload(wi32, wi_last, f1)
            V.append((X[f1][0] * wr - X[f1][1] * wi, X[f1][0] * wi + X[f1][1] * wr))
        U = _fft16(V, True)
        for a in range(16):
            gref[a, pl.ds(r0, 8), 0:128] = U[a][0]
            gref[a, pl.ds(r0, 8), 128:256] = U[a][1]

    def a3_step(az, ad, order, extra=()):
        w = {}
        if az is not None:
            u = jnp.concatenate([gs_refs[g % 4][az, 8 * (g // 4):8 * (g // 4) + 8, :] for g in range(R // 8)], 0)
            ur = u[:, 0:128]
            ui = u[:, 128:256]
            zops = [(ur + ui, 0), (ui, 2), (ur, 1)]
        for tok in order:
            if tok[0] == "z" and az is not None:
                v, n = zops[int(tok[1])]
                w[tok] = _dot_nt(v.astype(bf), _b16(rr32[az, n]))
            if tok[0] == "d" and ad is not None:
                n = int(tok[1])
                w[tok] = _dot(zs_ref[ad % 2, n], _b16(gg32[64 * n:64 * n + 64]))
            if tok == "E":
                for f in extra:
                    f()
        if ad is not None:
            v0 = w["d0"]
            v1r, v1i = w["d1"] - w["d2"], w["d1"] + w["d3"]
            v2r, v2i = w["d4"] - w["d5"], w["d4"] + w["d6"]
            A1 = v0 + C1 * v1r + C2 * v2r
            A2 = v0 + C2 * v1r + C1 * v2r
            B1 = S1 * v1i + S2 * v2i
            B2 = S2 * v1i - S1 * v2i
            y = [v0 + v1r + v2r, A1 - B1, A2 - B2, A2 + B2, A1 + B1]
            for t in range(5):
                if ad % 2 == 0:
                    ysc_ref[t] = y[t]
                else:
                    oa32[t, pl.ds(ad // 2, 128, stride=8), :] = _packi(ysc_ref[t], y[t])
        if az is not None:
            zr = w["z0"] - w["z1"]
            zi = w["z0"] - w["z2"]
            kop = [jnp.concatenate([zr[0:64], jnp.where(sub0, zr[64:72], zi[0:8]), zi[8:64]], 0)]
            for r0 in (80, 208):
                kop += [jnp.concatenate([zr[r0:r0 + 64] + zi[r0:r0 + 64], zr[r0 + 64:r0 + 128] - zi[r0 + 64:r0 + 128]], 0),
                        zi[r0:r0 + 128], zr[r0:r0 + 128]]
            for n in range(7):
                zs_ref[az % 2, n] = kop[n].T.astype(bf)

    def run(pieces, order=None):
        for k in (order or list(pieces)):
            if k in pieces:
                pieces[k]()

    PLAN = {-1: ["v0", "v1"], 0: ["q0", "k0"], 1: ["k1", "q1", "a3"], 2: ["k2", "q2"], 3: ["o0", "o1", "a1"],
            4: ["k3", "q3"], 5: ["o2", "o3", "a0"], 6: ["v2", "o4", "a2"], 7: ["k4", "q4", "v3", "v4"]}

    def mkplan(pieces):
        return {s_: [pieces[k] for k in ks if k in pieces] for s_, ks in PLAN.items()}

    def out_b_copy(i):
        return pltpu.make_async_copy(obo32.at[pl.ds(wrows_of(i), 64)],
                                     oh32.at[pl.ds(wrows_of(i), 64), pl.ds(D, D)], osem.at[0])

    for g in range(R // 8, 44):
        gs_refs[g % 4][0:16, 8 * (g // 4):8 * (g // 4) + 8, :] = jnp.zeros((16, 8, 256), f32)
    gs_refs[0][0:16, 96:104, :] = jnp.zeros((16, 8, 256), f32)
    c_x0.wait()
    c_wk.wait()
    prep_x(0)
    P0 = proj_pieces(0, do_q=False)
    run(P0, ["k0", "k1", "k2", "k3", "k4"])
    prep_x(1)
    P1 = proj_pieces(1, do_q=False)
    VS = ["v0", "v1", "v2", "v3", "v4"]
    run(P1, ["k0", "k1", "k2"])
    c_wv.wait()
    prep_wvt()
    run(P1, ["k3", "k4"])
    run(P0, VS)
    run(P1, VS)
    c_x1.wait()
    c_wq.wait()
    prep_x(2)
    run(proj_pieces(2), ["q0", "k0", "q1", "k1", "q2", "k2", "q3", "k3", "q4", "k4"] + VS)
    for i_ in range(2):
        xq_ref[i_] = _zip16(_b16(xb32[64 * i_:64 * i_ + 64, :]).astype(f32))

    def with_q(P, i_):
        Pq = proj_pieces(i_, do_kv=False, qdst=qw01_ref.at[i_], xz=xq_ref.at[i_])
        P.update({"o%d" % t: Pq["q%d" % t] for t in range(5)})
        return P

    prep_x(3)
    attn(2, mkplan(with_q(proj_pieces(3), 0)))
    prep_x(4)
    attn(3, mkplan(with_q(proj_pieces(4), 1)), head=finish(2))

    for cp in [c_ff] + c_xa + [c_rr]:
        cp.wait()
    a1o = "x0 x1 x2 x3 y0 x4 y1 x5 y2 x6".split()
    a1_step(0, None, a1o)
    for a in range(16):
        a1_step(a + 1 if a < 15 else None, a, a1o)
    for cp in c_w:
        cp.wait()
    c_x2.wait()
    c_wo.wait()
    c_gg.wait()

    def body(i, carry):
        nxt = jnp.minimum(i + 1, NB - 1)
        prep_x(nxt)
        P = proj_pieces(nxt)
        P.update(out_pieces(i - 1))
        for n in range(4):
            P["a%d" % n] = (lambda n=n: a2_group(n, i - 4, token()))
        last_m.clear()
        attn(i, mkplan(P), head=finish(i - 1))
        out_b_copy(i - 1).start()
        return carry

    lax.fori_loop(4, NB - 1, body, 0)

    finish(NB - 2)()
    a2_group(0, 2)

    extra = attn(0, {}, qsrc=qw01_ref.at[0], lazy=True) + attn(1, {}, head=finish(0), qsrc=qw01_ref.at[1], lazy=True)
    extra += [lambda: pv_group(7, 1), lambda: fin_tile(4, 2)]
    a3o = "z0 E z1 z2 d0 d1 d2 d3 d4 d5 d6".split()
    cut = [0, 1, 2, 2, 5, 5, 7, 8, 10, 11, 12, 13, 15, 16, 18, 18, 20]
    a3_step(0, None, a3o)
    for a in range(16):
        a3_step(a + 1 if a < 15 else None, a, a3o, extra[cut[a]:cut[a + 1]])
    c_oa = [pltpu.make_async_copy(oa32.at[t], oh32.at[:, pl.ds(128 * t, 128)], osem.at[1 + t]) for t in range(5)]
    for cp in c_oa:
        cp.start()
    c_pin.wait()

    fill = []
    for t in range(5):
        fill += [out_pieces(0, slot=0)["o%d" % t], out_pieces(1, slot=2)["o%d" % t],
                 out_pieces(2, slot=3)["o%d" % t], out_pieces(NB - 2)["o%d" % t]]
    last_m.clear()
    fc = [0, 3, 5, 7, 9, 11, 13, 15, 17, 20]
    attn(NB - 1, {s_: fill[fc[s_ + 1]:fc[s_ + 2]] for s_ in range(-1, 8)})
    for i_ in (0, 1, 2, NB - 2):
        out_b_copy(i_).start()
    c_pin2.wait()
    finish(NB - 1)()
    run(out_pieces(NB - 1))
    out_b_copy(NB - 1).start()

    for cp in c_oa:
        cp.wait()
    for i in range(NB):
        out_b_copy(i).wait()


def _build(FF32, GG32, RR32):
    scratch = [
        pltpu.VMEM((5, S // 2, 128), i32),
        pltpu.VMEM((NB, 160, 128), i32), pltpu.VMEM((NB, 160, 128), i32),
        pltpu.VMEM((1, S), bf), pltpu.VMEM((1, S), bf),
        pltpu.VMEM(FF32.shape, i32), pltpu.VMEM(GG32.shape, i32), pltpu.VMEM(RR32.shape, i32),
        pltpu.VMEM((2, 3, R, 128), bf),
        pltpu.VMEM((2, 7, 128, 128), bf),
        pltpu.VMEM((5, 128, 128), f32),
        pltpu.VMEM((5, S // 2, 128), i32),
        pltpu.VMEM((2, 8, 128), i32),
        pltpu.VMEM((2, 8, 64, 128), i32),
        pltpu.VMEM((2, 64, D), i32),
        pltpu.VMEM((S // 2, D), i32),
        pltpu.VMEM((D // 2, 3 * D), i32),
        pltpu.VMEM((D // 2, D), i32),
        pltpu.VMEM((D // 2, D), i32),
        pltpu.VMEM((4, 256, 128), f32),
        pltpu.VMEM((2, 4, 192, 128), i32),
        pltpu.VMEM((4, 64, D), i32),
        pltpu.VMEM((D, 128), f32),
        pltpu.VMEM((8, 64, 128), i32),
        pltpu.VMEM((2, 64, D), i32),
        pltpu.VMEM((S // 2, D), i32),
        pltpu.SemaphoreType.DMA((25,)),
        pltpu.SemaphoreType.DMA((6,)),
        pltpu.SemaphoreType.DMA((1,)),
    ]
    scratch += [pltpu.VMEM((17, 104, 256), f32)] * 4
    scratch += [pltpu.VMEM((S // 2, 128), i32)] * 8
    scratch += [pltpu.VMEM((4, NB, 32, 128), bf)] * 8
    return pl.pallas_call(
        _kernel,
        out_shape=jax.ShapeDtypeStruct((S, 2 * D), bf),
        in_specs=[pl.BlockSpec(memory_space=pl.ANY)] * 9,
        out_specs=pl.BlockSpec(memory_space=pl.ANY),
        scratch_shapes=scratch,
        compiler_params=pltpu.CompilerParams(vmem_limit_bytes=110 * 2 ** 20),
    )


@jax.jit
def pallas_concat_heads__spectral_gfnet__sliding_block__prompt_kernel(
    A_x: jax.Array,
    A_w_r: jax.Array,
    A_w_i: jax.Array,
    B_x: jax.Array,
    B_wqkv: jax.Array,
    B_wo: jax.Array,
):
    FF32, GG32, RR32 = _make_consts()
    out = _build(FF32, GG32, RR32)(
        A_x.reshape(S, D), A_w_r.T, A_w_i.T, B_x.reshape(S, D), B_wqkv, B_wo,
        jnp.asarray(FF32), jnp.asarray(GG32), jnp.asarray(RR32))
    return out.reshape(1, S, 2 * D)
```

```python
import numpy as np
import ml_dtypes
import jax
import jax.numpy as jnp
from jax import lax
import jax.experimental.pallas as pl
import jax.experimental.pallas.tpu as pltpu

S = 2048
D = 640
DF = 321
H = 32
DH = 20
NB = S // 128
R = 336
NEG = -1e30
f32 = jnp.float32
bf = jnp.bfloat16
i32 = jnp.int32

C1 = float(np.cos(2 * np.pi / 5))
C2 = float(np.cos(4 * np.pi / 5))
S1 = float(np.sin(2 * np.pi / 5))
S2 = float(np.sin(4 * np.pi / 5))


def _pack_rows(a):
    u = np.ascontiguousarray(a.astype(ml_dtypes.bfloat16)).view(np.uint16).astype(np.uint32)
    return (u[..., 0::2, :] | (u[..., 1::2, :] << 16)).astype(np.uint32).view(np.int32)


def _make_consts():
    b5 = np.arange(128)

    def cs(k):
        th = 2 * np.pi * np.outer(k, b5) / D
        return np.cos(th), np.sin(th)

    m32 = np.arange(32)
    k0 = np.concatenate([10 * m32, 5 + 10 * m32, [320]])
    c, s = cs(k0)
    F0 = np.zeros((160, 128))
    F0[0:65] = c
    F0[80:145] = -s

    def kpair(j):
        return (np.concatenate([j + 10 * m32, j + 5 + 10 * m32]),
                np.concatenate([5 - j + 10 * m32, 10 - j + 10 * m32]))

    def fwd(j):
        ka, kb = kpair(j)
        (ca, sa), (cb, sb) = cs(ka), cs(kb)
        return np.concatenate([ca, cb, ca + sa, cb - sb, ca - sa, cb + sb], 0)

    FF = np.concatenate([F0, fwd(1), fwd(2)], 0)

    b = np.arange(128)
    f2 = np.arange(128)
    RR = np.zeros((16, 3, 128, 128))
    for a in range(16):
        th = -2 * np.pi * (np.outer(b, f2) / 128.0 + a * f2[None, :] / float(S))
        Mr, Mi = np.cos(th), np.sin(th)
        RR[a, 0] = Mr
        RR[a, 1] = Mr + Mi
        RR[a, 2] = Mr - Mi

    sc = 1.0 / (S * D)
    G0 = np.zeros((128, 128))
    al = np.full(65, 2.0)
    al[0] = 1.0
    al[64] = 1.0
    G0[:, 0:64] = (al[0:64, None] * c[0:64]).T
    G0[:, 64:128] = (-al[0:64, None] * s[0:64]).T
    G0[:, 64] = al[64] * c[64]

    def inv(j):
        ka, kb = kpair(j)
        (ca, sa), (cb, sb) = cs(ka), cs(kb)
        return 2 * np.concatenate([np.concatenate([ca, cb], 0).T,
                                   np.concatenate([ca + sa, sb - cb], 0).T,
                                   np.concatenate([sa - ca, -sb - cb], 0).T], 0)

    GG = np.concatenate([G0, inv(1), inv(2)], 0) * sc
    GG = GG.reshape(7, 128, 128).transpose(0, 2, 1).reshape(896, 128)
    return _pack_rows(FF), _pack_rows(GG), _pack_rows(RR)


_NT = (((1,), (1,)), ((), ()))


def _dot(a, b):
    return jnp.dot(a, b, preferred_element_type=f32)


def _dot_nt(a, b):
    return lax.dot_general(a, b, _NT, preferred_element_type=f32)


def _b16(x):
    return pltpu.bitcast(x, bf)


def _packi(a, b):
    return pltpu.pack_elementwise([a, b], packed_dtype=bf)


def _unpacki(x, idx):
    return pltpu.unpack_elementwise(x, index=idx, packed_dtype=bf, unpacked_dtype=f32)


def _zip16(x):
    n = x.shape[0] // 16
    return jnp.concatenate([_packi(x[16 * j:16 * j + 8], x[16 * j + 8:16 * j + 16]) for j in range(n)], 0)


def _dft4(z, inv):
    (a, b, c, d) = z
    t0 = (a[0] + c[0], a[1] + c[1])
    t1 = (a[0] - c[0], a[1] - c[1])
    t2 = (b[0] + d[0], b[1] + d[1])
    t3 = (b[0] - d[0], b[1] - d[1])
    o0 = (t0[0] + t2[0], t0[1] + t2[1])
    o2 = (t0[0] - t2[0], t0[1] - t2[1])
    p = (t1[0] + t3[1], t1[1] - t3[0])
    q = (t1[0] - t3[1], t1[1] + t3[0])
    return [o0, q, o2, p] if inv else [o0, p, o2, q]


def _tw16(z, e, inv):
    if e == 0:
        return z
    zr, zi = z
    if e == 4:
        return (-zi, zr) if inv else (zi, -zr)
    h = float(np.sqrt(0.5))
    if e == 2:
        return ((zr - zi) * h, (zr + zi) * h) if inv else ((zr + zi) * h, (zi - zr) * h)
    if e == 6:
        return ((-zr - zi) * h, (zr - zi) * h) if inv else ((zi - zr) * h, (-zr - zi) * h)
    sgn = 1.0 if inv else -1.0
    c = float(np.cos(2 * np.pi * e / 16))
    s = float(sgn * np.sin(2 * np.pi * e / 16))
    return (zr * c - zi * s, zr * s + zi * c)


def _fft16(z, inv):
    hh = [_dft4([z[a0 + 4 * a1] for a1 in range(4)], inv) for a0 in range(4)]
    out = [None] * 16
    for fa in range(4):
        o = _dft4([_tw16(hh[a0][fa], a0 * fa, inv) for a0 in range(4)], inv)
        for fb in range(4):
            out[fa + 4 * fb] = o[fb]
    return out


def _gwin(g):
    lo, hi = 80 * g, 80 * g + 79
    if lo // 128 == hi // 128:
        return ("nat", lo // 128, lo - 128 * (lo // 128))
    t = (lo - 64) // 128
    return ("shf", t, lo - 64 - 128 * t)


def _kernel(xa_hbm, wr_hbm, wi_hbm, xb_hbm, wqkv_hbm, wo_hbm, ff_hbm, gg_hbm, rr_hbm, out_hbm,
            xa32, wr32, wi32, wr_last, wi_last, ff32, gg32, rr32, ys_ref, zs_ref, ysc_ref, oa32,
            pin_ref, qw01_ref, xq_ref, xb32, wqkv32, wo32, wvt32, s_ref, p_ref, ob32, ot_ref, qw_ref, xz_ref, obo32,
            sem, osem, wsem, *groups):
    gs_refs = groups[0:4]
    kw_refs = groups[4:12]
    vt_refs = groups[12:20]

    def copy(src, dst, k):
        return pltpu.make_async_copy(src, dst, sem.at[k])

    xbh = xb_hbm.bitcast(i32)
    wqh = wqkv_hbm.bitcast(i32)
    xah = xa_hbm.bitcast(i32)
    oh32 = out_hbm.bitcast(i32)
    c_x0 = copy(xbh.at[pl.ds(0, 128)], xb32.at[pl.ds(0, 128)], 0)
    c_wk = copy(wqh.at[:, pl.ds(640, 640)], wqkv32.at[:, pl.ds(640, 640)], 1)
    c_wv = copy(wqh.at[:, pl.ds(1280, 640)], wqkv32.at[:, pl.ds(1280, 640)], 2)
    c_x1 = copy(xbh.at[pl.ds(128, 192)], xb32.at[pl.ds(128, 192)], 3)
    c_wq = copy(wqh.at[:, pl.ds(0, 640)], wqkv32.at[:, pl.ds(0, 640)], 4)
    c_ff = copy(ff_hbm, ff32, 5)
    c_xa = [copy(xah.at[:, pl.ds(128 * t, 128)], xa32.at[t], 6 + t) for t in range(5)]
    c_rr = copy(rr_hbm, rr32, 11)
    c_w = []
    for n, (src, dst, dst1) in enumerate(((wr_hbm, wr32, wr_last), (wi_hbm, wi32, wi_last))):
        w320 = src.at[pl.ds(0, 320)].bitcast(i32)
        for t in range(NB):
            c_w.append(pltpu.make_async_copy(w320.at[:, pl.ds(128 * t, 128)], dst.at[t], wsem.at[0]))
        c_w.append(copy(src.at[pl.ds(320, 1)], dst1, 13 + n))
    c_x2 = copy(xbh.at[pl.ds(320, 704)], xb32.at[pl.ds(320, 704)], 21)
    c_wo = copy(wo_hbm.bitcast(i32), wo32, 22)
    c_gg = copy(gg_hbm, gg32, 23)
    c_pin = copy(xbh.at[pl.ds(0, 8), pl.ds(0, 128)], pin_ref.at[0], 24)
    c_pin2 = copy(xbh.at[pl.ds(0, 8), pl.ds(0, 128)], pin_ref.at[1], 12)
    for cp in ([c_x0, c_wk, c_wv, c_x1, c_wq, c_ff] + c_xa + [c_rr]
               + c_w + [c_x2, c_wo, c_gg, c_pin, c_pin2]):
        cp.start()

    scale = float(DH ** -0.5 * np.log2(np.e))
    def _qpos(l):
        return (l & 16) + 4 * (l & 3) + ((l & 15) >> 2)
    rr_ = lax.broadcasted_iota(i32, (32, 128), 0)
    ll_ = _qpos(lax.broadcasted_iota(i32, (32, 128), 1))
    pos_ = rr_ & 15
    key_ = (rr_ & 16) + jnp.where(pos_ < 8, 2 * pos_, 2 * (pos_ - 8) + 1)
    le32 = key_ <= ll_
    wr_ = lax.broadcasted_iota(i32, (16, 128), 0)
    wq_ = _qpos(lax.broadcasted_iota(i32, (16, 128), 1))
    le_pk = (jnp.where(2 * wr_ <= wq_, jnp.int32(0xFFFF), jnp.int32(0))
             | jnp.where(2 * wr_ + 1 <= wq_, jnp.int32(-65536), jnp.int32(0)))
    lane8 = lax.broadcasted_iota(i32, (8, 128), 1)
    lane16 = lax.broadcasted_iota(i32, (16, 128), 1)
    bit0 = (lane16 & 32) != 0
    bit1 = (lane16 & 64) != 0
    bit0_8 = (lane8 & 32) != 0
    sub4 = lax.broadcasted_iota(i32, (8, 128), 0) < 4
    sub0 = lax.broadcasted_iota(i32, (8, 128), 0) == 0
    ones8 = jnp.ones((8, 128), f32)
    lo64 = lax.broadcasted_iota(i32, (64, 128), 1) < 64

    def wrows_of(i):
        return i * 64 if isinstance(i, int) else pl.multiple_of(i * 64, 64)

    def prep_wvt():
        for tr in range(5):
            wvt32[64 * tr:64 * tr + 64, :] = pltpu.bitcast(
                _b16(wqkv32[:, 1280 + tr * 128:1280 + (tr + 1) * 128]).T, i32)

    def prep_x(i):
        w = xb32[pl.ds(wrows_of(i), 64), :]
        z1 = _zip16(_b16(w).astype(f32))
        xz_ref[0] = z1
        xz_ref[1] = _zip16(_b16(z1).astype(f32))

    def win_ready(tiles, rolled, done, emit):
        for g in range(8):
            if g in done:
                continue
            kind, t, _ = _gwin(g)
            if kind == "nat":
                if t in tiles:
                    emit(g, tiles[t])
                    done.add(g)
            elif t in tiles and (t + 1) in tiles:
                for tt in (t, t + 1):
                    if tt not in rolled:
                        rolled[tt] = pltpu.roll(tiles[tt], 64, 1)
                emit(g, jnp.where(lo64, rolled[t], rolled[t + 1]))
                done.add(g)

    def proj_pieces(i, do_q=True, do_kv=True, qdst=None, xz=None):
        qdst = qw_ref if qdst is None else qdst
        xz = xz_ref.at[0] if xz is None else xz
        pieces = {}
        if do_kv:
            v8 = {}
            vdone = set()

            def vpiece(r):
                def f():
                    xb = _b16(xb32[pl.ds(wrows_of(i), 64), :])
                    vt = _dot_nt(_b16(wvt32[64 * r:64 * r + 64, :]), xb)
                    for j in range(16):
                        v8[16 * r + j] = vt[8 * j:8 * j + 8]
                    for p in range(16):
                        if p in vdone or any((5 * p + j) not in v8 for j in range(5)):
                            continue
                        v = [v8[5 * p + j] for j in range(5)]
                        h0, h1 = 2 * p, 2 * p + 1
                        vt_refs[h0 // 4][h0 % 4, i] = jnp.concatenate([v[0], v[1], v[2], ones8], 0).astype(bf)
                        vt_refs[h1 // 4][h1 % 4, i] = jnp.concatenate([v[2], v[3], v[4], ones8], 0).astype(bf)
                        vdone.add(p)
                return f

            kt, kr, kd = {}, {}, set()

            def kpiece(t):
                def f():
                    kt[t] = _zip16(_dot(_b16(xz_ref[1]), _b16(wqkv32[:, 640 + 128 * t:640 + 128 * t + 128])))

                    def emit(g, val):
                        kw_refs[g][pl.ds(wrows_of(i), 64), :] = val
                    win_ready(kt, kr, kd, emit)
                return f

            for r in range(5):
                pieces["v%d" % r] = vpiece(r)
                pieces["k%d" % r] = kpiece(r)
        if do_q:
            qt, qr, qd = {}, {}, set()

            def qpiece(t):
                def f():
                    qt[t] = _zip16(_dot(_b16(xz[...]), _b16(wqkv32[:, 128 * t:128 * t + 128])) * scale)

                    def emit(g, val):
                        qdst[g] = val
                    win_ready(qt, qr, qd, emit)
                return f

            for t in range(5):
                pieces["q%d" % t] = qpiece(t)
        return pieces

    def out_pieces(i, slot=1):
        def opiece(t):
            def f():
                res = _dot(_b16(ob32[slot]), _b16(wo32[:, 128 * t:128 * t + 128]))
                obo32[pl.ds(wrows_of(i), 64), 128 * t:128 * t + 128] = _zip16(res)
            return f
        return {"o%d" % t: opiece(t) for t in range(5)}

    def key_tiles(i):
        return list(range(3)) if (not isinstance(i, int) or i >= 2) else list(range(2 - i, 3))

    pv_outs = {}

    def pv_group(g, i, es=(0, 1, 2, 3)):
        tiles = key_tiles(i)
        sl = g % 2
        for e in es:
            P = _b16(p_ref[sl, e, 64 * tiles[0]:192, :])
            if len(tiles) > 1:
                vw = jnp.concatenate([vt_refs[g][e, i - 2 + j] for j in tiles], 1)
            else:
                vw = vt_refs[g][e, i]
            o = _dot(vw, P)
            rl = pltpu.reciprocal(o[24:32])
            res = [o[0:8] * rl, o[8:16] * rl, o[16:24] * rl]
            if e == 2:
                res = [pltpu.roll(r, 64, 1) for r in res]
            elif e == 1:
                res = [jnp.where(bit0_8, pltpu.roll(r, 32, 1), pltpu.roll(r, 96, 1)) for r in res]
            elif e == 3:
                res = [jnp.where(bit0_8, pltpu.roll(r, 96, 1), pltpu.roll(r, 32, 1)) for r in res]
            pv_outs[(g, e)] = res
            if (g, e ^ 1) in pv_outs:
                p = e // 2
                a, b = pv_outs.pop((g, 2 * p)), pv_outs.pop((g, 2 * p + 1))
                ot_ref[80 * g + 40 * p:80 * g + 40 * p + 40, :] = jnp.concatenate(
                    [a[0], a[1], jnp.where(sub4, a[2], b[0]), b[1], b[2]], 0)

    def fin_tile(t, slot):
        ob32[slot, :, 128 * t:128 * t + 128] = _zip16(ot_ref[128 * t:128 * t + 128, :].T)

    def ob_slot(i):
        return {0: 0, 1: 2, 2: 3}.get(i, 1) if isinstance(i, int) else 1

    def finish(i):
        def f():
            pv_group(7, i)
            fin_tile(4, ob_slot(i))
        return f

    last_m = {}

    def token():
        return jnp.broadcast_to(last_m[max(last_m)], (8, 128))

    def attn(i, plan, head=None, qsrc=None, lazy=False):
        qsrc = qw_ref if qsrc is None else qsrc
        static = isinstance(i, int)
        lov = (lambda u: max(0, 8 - u - 4 * i)) if static else (lambda u: 0)
        tiles = key_tiles(i)
        ms = last_m

        def phase_a(g, us):
            _, _, off = _gwin(g)
            hm = [jnp.where((lane16 >= off + 20 * e) & (lane16 < off + 20 * e + 20), jnp.int32(-1), jnp.int32(0))
                  for e in range(4)]
            for u in us:
                lo = lov(u)
                nrow = 32 * (9 - lo)
                k0 = 64 * i - 128 + 16 * u + 16 * lo
                if not static:
                    k0 = pl.multiple_of(k0, 16)
                kw = _b16(kw_refs[g][pl.ds(k0, nrow // 2), :])
                qu = qsrc[g, 16 * u:16 * u + 16, :]
                qm = _b16(jnp.concatenate([qu & hm[lam ^ u] for lam in range(4)], 0))
                s = _dot_nt(kw, qm)
                sd = s[nrow - 32:nrow]
                if lo == 0:
                    T = jnp.where(le32, sd, s[0:32])
                    F = s[32:256]
                else:
                    T = jnp.where(le32, sd, NEG)
                    F = s[0:nrow - 32]
                m = jnp.max(T, axis=0, keepdims=True)
                s_ref[u, 0:32] = T
                if F.shape[0] > 0:
                    m = jnp.maximum(m, jnp.max(F, axis=0, keepdims=True))
                    s_ref[u, 32:32 + F.shape[0]] = F
                ms[(g, u)] = m

        def sel(m, a, b):
            if a is None and b is None:
                return None
            if a is None:
                a = jnp.zeros((16, 128), i32)
            if b is None:
                b = jnp.zeros((16, 128), i32)
            return jnp.where(m, a, b)

        def phase_b1(g):
            slp = g % 2
            lo_ = [lov(u) for u in range(4)]
            nf = [7 if lo_[u] == 0 else 8 - lo_[u] for u in range(4)]

            def pblock(u, row0):
                p = jnp.exp2(s_ref[u, row0:row0 + 32] - ms[(g, u)])
                return jnp.concatenate([_packi(p[16 * j:16 * j + 8], p[16 * j + 8:16 * j + 16]) for j in range(2)], 0)

            tri = {}

            def block(u, rel):
                if rel < 0 or rel > 8:
                    return None
                if rel == 0 or rel == 8:
                    if u not in tri:
                        pt = pblock(u, 0)
                        if lo_[u] == 0:
                            p8 = pt & le_pk
                            tri[u] = {8: p8, 0: pt ^ p8}
                        else:
                            tri[u] = {8: pt, 0: None}
                    return tri[u][rel]
                first = 8 - nf[u]
                if rel < first:
                    return None
                return pblock(u, 32 + 32 * (rel - first))

            for beta in range(4 * tiles[0], 12):
                src = [block(u, beta - u) for u in range(4)]
                a0 = sel(bit0, src[1], src[0])
                a1 = sel(bit0, src[0], src[1])
                c0 = sel(bit0, src[3], src[2])
                c1 = sel(bit0, src[2], src[3])
                o4 = [sel(bit1, c0, a0), sel(bit1, c1, a1), sel(bit1, a0, c0), sel(bit1, a1, c1)]
                for e in range(4):
                    p_ref[slp, e, 16 * beta:16 * beta + 16, :] = (
                        o4[e] if o4[e] is not None else jnp.zeros((16, 128), i32))

        okey = "order" if not static else ("order_pre" if i in (2, 3) else ("order_post" if i == NB - 1 else "order_01"))
        order = {"order": "B P0 A0 A1 A2 A3 P1 P2 P3 X X Y",
                 "order_pre": "B A0 A1 P0 A2 P1 A3 P2 P3 X X Y",
                 "order_post": "B A0 A1 A2 P0 P1 P2 A3 P3 X X Y",
                 "order_01": "B P0 P1 A0 A1 A2 A3 P2 P3 X X Y"}[okey]

        def step(s):
            if s == -1 and head is not None:
                head()
            px = plan.get(s, [])
            todo = list(range(len(px)))
            for tok in order.split():
                if tok[0] == "A" and 0 <= s + 1 < 8:
                    phase_a(s + 1, [int(c) for c in tok[1:]])
                if tok[0] == "B" and 0 <= s < 8:
                    phase_b1(s)
                if tok[0] == "P" and 0 <= s - 1 < 8:
                    pv_group(s - 1, i, [int(c) for c in tok[1:]])
                if tok[0] == "X" and todo:
                    px[todo.pop(0)]()
                if tok[0] == "Y":
                    while todo:
                        px[todo.pop(0)]()
            while todo:
                px[todo.pop(0)]()
            if s == 7:
                for t in range(4):
                    fin_tile(t, ob_slot(i))

        steps = [(lambda s=s: step(s)) for s in range(-1, 8)]
        if lazy:
            return steps
        for f in steps:
            f()

    def a1_step(ax, ay, order):
        w = {}
        if ax is not None:
            j, par = ax // 2, ax % 2
            x = [_unpacki(xa32[t, pl.ds(j, 128, stride=8), :], par) for t in range(5)]
            t1 = x[1] + x[4]
            t2 = x[2] + x[3]
            t3 = x[1] - x[4]
            t4 = x[2] - x[3]
            p1 = x[0] + C1 * t1 + C2 * t2
            p2 = x[0] + C2 * t1 + C1 * t2
            q1 = S1 * t3 + S2 * t4
            q2 = S2 * t3 - S1 * t4
            ops = [x[0] + t1 + t2, p1 + q1, q1, p1, p2 + q2, q2, p2]
            w0s = [0, 80, 144, 208, 272, 336, 400, 464]
        for tok in order:
            if tok[0] == "x" and ax is not None:
                n = int(tok[1])
                w[tok] = _dot_nt(_b16(ff32[w0s[n]:w0s[n + 1]]), ops[n].astype(bf))
            if tok[0] == "y" and ay is not None:
                n = int(tok[1])
                w[tok] = _dot(ys_ref[ay % 2, n], _b16(rr32[ay, n]))
        if ay is not None:
            g_ = jnp.concatenate([w["y0"] - w["y1"], w["y0"] - w["y2"]], 1)
            for g in range(R // 8):
                gs_refs[g % 4][ay, 8 * (g // 4):8 * (g // 4) + 8, :] = g_[8 * g:8 * g + 8]
        if ax is not None:
            re, im = [w["x0"][0:80]], [w["x0"][80:160]]
            for n in (1, 4):
                t1, t2, t3 = w["x%d" % n], w["x%d" % (n + 1)], w["x%d" % (n + 2)]
                re.append(t1 - t2)
                im += [t3[0:64] - t1[0:64], t1[64:128] - t3[64:128]]
            yr = jnp.concatenate(re, 0)
            yi = jnp.concatenate(im, 0)
            ys_ref[ax % 2, 0] = (yr + yi).astype(bf)
            ys_ref[ax % 2, 1] = yi.astype(bf)
            ys_ref[ax % 2, 2] = yr.astype(bf)

    def a2_group(n, gq, token=None):
        g = 4 * gq + n
        special = isinstance(gq, int) and g == 8
        if isinstance(gq, int):
            w8 = g if g < 8 else (g - 10) % 8
            c10 = [0, 1, 4, 2, 3][0 if g < 8 else (g - 10) // 8 + 1] + 5 * (w8 // 4)
            r0 = 8 * gq
        else:
            w8 = jnp.where(g < 8, g, (g - 10) & 7)
            blk = jnp.minimum(jnp.where(g < 10, 0, ((g - 10) >> 3) + 1), 4)
            c10 = jnp.where(blk == 2, 4, jnp.where(blk > 2, blk - 1, blk)) + 5 * (w8 >> 2)
            r0 = 8 * gq
            if n == 0:
                r0 = jnp.where(g == 8, 96, r0)
            r0 = pl.multiple_of(r0, 8)
        w0 = (c10 >> 1) + 40 * (w8 & 3)
        sh = 16 * (1 - (c10 & 1))

        def wload(ref, last, f1):
            if special:
                return jnp.broadcast_to(last[0:1, 128 * f1:128 * f1 + 128].astype(f32), (8, 128))
            return pltpu.bitcast((ref[f1, pl.ds(w0, 8, stride=5), :] << sh) & jnp.int32(-65536), f32)

        gref = gs_refs[n]
        if token is not None:
            gref[16, pl.ds(pl.multiple_of(8 * (gq & 15), 8), 8), 0:128] = token
        z = [(gref[a, pl.ds(r0, 8), 0:128], gref[a, pl.ds(r0, 8), 128:256]) for a in range(16)]
        X = _fft16(z, False)
        V = []
        for f1 in range(16):
            wr = wload(wr32, wr_last, f1)
            wi = wload(wi32, wi_last, f1)
            V.append((X[f1][0] * wr - X[f1][1] * wi, X[f1][0] * wi + X[f1][1] * wr))
        U = _fft16(V, True)
        for a in range(16):
            gref[a, pl.ds(r0, 8), 0:128] = U[a][0]
            gref[a, pl.ds(r0, 8), 128:256] = U[a][1]

    def a3_step(az, ad, order, extra=()):
        w = {}
        if az is not None:
            u = jnp.concatenate([gs_refs[g % 4][az, 8 * (g // 4):8 * (g // 4) + 8, :] for g in range(R // 8)], 0)
            ur = u[:, 0:128]
            ui = u[:, 128:256]
            zops = [(ur + ui, 0), (ui, 2), (ur, 1)]
        for tok in order:
            if tok[0] == "z" and az is not None:
                v, n = zops[int(tok[1])]
                w[tok] = _dot_nt(v.astype(bf), _b16(rr32[az, n]))
            if tok[0] == "d" and ad is not None:
                n = int(tok[1])
                w[tok] = _dot(zs_ref[ad % 2, n], _b16(gg32[64 * n:64 * n + 64]))
            if tok == "E":
                for f in extra:
                    f()
        if ad is not None:
            v0 = w["d0"]
            v1r, v1i = w["d1"] - w["d2"], w["d1"] + w["d3"]
            v2r, v2i = w["d4"] - w["d5"], w["d4"] + w["d6"]
            A1 = v0 + C1 * v1r + C2 * v2r
            A2 = v0 + C2 * v1r + C1 * v2r
            B1 = S1 * v1i + S2 * v2i
            B2 = S2 * v1i - S1 * v2i
            y = [v0 + v1r + v2r, A1 - B1, A2 - B2, A2 + B2, A1 + B1]
            for t in range(5):
                if ad % 2 == 0:
                    ysc_ref[t] = y[t]
                else:
                    oa32[t, pl.ds(ad // 2, 128, stride=8), :] = _packi(ysc_ref[t], y[t])
        if az is not None:
            zr = w["z0"] - w["z1"]
            zi = w["z0"] - w["z2"]
            kop = [jnp.concatenate([zr[0:64], jnp.where(sub0, zr[64:72], zi[0:8]), zi[8:64]], 0)]
            for r0 in (80, 208):
                kop += [jnp.concatenate([zr[r0:r0 + 64] + zi[r0:r0 + 64], zr[r0 + 64:r0 + 128] - zi[r0 + 64:r0 + 128]], 0),
                        zi[r0:r0 + 128], zr[r0:r0 + 128]]
            for n in range(7):
                zs_ref[az % 2, n] = kop[n].T.astype(bf)

    def run(pieces, order=None):
        for k in (order or list(pieces)):
            if k in pieces:
                pieces[k]()

    PLAN = {-1: ["v0", "v1"], 0: ["q0", "k0"], 1: ["k1", "q1", "a3"], 2: ["k2", "q2"], 3: ["o0", "o1", "a1"],
            4: ["k3", "q3"], 5: ["o2", "o3", "a0"], 6: ["v2", "o4", "a2"], 7: ["k4", "q4", "v3", "v4"]}

    def mkplan(pieces):
        return {s_: [pieces[k] for k in ks if k in pieces] for s_, ks in PLAN.items()}

    def out_b_copy(i):
        return pltpu.make_async_copy(obo32.at[pl.ds(wrows_of(i), 64)],
                                     oh32.at[pl.ds(wrows_of(i), 64), pl.ds(D, D)], osem.at[0])

    for g in range(R // 8, 44):
        gs_refs[g % 4][0:16, 8 * (g // 4):8 * (g // 4) + 8, :] = jnp.zeros((16, 8, 256), f32)
    gs_refs[0][0:16, 96:104, :] = jnp.zeros((16, 8, 256), f32)
    c_x0.wait()
    c_wk.wait()
    prep_x(0)
    P0 = proj_pieces(0, do_q=False)
    run(P0, ["k0", "k1", "k2", "k3", "k4"])
    prep_x(1)
    P1 = proj_pieces(1, do_q=False)
    VS = ["v0", "v1", "v2", "v3", "v4"]
    run(P1, ["k0", "k1", "k2"])
    c_wv.wait()
    prep_wvt()
    run(P1, ["k3", "k4"])
    run(P0, VS)
    run(P1, VS)
    c_x1.wait()
    c_wq.wait()
    prep_x(2)
    run(proj_pieces(2), ["q0", "k0", "q1", "k1", "q2", "k2", "q3", "k3", "q4", "k4"] + VS)
    for i_ in range(2):
        xq_ref[i_] = _zip16(_b16(xb32[64 * i_:64 * i_ + 64, :]).astype(f32))

    def with_q(P, i_):
        Pq = proj_pieces(i_, do_kv=False, qdst=qw01_ref.at[i_], xz=xq_ref.at[i_])
        P.update({"o%d" % t: Pq["q%d" % t] for t in range(5)})
        return P

    prep_x(3)
    attn(2, mkplan(with_q(proj_pieces(3), 0)))
    prep_x(4)
    attn(3, mkplan(with_q(proj_pieces(4), 1)), head=finish(2))

    for cp in [c_ff] + c_xa + [c_rr]:
        cp.wait()
    a1o = "x0 x1 x2 x3 y0 x4 y1 x5 y2 x6".split()
    a1_step(0, None, a1o)
    for a in range(16):
        a1_step(a + 1 if a < 15 else None, a, a1o)
    for cp in c_w:
        cp.wait()
    c_x2.wait()
    c_wo.wait()
    c_gg.wait()

    def body(i, carry):
        nxt = jnp.minimum(i + 1, NB - 1)
        prep_x(nxt)
        P = proj_pieces(nxt)
        P.update(out_pieces(i - 1))
        for n in range(4):
            P["a%d" % n] = (lambda n=n: a2_group(n, i - 4, token()))
        last_m.clear()
        attn(i, mkplan(P), head=finish(i - 1))
        out_b_copy(i - 1).start()
        return carry

    lax.fori_loop(4, NB - 1, body, 0)

    finish(NB - 2)()
    a2_group(0, 2)

    extra = attn(0, {}, qsrc=qw01_ref.at[0], lazy=True) + attn(1, {}, head=finish(0), qsrc=qw01_ref.at[1], lazy=True)
    extra += [lambda: pv_group(7, 1), lambda: fin_tile(4, 2)]
    a3o = "z0 E z1 z2 d0 d1 d2 d3 d4 d5 d6".split()
    cut = [0, 1, 2, 2, 5, 5, 7, 8, 10, 11, 12, 13, 15, 16, 18, 18, 20]
    a3_step(0, None, a3o)
    for a in range(16):
        a3_step(a + 1 if a < 15 else None, a, a3o, extra[cut[a]:cut[a + 1]])
    c_oa = [pltpu.make_async_copy(oa32.at[t], oh32.at[:, pl.ds(128 * t, 128)], osem.at[1 + t]) for t in range(5)]
    for cp in c_oa:
        cp.start()
    c_pin.wait()

    fill = []
    for t in range(5):
        fill += [out_pieces(0, slot=0)["o%d" % t], out_pieces(1, slot=2)["o%d" % t], out_pieces(NB - 2)["o%d" % t]]
    last_m.clear()
    fc = [0, 2, 4, 4, 6, 8, 10, 11, 13, 15]
    attn(NB - 1, {s_: fill[fc[s_ + 1]:fc[s_ + 2]] for s_ in range(-1, 8)})
    for i_ in (0, 1, NB - 2):
        out_b_copy(i_).start()
    c_pin2.wait()
    pv_group(7, NB - 1)
    run(out_pieces(2, slot=3))
    out_b_copy(2).start()
    fin_tile(4, 1)
    run(out_pieces(NB - 1))
    out_b_copy(NB - 1).start()

    for cp in c_oa:
        cp.wait()
    for i in range(NB):
        out_b_copy(i).wait()


def _build(FF32, GG32, RR32):
    scratch = [
        pltpu.VMEM((5, S // 2, 128), i32),
        pltpu.VMEM((NB, 160, 128), i32), pltpu.VMEM((NB, 160, 128), i32),
        pltpu.VMEM((1, S), bf), pltpu.VMEM((1, S), bf),
        pltpu.VMEM(FF32.shape, i32), pltpu.VMEM(GG32.shape, i32), pltpu.VMEM(RR32.shape, i32),
        pltpu.VMEM((2, 3, R, 128), bf),
        pltpu.VMEM((2, 7, 128, 128), bf),
        pltpu.VMEM((5, 128, 128), f32),
        pltpu.VMEM((5, S // 2, 128), i32),
        pltpu.VMEM((2, 8, 128), i32),
        pltpu.VMEM((2, 8, 64, 128), i32),
        pltpu.VMEM((2, 64, D), i32),
        pltpu.VMEM((S // 2, D), i32),
        pltpu.VMEM((D // 2, 3 * D), i32),
        pltpu.VMEM((D // 2, D), i32),
        pltpu.VMEM((D // 2, D), i32),
        pltpu.VMEM((4, 256, 128), f32),
        pltpu.VMEM((2, 4, 192, 128), i32),
        pltpu.VMEM((4, 64, D), i32),
        pltpu.VMEM((D, 128), f32),
        pltpu.VMEM((8, 64, 128), i32),
        pltpu.VMEM((2, 64, D), i32),
        pltpu.VMEM((S // 2, D), i32),
        pltpu.SemaphoreType.DMA((25,)),
        pltpu.SemaphoreType.DMA((6,)),
        pltpu.SemaphoreType.DMA((1,)),
    ]
    scratch += [pltpu.VMEM((17, 104, 256), f32)] * 4
    scratch += [pltpu.VMEM((S // 2, 128), i32)] * 8
    scratch += [pltpu.VMEM((4, NB, 32, 128), bf)] * 8
    return pl.pallas_call(
        _kernel,
        out_shape=jax.ShapeDtypeStruct((S, 2 * D), bf),
        in_specs=[pl.BlockSpec(memory_space=pl.ANY)] * 9,
        out_specs=pl.BlockSpec(memory_space=pl.ANY),
        scratch_shapes=scratch,
        compiler_params=pltpu.CompilerParams(vmem_limit_bytes=110 * 2 ** 20),
    )


@jax.jit
def pallas_concat_heads__spectral_gfnet__sliding_block__prompt_kernel(
    A_x: jax.Array,
    A_w_r: jax.Array,
    A_w_i: jax.Array,
    B_x: jax.Array,
    B_wqkv: jax.Array,
    B_wo: jax.Array,
):
    FF32, GG32, RR32 = _make_consts()
    out = _build(FF32, GG32, RR32)(
        A_x.reshape(S, D), A_w_r.T, A_w_i.T, B_x.reshape(S, D), B_wqkv, B_wo,
        jnp.asarray(FF32), jnp.asarray(GG32), jnp.asarray(RR32))
    return out.reshape(1, S, 2 * D)
```
